```python
import jax
import jax.numpy as jnp

def _softmax(x, axis=-1):
    return jax.nn.softmax(x, axis=axis)

def _gelu(x):
    return jax.nn.gelu(x, approximate=True)

def _silu(x):
    return jax.nn.silu(x)

def _sigmoid(x):
    return jax.nn.sigmoid(x)

def _layernorm(x, axis=-1, eps=1e-05):
    m = jnp.mean(x, axis=axis, keepdims=True)
    v = jnp.var(x, axis=axis, keepdims=True)
    return (x - m) / jnp.sqrt(v + eps)

def _scatter_add(tgt, idx, src, axis=0):
    return tgt.at[idx].add(src)

def _segment_sum(src, seg, n):
    return jax.ops.segment_sum(src, seg, n)

class _Rng:

    def __init__(self, key):
        self._k = key

    def _next(self):
        self._k, sub = jax.random.split(self._k)
        return sub

    def normal(self, shape):
        return jax.random.normal(self._next(), shape, dtype=jnp.bfloat16)

    def randint(self, lo, hi, shape):
        return jax.random.randint(self._next(), shape, lo, hi, dtype=jnp.int32)

    def uniform(self, shape, lo=0.0, hi=1.0):
        return jax.random.uniform(self._next(), shape, jnp.bfloat16, lo, hi)

    def permutation(self, n):
        return jax.random.permutation(self._next(), n)
kernel_name = 'concat_heads__memory_aug_recurrent_mem_tr__sliding_local_dilated__prompt'

def setup_inputs():
    _rng = _Rng(jax.random.key(int.from_bytes(__import__("os").urandom(4), "little")))
    _w = lambda a: (lambda t: t.astype(jnp.bfloat16) if jnp.issubdtype(t.dtype, jnp.floating) else t)(jnp.asarray(a))

    def _A_setup():
        B, S, Dm = (1, 2048, 1024)
        H, Dh = (32, 128)
        M, seg = (8, 32)
        seg = min(seg, S)
        S = S // seg * seg
        return {'x': _w((lambda *s: _rng.normal(s) * 0.05)(B, S, Dm)), 'mem0': _w((lambda *s: _rng.normal(s) * 0.05)(B, M, Dm)), 'Wq': _w((lambda *s: _rng.normal(s) * 0.05)(Dm, H, Dh) * Dm ** (-0.5)), 'Wk': _w((lambda *s: _rng.normal(s) * 0.05)(Dm, H, Dh) * Dm ** (-0.5)), 'Wv': _w((lambda *s: _rng.normal(s) * 0.05)(Dm, H, Dh) * Dm ** (-0.5)), 'Wo': _w((lambda *s: _rng.normal(s) * 0.05)(H, Dh, Dm) * (H * Dh) ** (-0.5)), 'seg_len': seg}
    _A_in = _A_setup()

    def _B_setup():
        B, S, D = (1, 2048, 1024)
        return {'x': _w((lambda *s: _rng.normal(s) * 0.05)(B, S, D)), 'wqkv': _w((lambda *s: _rng.normal(s) * 0.05)(D, 3 * D)), 'wo': _w((lambda *s: _rng.normal(s) * 0.05)(D, D))}
    _B_in = _B_setup()
    return {'A_x': _A_in['x'], 'A_mem0': _A_in['mem0'], 'A_Wq': _A_in['Wq'], 'A_Wk': _A_in['Wk'], 'A_Wv': _A_in['Wv'], 'A_Wo': _A_in['Wo'], 'A_seg_len': _A_in['seg_len'], 'B_x': _B_in['x'], 'B_wqkv': _B_in['wqkv'], 'B_wo': _B_in['wo']}

def reference(A_x, A_mem0, A_Wq, A_Wk, A_Wv, A_Wo, A_seg_len, B_x, B_wqkv, B_wo):

    def _A_ref(x, mem0, Wq, Wk, Wv, Wo, seg_len):
        B, S, Dm = x.shape
        H, Dh = (Wq.shape[1], Wq.shape[2])
        M = mem0.shape[1]
        scale = Dh ** (-0.5)
        n_seg = S // seg_len
        L = M + seg_len
        idx = jnp.arange(L)
        mask = (idx[:, None] < M) | (idx[:, None] >= idx[None, :])
        mem = mem0
        outs = []
        for s in range(n_seg):
            xs = x[:, s * seg_len:(s + 1) * seg_len, :].copy()
            h = jnp.concatenate([mem, xs], axis=1)
            q = jnp.einsum('btd,dhe->bhte', h, Wq)
            k = jnp.einsum('btd,dhe->bhte', h, Wk)
            v = jnp.einsum('btd,dhe->bhte', h, Wv)
            scores = jnp.einsum('bhqe,bhke->bhqk', q, k) * scale
            scores = jnp.where(mask[None, None], scores, -1000000000.0)
            p = _softmax(scores, axis=-1)
            o = jnp.einsum('bhqk,bhke->bhqe', p, v)
            o = jnp.einsum('bhte,hed->btd', o, Wo)
            mem = o[:, :M, :].copy()
            outs.append(o[:, M:, :])
        return jnp.concatenate(outs, axis=1)

    def _B_ref(x, wqkv, wo):
        B, S, D = x.shape
        H = 32
        Dh = D // H
        W, dil = (8, 2)
        qkv = (lambda x, *d: x.transpose(*d))((x @ wqkv).reshape(B, S, 3, H, Dh), 2, 0, 3, 1, 4)
        q, k, v = (qkv[0], qkv[1], qkv[2])
        scale = Dh ** (-0.5)
        pos = jnp.arange(S)
        off = jnp.arange(W) * dil
        idx = pos[:, None] - off[None, :]
        mask = idx >= 0
        idx_c = jnp.where(mask, idx, 0).reshape(-1)
        kg = k[:, :, idx_c, :].reshape(B, H, S, W, Dh)
        vg = v[:, :, idx_c, :].reshape(B, H, S, W, Dh)
        logits = jnp.einsum('bhsd,bhswd->bhsw', q, kg) * scale
        logits = jnp.where(mask[None, None, :, :], logits, -1000000000.0)
        attn = _softmax(logits, axis=-1)
        o = jnp.einsum('bhsw,bhswd->bhsd', attn, vg)
        return (lambda x, *d: x.transpose(*d))(o, 0, 2, 1, 3).reshape(B, S, D) @ wo
    a = _A_ref(A_x, A_mem0, A_Wq, A_Wk, A_Wv, A_Wo, A_seg_len)
    b = _B_ref(B_x, B_wqkv, B_wo)
    return jnp.concatenate([a, b], axis=-1)
```

```python
import functools

import jax
import jax.numpy as jnp
from jax import lax
import jax.experimental.pallas as pl
import jax.experimental.pallas.tpu as pltpu

bf16, f32, u32, i32 = jnp.bfloat16, jnp.float32, jnp.uint32, jnp.int32

S, DM = 2048, 1024
H, DH = 32, 128
M, SEG = 8, 32
L = M + SEG
DHB, WIN, DIL = 32, 8, 2
NC = DM // 128

TB = 64
UB = 4
HALO = 16
NIT = S // (TB * UB)
LQK, LPV, KA = 1, 3, 12

SEM_BW, SEM_BX, SEM_BWO, SEM_AW, SEM_AWO, SEM_AX, SEM_MEM, SEM_OB, SEM_OA = 0, 3, 11, 12, 18, 19, 20, 21, 22
NSEM = 23


def _b16(v):
    return pltpu.bitcast(v, bf16)


def _kernel(ax_h, mem_h, wq_h, wk_h, wv_h, wo_h, bx_h, bw_h, bwo_h, out_h,
            ax_v, mem_v, raw_v, wa_v, wo_v, bx_v, bw_v, bwo_v, t32_v, outa_v, outb_v,
            qb_v, kb_v, vb_v, ob_v, mem_s, stash, ostash, o_s, sem):
    def bw_cp(n):
        return pltpu.make_async_copy(bw_h.at[:, pl.ds(128 * n, 128)], bw_v.at[n], sem.at[SEM_BW + n // 8])

    def bx_cp(it, j):
        rows = pl.ds(TB * UB * it, TB * UB)
        return pltpu.make_async_copy(bx_h.at[rows, pl.ds(128 * j, 128)], bx_v.at[j, rows, :], sem.at[SEM_BX + it])

    def bwo_cp(n):
        return pltpu.make_async_copy(bwo_h.at[:, pl.ds(128 * n, 128)], bwo_v.at[n], sem.at[SEM_BWO])

    def aw_cp(c):
        src = (wq_h, wk_h, wv_h)[c // 2]
        return pltpu.make_async_copy(src.at[pl.ds((c % 2) * (DM * H // 2), DM * H // 2), :], raw_v.at[c],
                                     sem.at[SEM_AW + c])

    def aw_wait(c):
        pltpu.make_async_copy(raw_v.at[c], raw_v.at[c], sem.at[SEM_AW + c]).wait()

    def awo_cp(n):
        return pltpu.make_async_copy(wo_h.at[:, pl.ds(128 * n, 128)], wo_v.at[n], sem.at[SEM_AWO])

    def ax_cp(j):
        return pltpu.make_async_copy(ax_h.at[:, pl.ds(128 * j, 128)], ax_v.at[j], sem.at[SEM_AX])

    mem_cp = pltpu.make_async_copy(mem_h, mem_v, sem.at[SEM_MEM])

    def ob_cp(r0, n):
        return pltpu.make_async_copy(outb_v.at[pl.ds(r0, n), :], out_h.at[pl.ds(r0, n), pl.ds(DM, DM)],
                                     sem.at[SEM_OB])

    def oa_cp(r0, n):
        return pltpu.make_async_copy(outa_v.at[pl.ds(r0, n), :], out_h.at[pl.ds(r0, n), pl.ds(0, DM)],
                                     sem.at[SEM_OA])

    for n in range(8):
        bw_cp(n).start()
    for j in range(NC):
        bx_cp(0, j).start()
    for n in range(8, 24):
        bw_cp(n).start()
    for n in range(NC):
        bwo_cp(n).start()

    bxu, bwu, bwou = bx_v.bitcast(u32), bw_v.bitcast(u32), bwo_v.bitcast(u32)
    rawu, wou, axu = raw_v.bitcast(u32), wo_v.bitcast(u32), ax_v.bitcast(u32)

    lane = lax.broadcasted_iota(i32, (8, 128), 1)
    sub = lax.broadcasted_iota(i32, (8, 128), 0)

    def perm_section(s):
        bits = [((lane >> b) & 1) == 1 for b in range(3)]
        idx = [32 * ((lane >> 3) & 3) + 8 * (lane >> 5) + ((u + lane) & 7) for u in range(8)]

        def body(r8, c):
            for rr in range(8):
                rows = pl.ds(pl.multiple_of(r8 * 64 + rr * 8, 8), 8)
                z = [bwu[8 * s + (-t) % 8, rows, :] for t in range(8)]
                for b in range(3):
                    z = [jnp.where(bits[b], z[(t - (1 << b)) % 8], z[t]) for t in range(8)]
                for u in range(8):
                    bwu[8 * s + u, rows, :] = jnp.take_along_axis(z[u], idx[u], axis=1)
            return c
        lax.fori_loop(0, 8, body, 0)

    def prep_bwo():
        for n in range(NC):
            t32_v[n, 0:8, :] = jnp.zeros((8, 128), f32)
            t32_v[n, 8 + DM:16 + DM, :] = jnp.zeros((8, 128), f32)
            for r in range(0, DM, 128):
                t32_v[n, 8 + r:8 + r + 128, :] = _b16(bwou[n, r // 2:r // 2 + 64, :]).astype(f32)
        for n in range(NC):
            for u in range(8):
                for c in range(4):
                    for a2 in range(2):
                        parts = []
                        for A in (2 * a2, 2 * a2 + 1):
                            base = 32 * A + 8 * c + u
                            x = t32_v[n, pl.ds(8 + base, 8, stride=129), :]
                            if u > 0:
                                x = jnp.where(sub + u < 8, x, t32_v[n, pl.ds(base, 8, stride=129), :])
                            parts.append(x)
                        r = (128 * u + 32 * c + 16 * a2) // 2
                        bwou[n, r:r + 8, :] = pltpu.bitcast(jnp.concatenate(parts, axis=0).astype(bf16), u32)

    scale_b = DHB ** -0.5

    def b_qkv(i, st):
        r0 = i * (TB // 2)
        if not isinstance(r0, int):
            r0 = pl.multiple_of(r0, TB // 2)
        lhs = jnp.concatenate([_b16(bxu[j, pl.ds(r0, TB // 2), :]) for j in range(NC)], axis=1)
        for n in range(24):
            y = jnp.dot(lhs, _b16(bwu[n]), preferred_element_type=f32)
            if n < 8:
                qb_v[st, n] = y * scale_b
            elif n < 16:
                kb_v[st, n - 8, HALO:HALO + TB, :] = y
            else:
                vb_v[st, n - 16, HALO:HALO + TB, :] = y

    def b_halo(st, first):
        sp = (st - 1) % UB
        for u in range(8):
            if first:
                kb_v[st, u, 0:HALO, :] = jnp.zeros((HALO, 128), f32)
                vb_v[st, u, 0:HALO, :] = jnp.zeros((HALO, 128), f32)
            else:
                kb_v[st, u, 0:HALO, :] = kb_v[sp, u, TB:TB + HALO, :]
                vb_v[st, u, 0:HALO, :] = vb_v[sp, u, TB:TB + HALO, :]

    def b_attn(st, first):
        for g2 in range(TB // 16):
            o2 = []
            for g in (2 * g2, 2 * g2 + 1):
                r = 8 * g
                q = [qb_v[st, u, r:r + 8, :] for u in range(8)]
                lg = []
                for w in range(WIN):
                    a = HALO + r - DIL * w
                    p = q[0] * kb_v[st, 0, a:a + 8, :]
                    for u in range(1, 8):
                        p = p + q[u] * kb_v[st, u, a:a + 8, :]
                    p = p + pltpu.roll(p, 32, 1)
                    p = p + pltpu.roll(p, 64, 1)
                    if first and r - DIL * w < 0:
                        p = jnp.where(sub + (r - DIL * w) >= 0, p, -1e9)
                    lg.append(p)
                m = functools.reduce(jnp.maximum, lg)
                e = [jnp.exp(p - m) for p in lg]
                l = functools.reduce(lambda x, y: x + y, e)
                rc = pl.reciprocal(l, approx=True)
                rc = rc * (2.0 - l * rc)
                e = [x * rc for x in e]
                o = []
                for u in range(8):
                    acc = None
                    for w in range(WIN):
                        a = HALO + r - DIL * w
                        if first and r - DIL * w < 0:
                            vv = jnp.where(sub + (r - DIL * w) >= 0, vb_v[st, u, a:a + 8, :],
                                           vb_v[st, u, HALO:HALO + 1, :])
                        else:
                            vv = vb_v[st, u, a:a + 8, :]
                        t = e[w] * vv
                        acc = t if acc is None else acc + t
                    o.append(acc)
                o2.append(o)
            for u in range(8):
                ob_v[st, u, 8 * g2:8 * g2 + 8, :] = pltpu.bitcast(
                    jnp.concatenate([o2[0][u], o2[1][u]], axis=0).astype(bf16), u32)

    def b_proj(i, st):
        lhs = jnp.concatenate([_b16(ob_v[st, j]) for j in range(NC)], axis=1)
        y = jnp.concatenate([jnp.dot(lhs, _b16(bwou[n]), preferred_element_type=f32) for n in range(NC)], axis=1)
        r0 = i * TB
        if not isinstance(r0, int):
            r0 = pl.multiple_of(r0, TB)
        outb_v[pl.ds(r0, TB), :] = y.astype(bf16)

    def a_relayout(c, g0, g1):
        hb = (c // 2) * H
        rb = (c % 2) * (DM // 4)
        for g in range(g0, g1):
            uv = rawu.at[c, pl.ds(256 * g, 256), :]
            r = rb + 8 * g
            if not isinstance(r, int):
                r = pl.multiple_of(r, 8)
            for hp in range(16):
                a = uv[pl.ds(hp, 16, stride=16), :]
                lo = pltpu.bitcast(a << 16, f32).astype(bf16)
                hi = pltpu.bitcast(a & jnp.uint32(0xFFFF0000), f32).astype(bf16)
                wa_v[hb + 2 * hp, pl.ds(r, 8), :] = pltpu.bitcast(lo, u32)
                wa_v[hb + 2 * hp + 1, pl.ds(r, 8), :] = pltpu.bitcast(hi, u32)

    def b_iter(it, first, relayout):
        for k in range(UB):
            i = UB * it + k
            b_halo(k, first and k == 0)
            b_qkv(i, k)
            if first and k == 0:
                prep_bwo()
            if relayout is not None:
                a_relayout(relayout, 8 * k, 8 * k + 8)
            if not (first and k < 1):
                b_attn((k - 1) % UB, first and k == 1)
            if not (first and k < 2):
                b_proj(i - 2, (k - 2) % UB)

    for s in range(3):
        for n in range(8 * s, 8 * s + 8):
            bw_cp(n).wait()
        if s == 0:
            for it in range(1, NIT):
                for j in range(NC):
                    bx_cp(it, j).start()
            for c in range(6):
                aw_cp(c).start()
            for n in range(NC):
                awo_cp(n).start()
            for j in range(NC):
                ax_cp(j).start()
            mem_cp.start()
        perm_section(s)
    for j in range(NC):
        bx_cp(0, j).wait()
    for n in range(NC):
        bwo_cp(n).wait()
    b_iter(0, True, None)
    ob_cp(0, (UB - 2) * TB).start()
    for j in range(NC):
        bx_cp(1, j).wait()
    b_iter(1, False, None)
    ob_cp((UB - 2) * TB, UB * TB).start()

    def b_body(it, c):
        for j in range(NC):
            bx_cp(it, j).wait()
        aw_wait(it - 2)
        b_iter(it, False, it - 2)
        ob_cp(pl.multiple_of((UB * it - 2) * TB, TB), UB * TB).start()
        return c
    lax.fori_loop(2, NIT, b_body, 0)
    nb = S // TB
    b_attn(UB - 1, False)
    b_proj(nb - 2, UB - 2)
    b_proj(nb - 1, UB - 1)
    ob_cp(S - 2 * TB, 2 * TB).start()

    for n in range(NC):
        awo_cp(n).wait()
    for j in range(NC):
        ax_cp(j).wait()
    mem_cp.wait()

    scale_a = DH ** -0.5
    rr = lax.broadcasted_iota(i32, (2 * L, 2 * L), 0)
    cc = lax.broadcasted_iota(i32, (2 * L, 2 * L), 1)
    rb_, cb_ = rr >= L, cc >= L
    ri, ci = jnp.where(rb_, rr - L, rr), jnp.where(cb_, cc - L, cc)
    same = rb_ == cb_
    valid = same & ((ri < M) | (ri >= ci))
    fill = jnp.where(same, -1e9, -jnp.inf).astype(f32)

    mem_s[...] = mem_v[...].astype(f32)
    NP = H // 2

    def a_step(lhs, even):
        qkv, pp = {}, {}
        nrow = 32 if even else 48

        def do_qkv(j):
            res = []
            for wi in range(3):
                parts = []
                for hh in (2 * j, 2 * j + 1):
                    y = jnp.dot(lhs, _b16(wa_v[wi * H + hh]), preferred_element_type=f32)
                    if even:
                        stash[wi * H + hh] = y[32:40]
                        parts += [y[40:48], y[0:32]]
                    else:
                        parts += [y[0:8], stash[wi * H + hh], y[8:32]]
                res.append(jnp.concatenate(parts, axis=0).astype(bf16))
            qkv[j] = res

        def do_qk(j):
            q2, k2, _ = qkv[j]
            s = lax.dot_general(q2, k2, (((1,), (1,)), ((), ())), preferred_element_type=f32) * scale_a
            s = jnp.where(valid, s, fill)
            m = jnp.max(s, axis=1, keepdims=True)
            e = jnp.exp(s - m)
            l = jnp.sum(e, axis=1, keepdims=True)
            rc = pl.reciprocal(l, approx=True)
            rc = rc * (2.0 - l * rc)
            pp[j] = (e * rc).astype(bf16)

        def do_pv(j):
            o2 = jnp.dot(pp.pop(j), qkv.pop(j)[2], preferred_element_type=f32)
            for i, hh in enumerate((2 * j, 2 * j + 1)):
                o = o2[L * i:L * (i + 1)]
                if even:
                    o_s[hh, 0:16, :] = pltpu.bitcast(o[0:32].astype(bf16), u32)
                    ostash[hh] = o[32:40]
                else:
                    o_s[hh] = pltpu.bitcast(
                        jnp.concatenate([o[0:8], ostash[hh], o[8:40]], axis=0).astype(bf16), u32)

        def wo_part(n, h0, h1):
            lo = jnp.concatenate([_b16(o_s[hh, 0:nrow // 2, :]) for hh in range(h0, h1)], axis=1)
            return jnp.dot(lo, _b16(wou[n, h0 * 64:h1 * 64, :]), preferred_element_type=f32)

        for j in range(NP):
            do_qkv(j)
            if j - LQK >= 0:
                do_qk(j - LQK)
            if j - LPV >= 0:
                do_pv(j - LPV)
        ya = []
        nper = NC // (LPV + 1)
        for j in range(NP, NP + LPV):
            for _ in range(nper):
                ya.append(wo_part(len(ya), 0, 2 * KA))
            if j - LQK < NP:
                do_qk(j - LQK)
            do_pv(j - LPV)
        while len(ya) < NC:
            ya.append(wo_part(len(ya), 0, 2 * KA))
        return jnp.concatenate([wo_part(n, 2 * KA, H) + ya[n] for n in range(NC)], axis=1)

    def a_body(t, c):
        r0 = pl.multiple_of(t * 32, 32)
        X = jnp.concatenate([_b16(axu[j, pl.ds(r0, 32), :]) for j in range(NC)], axis=1)
        Xm = X[32:48].astype(f32)
        mixed = jnp.concatenate([Xm[0:8], mem_s[...]], axis=0).astype(bf16)
        ye = a_step(jnp.concatenate([X[0:32], mixed], axis=0), True)
        mixed = jnp.concatenate([ye[0:8], Xm[8:16]], axis=0).astype(bf16)
        yo = a_step(jnp.concatenate([mixed, X[48:64]], axis=0), False)
        mem_s[...] = yo[0:8]
        o0 = pl.multiple_of(t * 64, 64)
        outa_v[pl.ds(o0, 64), :] = jnp.concatenate([ye[8:32], yo[8:48]], axis=0).astype(bf16)
        oa_cp(o0, 64).start()
        return c
    lax.fori_loop(0, S // 64, a_body, 0)

    ob_cp(0, S).wait()
    oa_cp(0, S).wait()


@jax.jit
def _run(A_x, A_mem0, A_Wq, A_Wk, A_Wv, A_Wo, B_x, B_wqkv, B_wo):
    hbm = pl.BlockSpec(memory_space=pl.ANY)
    out = pl.pallas_call(
        _kernel,
        out_shape=jax.ShapeDtypeStruct((S, 2 * DM), bf16),
        in_specs=[hbm] * 9,
        out_specs=hbm,
        scratch_shapes=[
            pltpu.VMEM((NC, S, 128), bf16),
            pltpu.VMEM((M, DM), bf16),
            pltpu.VMEM((6, DM * H // 2, 128), bf16),
            pltpu.VMEM((3 * H, DM // 2, 128), u32),
            pltpu.VMEM((NC, H * DH, 128), bf16),
            pltpu.VMEM((NC, S, 128), bf16),
            pltpu.VMEM((24, DM, 128), bf16),
            pltpu.VMEM((NC, DM, 128), bf16),
            pltpu.VMEM((NC, DM + 16, 128), f32),
            pltpu.VMEM((S, DM), bf16),
            pltpu.VMEM((S, DM), bf16),
            pltpu.VMEM((UB, 8, TB, 128), f32),
            pltpu.VMEM((UB, 8, TB + HALO, 128), f32),
            pltpu.VMEM((UB, 8, TB + HALO, 128), f32),
            pltpu.VMEM((UB, 8, TB // 2, 128), u32),
            pltpu.VMEM((M, DM), f32),
            pltpu.VMEM((3 * H, 8, DH), f32),
            pltpu.VMEM((H, 8, DH), f32),
            pltpu.VMEM((H, 24, DH), u32),
            pltpu.SemaphoreType.DMA((NSEM,)),
        ],
        compiler_params=pltpu.CompilerParams(vmem_limit_bytes=110 * 1024 * 1024),
    )(
        A_x.reshape(S, DM), A_mem0.reshape(M, DM),
        A_Wq.reshape(DM * H, DH), A_Wk.reshape(DM * H, DH), A_Wv.reshape(DM * H, DH),
        A_Wo.reshape(H * DH, DM),
        B_x.reshape(S, DM), B_wqkv, B_wo,
    )
    return out.reshape(1, S, 2 * DM)


def pallas_concat_heads__memory_aug_recurrent_mem_tr__sliding_local_dilated__prompt_kernel(
    A_x, A_mem0, A_Wq, A_Wk, A_Wv, A_Wo, A_seg_len, B_x, B_wqkv, B_wo,
):
    if isinstance(A_seg_len, int):
        assert A_seg_len == SEG
    return _run(A_x, A_mem0, A_Wq, A_Wk, A_Wv, A_Wo, B_x, B_wqkv, B_wo)
```

```python
import functools

import jax
import jax.numpy as jnp
from jax import lax
import jax.experimental.pallas as pl
import jax.experimental.pallas.tpu as pltpu

bf16, f32, u32, i32 = jnp.bfloat16, jnp.float32, jnp.uint32, jnp.int32

S, DM = 2048, 1024
H, DH = 32, 128
M, SEG = 8, 32
L = M + SEG
DHB, WIN, DIL = 32, 8, 2
NC = DM // 128

TB = 64
UB = 4
HALO = 16
NIT = S // (TB * UB)
LQK, LPV, KA = 1, 3, 12

PITCH = DM // 2 + 2
STG_AW, STG_BW, STG_BWO = 0, 3 * DM * H, 3 * DM * H + 24 * DM
STG_TOK = STG_BWO + NC * DM
STG_ROWS = STG_TOK + 16
T32_ROWS = 8 + 128 + 8 * 129

SEM_BW, SEM_BX, SEM_BWO, SEM_AW, SEM_AWO, SEM_AX, SEM_MEM, SEM_OB, SEM_OA = 0, 3, 11, 12, 18, 19, 20, 21, 22
NSEM = 23


def _b16(v):
    return pltpu.bitcast(v, bf16)


def _interleave(dots, *filler_lists):
    pos = [0] * len(filler_lists)
    for n, d in enumerate(dots):
        d(any(pos[k] < len(f) and pos[k] * len(dots) <= n * len(f) for k, f in enumerate(filler_lists)))
        for k, f in enumerate(filler_lists):
            while pos[k] < len(f) and pos[k] * len(dots) <= n * len(f):
                f[pos[k]]()
                pos[k] += 1
    for k, f in enumerate(filler_lists):
        while pos[k] < len(f):
            f[pos[k]]()
            pos[k] += 1


def _kernel(ax_h, mem_h, wq_h, wk_h, wv_h, wo_h, bx_h, bw_h, bwo_h, out_h,
            ax_v, mem_v, stg_v, wa_v, wo_v, bx_v, bw_v, bwo_v, t32_v, outa_v, outb_v,
            buf_v, ob_v, mem_s, stash, ostash, o_s, zero_s, sem):
    def bw_cp(n):
        return pltpu.make_async_copy(bw_h.at[:, pl.ds(128 * n, 128)], stg_v.at[pl.ds(STG_BW + DM * n, DM), :],
                                     sem.at[SEM_BW + n // 8])

    def bx_cp(it, j):
        rows = pl.ds(TB * UB * it, TB * UB)
        return pltpu.make_async_copy(bx_h.at[rows, pl.ds(128 * j, 128)], bx_v.at[j, rows, :], sem.at[SEM_BX + it])

    def bwo_cp(n):
        return pltpu.make_async_copy(bwo_h.at[:, pl.ds(128 * n, 128)], stg_v.at[pl.ds(STG_BWO + DM * n, DM), :],
                                     sem.at[SEM_BWO])

    HW = DM * H // 2

    def aw_cp(c):
        src = (wq_h, wk_h, wv_h)[c // 2]
        return pltpu.make_async_copy(src.at[pl.ds((c % 2) * HW, HW), :], stg_v.at[pl.ds(STG_AW + c * HW, HW), :],
                                     sem.at[SEM_AW + c])

    def aw_wait(c):
        dst = stg_v.at[pl.ds(pl.multiple_of(STG_AW + c * HW, HW), HW), :]
        pltpu.make_async_copy(dst, dst, sem.at[SEM_AW + c]).wait()

    def awo_cp(n):
        return pltpu.make_async_copy(wo_h.at[:, pl.ds(128 * n, 128)], wo_v.at[n], sem.at[SEM_AWO])

    def ax_cp(j):
        return pltpu.make_async_copy(ax_h.at[:, pl.ds(128 * j, 128)], ax_v.at[j], sem.at[SEM_AX])

    mem_cp = pltpu.make_async_copy(mem_h, mem_v, sem.at[SEM_MEM])

    def ob_cp(r0, n):
        return pltpu.make_async_copy(outb_v.at[pl.ds(r0, n), :], out_h.at[pl.ds(r0, n), pl.ds(DM, DM)],
                                     sem.at[SEM_OB])

    def oa_cp(r0, n):
        return pltpu.make_async_copy(outa_v.at[pl.ds(r0, n), :], out_h.at[pl.ds(r0, n), pl.ds(0, DM)],
                                     sem.at[SEM_OA])

    for n in range(8):
        bw_cp(n).start()
    for j in range(NC):
        bx_cp(0, j).start()
    for n in range(8, 24):
        bw_cp(n).start()
    for n in range(NC):
        bwo_cp(n).start()

    bxu, stgu, obu, bwou = bx_v.bitcast(u32), stg_v.bitcast(u32), ob_v.bitcast(u32), bwo_v.bitcast(u32)
    wou, axu, osu = wo_v.bitcast(u32), ax_v.bitcast(u32), o_s.bitcast(u32)

    lane = lax.broadcasted_iota(i32, (8, 128), 1)
    sub = lax.broadcasted_iota(i32, (8, 128), 0)

    zero_s[0] = 0

    def zero():
        return pl.multiple_of(zero_s[0], 8)

    def token(y):
        stgu[STG_TOK // 2:STG_TOK // 2 + 8, :] = pltpu.bitcast(y[0:8], u32)

    PR = 32
    lane_p = lax.broadcasted_iota(i32, (PR, 128), 1)

    def perm_chunk(s, r, z):
        src = stgu.at[pl.ds(z + (STG_BW + 8 * s * DM) // 2, 4 * DM), :]
        zs = [src[((-t) % 8) * (DM // 2) + r:((-t) % 8) * (DM // 2) + r + PR, :] for t in range(8)]
        for b in range(3):
            bit = ((lane_p >> b) & 1) == 1
            zs = [jnp.where(bit, zs[(t - (1 << b)) % 8], zs[t]) for t in range(8)]
        for u in range(8):
            idx = 32 * ((lane_p >> 3) & 3) + 8 * (lane_p >> 5) + ((u + lane_p) & 7)
            bw_v[8 * s + u, r:r + PR, :] = jnp.take_along_axis(zs[u], idx, axis=1)

    def perm_fillers(s, z):
        return [functools.partial(perm_chunk, s, r, z) for r in range(0, DM // 2, PR)]

    def prep_bwo(n, z):
        t = t32_v.at[n % 2]
        src = stgu.at[pl.ds(z + (STG_BWO + n * DM) // 2, DM // 2), :]
        if n < 2:
            t[0:8, :] = jnp.zeros((8, 128), f32)
            t[8 + DM:16 + DM, :] = jnp.zeros((8, 128), f32)
        for r in range(0, DM, 128):
            t[8 + r:8 + r + 128, :] = _b16(src[r // 2:r // 2 + 64, :]).astype(f32)
        for u in range(8):
            for c in range(4):
                for a2 in range(2):
                    parts = []
                    for A in (2 * a2, 2 * a2 + 1):
                        base = 32 * A + 8 * c + u
                        x = t[pl.ds(8 + base, 8, stride=129), :]
                        if u > 0:
                            x = jnp.where(sub + u < 8, x, t[pl.ds(base, 8, stride=129), :])
                        parts.append(x)
                    r = 128 * u + 32 * c + 16 * a2
                    bwo_v[n, r:r + 16, :] = jnp.concatenate(parts, axis=0).astype(bf16)

    scale_b = DHB ** -0.5

    def b_qkv_dots(i, st, n0, n1):
        r0 = i * (TB // 2)
        if not isinstance(r0, int):
            r0 = pl.multiple_of(r0, TB // 2)
        lhs = []

        def dot(n, tok):
            if not lhs:
                lhs.append(jnp.concatenate([_b16(bxu[j, pl.ds(r0, TB // 2), :]) for j in range(NC)], axis=1))
            y = jnp.dot(lhs[0], _b16(bw_v[n]), preferred_element_type=f32)
            buf_v[st, n, HALO:HALO + TB, :] = y * scale_b if n < 8 else y
            if tok:
                token(y)
        return [functools.partial(dot, n) for n in range(n0, n1)]

    def b_halo(st, first, n0=8, n1=24):
        for n in range(n0, n1):
            if first:
                buf_v[st, n, 0:HALO, :] = jnp.zeros((HALO, 128), f32)
            else:
                buf_v[st, n, 0:HALO, :] = buf_v[(st - 1) % UB, n, TB:TB + HALO, :]

    def b_attn_fillers(st, first, z):
        pend = []

        def group(g):
            r = 8 * g
            q = [buf_v[st, u, pl.ds(z + HALO + r, 8), :] for u in range(8)]
            lg = []
            for w in range(WIN):
                a = HALO + r - DIL * w
                p = q[0] * buf_v[st, 8, a:a + 8, :]
                for u in range(1, 8):
                    p = p + q[u] * buf_v[st, 8 + u, a:a + 8, :]
                p = p + pltpu.roll(p, 32, 1)
                p = p + pltpu.roll(p, 64, 1)
                if first and r - DIL * w < 0:
                    p = jnp.where(sub + (r - DIL * w) >= 0, p, -1e9)
                lg.append(p)
            m = functools.reduce(jnp.maximum, lg)
            e = [jnp.exp(p - m) for p in lg]
            l = functools.reduce(lambda x, y: x + y, e)
            rc = pl.reciprocal(l, approx=True)
            rc = rc * (2.0 - l * rc)
            e = [x * rc for x in e]
            o = []
            for u in range(8):
                acc = None
                for w in range(WIN):
                    a = HALO + r - DIL * w
                    vv = buf_v[st, 16 + u, a:a + 8, :]
                    if first and r - DIL * w < 0:
                        vv = jnp.where(sub + (r - DIL * w) >= 0, vv, buf_v[st, 16 + u, HALO:HALO + 1, :])
                    t = e[w] * vv
                    acc = t if acc is None else acc + t
                o.append(acc)
            pend.append(o)
            if len(pend) == 2:
                for u in range(8):
                    ob_v[st, u, r - 8:r + 8, :] = jnp.concatenate([pend[0][u], pend[1][u]], axis=0).astype(bf16)
                pend.clear()
        return [functools.partial(group, g) for g in range(TB // 8)]

    def b_proj_dots(i, st):
        r0 = i * TB
        if not isinstance(r0, int):
            r0 = pl.multiple_of(r0, TB)
        lhs = []

        def dot(n, tok):
            if not lhs:
                lhs.append(jnp.concatenate([_b16(obu[st, j]) for j in range(NC)], axis=1))
            y = jnp.dot(lhs[0], _b16(bwou[n]), preferred_element_type=f32)
            outb_v[pl.ds(r0, TB), 128 * n:128 * n + 128] = y.astype(bf16)
            if tok:
                token(y)
                buf_v[UB, 0, 0:8, :] = y[0:8]
        return [functools.partial(dot, n) for n in range(NC)]

    def a_relayout(c, g):
        src = stgu.at[pl.ds(pl.multiple_of((STG_AW + c * HW) // 2 + 256 * g, 256), 256), :]
        dst = wa_v.at[pl.ds(pl.multiple_of((c // 2) * (H * PITCH) + (c % 2) * (DM // 4) + 8 * g, 8),
                            (H + 1) * PITCH + 14), :]
        for dp in range(8):
            for o in range(2):
                a = src[32 * dp + 8 * o:32 * dp + 8 * o + 8, :]
                b = src[32 * dp + 16 + 8 * o:32 * dp + 24 + 8 * o, :]
                dst[pl.ds(16 * o * PITCH + dp, 8, stride=2 * PITCH), :] = (a & jnp.uint32(0xFFFF)) | (b << 16)
                dst[pl.ds((16 * o + 1) * PITCH + dp, 8, stride=2 * PITCH), :] = (
                    (a >> 16) | (b & jnp.uint32(0xFFFF0000)))

    def b_iter(it, c):
        z = zero()
        for k in range(UB):
            i = UB * it + k
            b_halo(k, False)
            rel = [] if c is None else [functools.partial(a_relayout, c, g) for g in range(8 * k, 8 * k + 8)]
            _interleave(b_qkv_dots(i, k, 0, 24) + b_proj_dots(i - 2, (k - 2) % UB),
                        b_attn_fillers((k - 1) % UB, False, z) + [lambda: None] * 2, rel)

    def sec(k0, k1, s):
        return [d for k in range(k0, k1) for d in b_qkv_dots(k, k, 8 * s, 8 * s + 8)]

    for n in range(8):
        bw_cp(n).wait()
    for f in perm_fillers(0, 0):
        f()
    for j in range(NC):
        bx_cp(0, j).wait()
    _interleave(sec(0, 2, 0))
    for n in range(8, 16):
        bw_cp(n).wait()
    for it in range(1, NIT):
        for j in range(NC):
            bx_cp(it, j).start()
    _interleave(sec(2, 4, 0), perm_fillers(1, zero()))
    _interleave(sec(0, 2, 1))
    for n in range(16, 24):
        bw_cp(n).wait()
    for c in range(6):
        aw_cp(c).start()
    for n in range(NC):
        awo_cp(n).start()
    for j in range(NC):
        ax_cp(j).start()
    mem_cp.start()
    _interleave(sec(2, 4, 1), perm_fillers(2, zero()))
    for k in range(UB):
        b_halo(k, k == 0, 8, 16)
    _interleave(sec(0, 2, 2))
    b_halo(0, True, 16, 24)
    b_halo(1, False, 16, 24)
    for n in range(NC):
        bwo_cp(n).wait()
    z = zero()
    b_halo(2, False, 16, 24)
    _interleave(sec(2, 3, 2), b_attn_fillers(0, True, z), [functools.partial(prep_bwo, n, z) for n in range(4)])
    b_halo(3, False, 16, 24)
    _interleave(sec(3, 4, 2), b_attn_fillers(1, False, z), [functools.partial(prep_bwo, n, z) for n in range(4, 8)])
    _interleave(b_proj_dots(0, 0) + b_proj_dots(1, 1), b_attn_fillers(2, False, z))
    ob_cp(0, (UB - 2) * TB).start()
    for j in range(NC):
        bx_cp(1, j).wait()
    b_iter(1, None)
    ob_cp((UB - 2) * TB, UB * TB).start()

    def b_body(it, c):
        for j in range(NC):
            bx_cp(it, j).wait()
        aw_wait(it - 2)
        b_iter(it, it - 2)
        ob_cp(pl.multiple_of((UB * it - 2) * TB, TB), UB * TB).start()
        return c
    lax.fori_loop(2, NIT, b_body, 0)
    nb = S // TB
    for f in b_attn_fillers(UB - 1, False, 0):
        f()
    _interleave(b_proj_dots(nb - 2, UB - 2) + b_proj_dots(nb - 1, UB - 1))
    ob_cp(S - 2 * TB, 2 * TB).start()

    for n in range(NC):
        awo_cp(n).wait()
    for j in range(NC):
        ax_cp(j).wait()
    mem_cp.wait()

    scale_a = DH ** -0.5
    rr = lax.broadcasted_iota(i32, (2 * L, 2 * L), 0)
    cc = lax.broadcasted_iota(i32, (2 * L, 2 * L), 1)
    rb_, cb_ = rr >= L, cc >= L
    ri, ci = jnp.where(rb_, rr - L, rr), jnp.where(cb_, cc - L, cc)
    same = rb_ == cb_
    valid = same & ((ri < M) | (ri >= ci))
    fill = jnp.where(same, -1e9, -jnp.inf).astype(f32)

    mem_s[...] = mem_v[...].astype(f32)
    NP = H // 2

    def a_step(lhs, even):
        qkv, pp = {}, {}
        nrow = 32 if even else 48

        def do_qkv(j):
            res = []
            for wi in range(3):
                parts = []
                for hh in (2 * j, 2 * j + 1):
                    w0 = (wi * H + hh) * PITCH
                    y = jnp.dot(lhs, _b16(wa_v[w0:w0 + DM // 2, :]), preferred_element_type=f32)
                    if even:
                        stash[wi * H + hh] = y[32:40]
                        parts += [y[40:48], y[0:32]]
                    else:
                        parts += [y[0:8], stash[wi * H + hh], y[8:32]]
                res.append(jnp.concatenate(parts, axis=0).astype(bf16))
            qkv[j] = res

        def do_qk(j):
            q2, k2, _ = qkv[j]
            s = lax.dot_general(q2, k2, (((1,), (1,)), ((), ())), preferred_element_type=f32) * scale_a
            s = jnp.where(valid, s, fill)
            m = jnp.max(s, axis=1, keepdims=True)
            e = jnp.exp(s - m)
            l = jnp.sum(e, axis=1, keepdims=True)
            rc = pl.reciprocal(l, approx=True)
            rc = rc * (2.0 - l * rc)
            pp[j] = (e * rc).astype(bf16)

        def do_pv(j):
            o2 = jnp.dot(pp.pop(j), qkv.pop(j)[2], preferred_element_type=f32)
            for i, hh in enumerate((2 * j, 2 * j + 1)):
                o = o2[L * i:L * (i + 1)]
                if even:
                    o_s[hh, 0:32, :] = o[0:32].astype(bf16)
                    ostash[hh] = o[32:40]
                else:
                    o_s[hh] = jnp.concatenate([o[0:8], ostash[hh], o[8:40]], axis=0).astype(bf16)

        def wo_part(n, h0, h1):
            lo = jnp.concatenate([_b16(osu[hh, 0:nrow // 2, :]) for hh in range(h0, h1)], axis=1)
            return jnp.dot(lo, _b16(wou[n, h0 * 64:h1 * 64, :]), preferred_element_type=f32)

        for j in range(NP):
            do_qkv(j)
            if j - LQK >= 0:
                do_qk(j - LQK)
            if j - LPV >= 0:
                do_pv(j - LPV)
        ya = []
        nper = NC // (LPV + 1)
        for j in range(NP, NP + LPV):
            for _ in range(nper):
                ya.append(wo_part(len(ya), 0, 2 * KA))
            if j - LQK < NP:
                do_qk(j - LQK)
            do_pv(j - LPV)
        while len(ya) < NC:
            ya.append(wo_part(len(ya), 0, 2 * KA))
        return jnp.concatenate([wo_part(n, 2 * KA, H) + ya[n] for n in range(NC)], axis=1)

    def a_body(t, c):
        r0 = pl.multiple_of(t * 32, 32)
        X = jnp.concatenate([_b16(axu[j, pl.ds(r0, 32), :]) for j in range(NC)], axis=1)
        Xm = X[32:48].astype(f32)
        mixed = jnp.concatenate([Xm[0:8], mem_s[...]], axis=0).astype(bf16)
        ye = a_step(jnp.concatenate([X[0:32], mixed], axis=0), True)
        mixed = jnp.concatenate([ye[0:8], Xm[8:16]], axis=0).astype(bf16)
        yo = a_step(jnp.concatenate([mixed, X[48:64]], axis=0), False)
        mem_s[...] = yo[0:8]
        o0 = pl.multiple_of(t * 64, 64)
        outa_v[pl.ds(o0, 64), :] = jnp.concatenate([ye[8:32], yo[8:48]], axis=0).astype(bf16)
        oa_cp(o0, 64).start()
        return c
    lax.fori_loop(0, S // 64, a_body, 0)

    ob_cp(0, S).wait()
    oa_cp(0, S).wait()


@jax.jit
def _run(A_x, A_mem0, A_Wq, A_Wk, A_Wv, A_Wo, B_x, B_wqkv, B_wo):
    hbm = pl.BlockSpec(memory_space=pl.ANY)
    out = pl.pallas_call(
        _kernel,
        out_shape=jax.ShapeDtypeStruct((S, 2 * DM), bf16),
        in_specs=[hbm] * 9,
        out_specs=hbm,
        scratch_shapes=[
            pltpu.VMEM((NC, S, 128), bf16),
            pltpu.VMEM((M, DM), bf16),
            pltpu.VMEM((STG_ROWS, 128), bf16),
            pltpu.VMEM(((3 * H + 2) * PITCH + 12, 128), u32),
            pltpu.VMEM((NC, H * DH, 128), bf16),
            pltpu.VMEM((NC, S, 128), bf16),
            pltpu.VMEM((24, DM // 2, 128), u32),
            pltpu.VMEM((NC, DM, 128), bf16),
            pltpu.VMEM((2, T32_ROWS, 128), f32),
            pltpu.VMEM((S, DM), bf16),
            pltpu.VMEM((S, DM), bf16),
            pltpu.VMEM((UB + 1, 24, TB + HALO, 128), f32),
            pltpu.VMEM((UB, 8, TB, 128), bf16),
            pltpu.VMEM((M, DM), f32),
            pltpu.VMEM((3 * H, 8, DH), f32),
            pltpu.VMEM((H, 8, DH), f32),
            pltpu.VMEM((H, 48, DH), bf16),
            pltpu.SMEM((1,), i32),
            pltpu.SemaphoreType.DMA((NSEM,)),
        ],
        compiler_params=pltpu.CompilerParams(vmem_limit_bytes=110 * 1024 * 1024),
    )(
        A_x.reshape(S, DM), A_mem0.reshape(M, DM),
        A_Wq.reshape(DM * H, DH), A_Wk.reshape(DM * H, DH), A_Wv.reshape(DM * H, DH),
        A_Wo.reshape(H * DH, DM),
        B_x.reshape(S, DM), B_wqkv, B_wo,
    )
    return out.reshape(1, S, 2 * DM)


def pallas_concat_heads__memory_aug_recurrent_mem_tr__sliding_local_dilated__prompt_kernel(
    A_x, A_mem0, A_Wq, A_Wk, A_Wv, A_Wo, A_seg_len, B_x, B_wqkv, B_wo,
):
    if isinstance(A_seg_len, int):
        assert A_seg_len == SEG
    return _run(A_x, A_mem0, A_Wq, A_Wk, A_Wv, A_Wo, B_x, B_wqkv, B_wo)
```

```python
import contextlib
import functools

import jax
import jax.numpy as jnp
from jax import lax
import jax.experimental.pallas as pl
import jax.experimental.pallas.tpu as pltpu

bf16, f32, u32, i32 = jnp.bfloat16, jnp.float32, jnp.uint32, jnp.int32

S, DM = 2048, 1024
H, DH = 32, 128
M, SEG = 8, 32
L = M + SEG
DHB, WIN, DIL = 32, 8, 2
NC = DM // 128

TB = 64
UB = 4
HALO = 16
NIT = S // (TB * UB)
LQK, LPV, KA = 1, 3, 12

PITCH = DM // 2 + 2
STG_AW, STG_BW, STG_BWO = 0, 3 * DM * H, 3 * DM * H + 24 * DM
STG_TOK = STG_BWO + NC * DM
STG_ROWS = STG_TOK + 16
T32_ROWS = 8 + 128 + 8 * 129

SEM_BW, SEM_BX, SEM_BWO, SEM_AW, SEM_AWO, SEM_AX, SEM_MEM, SEM_OB, SEM_OA, SEM_BQ = 0, 3, 11, 12, 18, 19, 20, 21, 22, 23
NSEM = 24
_SCOPES = False


def _scope(name):
    return jax.named_scope(name) if _SCOPES else contextlib.nullcontext()


def _b16(v):
    return pltpu.bitcast(v, bf16)


def _interleave(dots, *filler_lists):
    pos = [0] * len(filler_lists)
    for n, d in enumerate(dots):
        d(any(pos[k] < len(f) and pos[k] * len(dots) <= n * len(f) for k, f in enumerate(filler_lists)))
        for k, f in enumerate(filler_lists):
            while pos[k] < len(f) and pos[k] * len(dots) <= n * len(f):
                f[pos[k]]()
                pos[k] += 1
    for k, f in enumerate(filler_lists):
        while pos[k] < len(f):
            f[pos[k]]()
            pos[k] += 1


def _kernel(ax_h, mem_h, wq_h, wk_h, wv_h, wo_h, bx_h, bw_h, bwo_h, out_h,
            ax_v, mem_v, stg_v, wa_v, wo_v, bx_v, bw_v, bwo_v, t32_v, outa_v, outb_v,
            buf_v, ob_v, mem_s, stash, ostash, o_s, zero_s, sem):
    def bw_cp(n):
        return pltpu.make_async_copy(bw_h.at[:, pl.ds(128 * n, 128)], stg_v.at[pl.ds(STG_BW + DM * n, DM), :],
                                     sem.at[SEM_BW + n // 8])

    def bq_cp(n, half):
        return pltpu.make_async_copy(bw_h.at[pl.ds(half * (DM // 2), DM // 2), pl.ds(128 * n, 128)],
                                     stg_v.at[pl.ds(STG_BW + DM * n + half * (DM // 2), DM // 2), :],
                                     sem.at[SEM_BQ if half == 0 else SEM_BW])

    def bx_cp(it, j):
        r0 = TB * UB * it
        rows = pl.ds(r0 if isinstance(r0, int) else pl.multiple_of(r0, TB * UB), TB * UB)
        return pltpu.make_async_copy(bx_h.at[rows, pl.ds(128 * j, 128)], bx_v.at[j, rows, :], sem.at[SEM_BX + it])

    def bwo_cp(n):
        return pltpu.make_async_copy(bwo_h.at[:, pl.ds(128 * n, 128)], stg_v.at[pl.ds(STG_BWO + DM * n, DM), :],
                                     sem.at[SEM_BWO])

    HW = DM * H // 2

    def aw_cp(c):
        src = (wq_h, wk_h, wv_h)[c // 2]
        return pltpu.make_async_copy(src.at[pl.ds((c % 2) * HW, HW), :], stg_v.at[pl.ds(STG_AW + c * HW, HW), :],
                                     sem.at[SEM_AW + c])

    def aw_wait(c):
        dst = stg_v.at[pl.ds(pl.multiple_of(STG_AW + c * HW, HW), HW), :]
        pltpu.make_async_copy(dst, dst, sem.at[SEM_AW + c]).wait()

    def col(n):
        return pl.ds(128 * n if isinstance(n, int) else pl.multiple_of(128 * n, 128), 128)

    def awo_cp(n):
        return pltpu.make_async_copy(wo_h.at[:, col(n)], wo_v.at[n], sem.at[SEM_AWO])

    def ax_cp(j):
        return pltpu.make_async_copy(ax_h.at[:, col(j)], ax_v.at[j], sem.at[SEM_AX])

    mem_cp = pltpu.make_async_copy(mem_h, mem_v, sem.at[SEM_MEM])

    def ob_cp(r0, n):
        return pltpu.make_async_copy(outb_v.at[pl.ds(r0, n), :], out_h.at[pl.ds(r0, n), pl.ds(DM, DM)],
                                     sem.at[SEM_OB])

    def oa_cp(r0, n):
        return pltpu.make_async_copy(outa_v.at[pl.ds(r0, n), :], out_h.at[pl.ds(r0, n), pl.ds(0, DM)],
                                     sem.at[SEM_OA])

    for half in range(2):
        for n in range(8):
            bq_cp(n, half).start()
    for j in range(NC):
        bx_cp(0, j).start()
    for n in range(8, 24):
        bw_cp(n).start()
    for n in range(NC):
        bwo_cp(n).start()

    bxu, stgu, obu, bwou = bx_v.bitcast(u32), stg_v.bitcast(u32), ob_v.bitcast(u32), bwo_v.bitcast(u32)
    wou, axu, osu = wo_v.bitcast(u32), ax_v.bitcast(u32), o_s.bitcast(u32)

    lane = lax.broadcasted_iota(i32, (8, 128), 1)
    sub = lax.broadcasted_iota(i32, (8, 128), 0)

    zero_s[0] = 0

    def zero():
        return pl.multiple_of(zero_s[0], 8)

    def token(y):
        stgu[STG_TOK // 2:STG_TOK // 2 + 8, :] = pltpu.bitcast(y[0:8], u32)

    PR = 128

    def perm_select(s, r, z):
        src = stgu.at[pl.ds(z + (STG_BW + 8 * s * DM) // 2, 4 * DM), :]
        bits = [((lane >> b) & 1) == 1 for b in range(3)]
        for rr in range(r, r + PR, 8):
            zs = [src[((-t) % 8) * (DM // 2) + rr:((-t) % 8) * (DM // 2) + rr + 8, :] for t in range(8)]
            for b in range(3):
                zs = [jnp.where(bits[b], zs[(t - (1 << b)) % 8], zs[t]) for t in range(8)]
            for u in range(8):
                bw_v[8 * s + u, rr:rr + 8, :] = zs[u]

    def perm_gather(s, r, u):
        idx = 32 * ((lane >> 3) & 3) + 8 * (lane >> 5) + ((u + lane) & 7)
        for rr in range(r, r + PR, 8):
            bw_v[8 * s + u, rr:rr + 8, :] = jnp.take_along_axis(bw_v[8 * s + u, rr:rr + 8, :], idx, axis=1)

    def perm_chunk(s, r, z):
        perm_select(s, r, z)
        for u in range(8):
            perm_gather(s, r, u)

    def perm_fillers(s, z):
        return [functools.partial(perm_chunk, s, r, z) for r in range(0, DM // 2, PR)]

    def prep_bwo(n, z):
        t = t32_v.at[n % 2]
        src = stgu.at[pl.ds(z + (STG_BWO + n * DM) // 2, DM // 2), :]
        if n < 2:
            t[0:8, :] = jnp.zeros((8, 128), f32)
            t[8 + DM:16 + DM, :] = jnp.zeros((8, 128), f32)
        for r in range(0, DM, 128):
            t[8 + r:8 + r + 128, :] = _b16(src[r // 2:r // 2 + 64, :]).astype(f32)
        for u in range(8):
            for c in range(4):
                for a2 in range(2):
                    parts = []
                    for A in (2 * a2, 2 * a2 + 1):
                        base = 32 * A + 8 * c + u
                        x = t[pl.ds(8 + base, 8, stride=129), :]
                        if u > 0:
                            x = jnp.where(sub + u < 8, x, t[pl.ds(base, 8, stride=129), :])
                        parts.append(x)
                    r = 128 * u + 32 * c + 16 * a2
                    bwo_v[n, r:r + 16, :] = jnp.concatenate(parts, axis=0).astype(bf16)

    scale_b = DHB ** -0.5

    def b_qkv_dots(i, st, n0, n1):
        r0 = i * (TB // 2)
        if not isinstance(r0, int):
            r0 = pl.multiple_of(r0, TB // 2)
        lhs = []

        def dot(n, tok):
            if not lhs:
                lhs.append(jnp.concatenate([_b16(bxu[j, pl.ds(r0, TB // 2), :]) for j in range(NC)], axis=1))
            y = jnp.dot(lhs[0], _b16(bw_v[n]), preferred_element_type=f32)
            buf_v[st, n, HALO:HALO + TB, :] = y * scale_b if n < 8 else y
            if tok:
                token(y)
        return [functools.partial(dot, n) for n in range(n0, n1)]

    def b_halo(st, first, n0=8, n1=24):
        for n in range(n0, n1):
            if first:
                buf_v[st, n, 0:HALO, :] = jnp.zeros((HALO, 128), f32)
            else:
                buf_v[st, n, 0:HALO, :] = buf_v[(st - 1) % UB, n, TB:TB + HALO, :]

    def b_attn_fillers(st, first, z):
        pend = []

        def group(g):
            r = 8 * g
            q = [buf_v[st, u, pl.ds(z + HALO + r, 8), :] for u in range(8)]
            lg = []
            for w in range(WIN):
                a = HALO + r - DIL * w
                p = q[0] * buf_v[st, 8, a:a + 8, :]
                for u in range(1, 8):
                    p = p + q[u] * buf_v[st, 8 + u, a:a + 8, :]
                p = p + pltpu.roll(p, 32, 1)
                p = p + pltpu.roll(p, 64, 1)
                if first and r - DIL * w < 0:
                    p = jnp.where(sub + (r - DIL * w) >= 0, p, -1e9)
                lg.append(p)
            m = functools.reduce(jnp.maximum, lg)
            e = [jnp.exp(p - m) for p in lg]
            l = functools.reduce(lambda x, y: x + y, e)
            rc = pl.reciprocal(l, approx=True)
            rc = rc * (2.0 - l * rc)
            e = [x * rc for x in e]
            o = []
            for u in range(8):
                acc = None
                for w in range(WIN):
                    a = HALO + r - DIL * w
                    vv = buf_v[st, 16 + u, a:a + 8, :]
                    if first and r - DIL * w < 0:
                        vv = jnp.where(sub + (r - DIL * w) >= 0, vv, buf_v[st, 16 + u, HALO:HALO + 1, :])
                    t = e[w] * vv
                    acc = t if acc is None else acc + t
                o.append(acc)
            pend.append(o)
            if len(pend) == 2:
                for u in range(8):
                    ob_v[st, u, r - 8:r + 8, :] = jnp.concatenate([pend[0][u], pend[1][u]], axis=0).astype(bf16)
                pend.clear()
        return [functools.partial(group, g) for g in range(TB // 8)]

    def b_proj_dots(i, st):
        r0 = i * TB
        if not isinstance(r0, int):
            r0 = pl.multiple_of(r0, TB)
        lhs = []

        def dot(n, tok):
            if not lhs:
                lhs.append(jnp.concatenate([_b16(obu[st, j]) for j in range(NC)], axis=1))
            y = jnp.dot(lhs[0], _b16(bwou[n]), preferred_element_type=f32)
            outb_v[pl.ds(r0, TB), 128 * n:128 * n + 128] = y.astype(bf16)
            if tok:
                token(y)
                buf_v[UB, 0, 0:8, :] = y[0:8]
        return [functools.partial(dot, n) for n in range(NC)]

    def a_relayout(c, g):
        src = stgu.at[pl.ds(pl.multiple_of((STG_AW + c * HW) // 2 + 256 * g, 256), 256), :]
        dst = wa_v.at[pl.ds(pl.multiple_of((c // 2) * (H * PITCH) + (c % 2) * (DM // 4) + 8 * g, 8),
                            (H + 1) * PITCH + 14), :]
        for dp in range(8):
            for o in range(2):
                a = src[32 * dp + 8 * o:32 * dp + 8 * o + 8, :]
                b = src[32 * dp + 16 + 8 * o:32 * dp + 24 + 8 * o, :]
                dst[pl.ds(16 * o * PITCH + dp, 8, stride=2 * PITCH), :] = (a & jnp.uint32(0xFFFF)) | (b << 16)
                dst[pl.ds((16 * o + 1) * PITCH + dp, 8, stride=2 * PITCH), :] = (
                    (a >> 16) | (b & jnp.uint32(0xFFFF0000)))

    def b_iter(it, c):
        z = zero()
        for k in range(UB):
            i = UB * it + k
            b_halo(k, False)
            rel = [functools.partial(a_relayout, c, g) for g in range(8 * k, 8 * k + 8)]
            _interleave(b_qkv_dots(i, k, 0, 24) + b_proj_dots(i - 4, k),
                        b_attn_fillers((k - 2) % UB, False, z) + [lambda: None] * 2, rel)

    def sec(k0, k1, s):
        return [d for k in range(k0, k1) for d in b_qkv_dots(k, k, 8 * s, 8 * s + 8)]

    nop = lambda: None
    with _scope("perm_q"):
        pf = perm_fillers(0, 0)
        for half in range(2):
            for n in range(8):
                bq_cp(n, half).wait()
            for f in pf[half * len(pf) // 2:(half + 1) * len(pf) // 2]:
                f()
    with _scope("Qa"):
        for j in range(NC):
            bx_cp(0, j).wait()
        _interleave(sec(0, 2, 0))
    with _scope("QbKa"):
        for n in range(8, 16):
            bw_cp(n).wait()
        for j in range(NC):
            bx_cp(1, j).start()
        aw_cp(0).start()
        awo_cp(NC - 1).start()
        ax_cp(NC - 1).start()
        mem_cp.start()
        _interleave(sec(2, 4, 0), perm_fillers(1, zero()) + [nop])
        _interleave(sec(0, 2, 1))
    with _scope("KbVa"):
        for n in range(16, 24):
            bw_cp(n).wait()
        z = zero()
        _interleave(sec(2, 4, 1), perm_fillers(2, z) + [nop])
        for k in range(UB):
            b_halo(k, k == 0, 8, 16)
        _interleave(sec(0, 1, 2))
        b_halo(0, True, 16, 24)
        b_halo(1, False, 16, 24)
        at0 = b_attn_fillers(0, True, z)
        _interleave(sec(1, 2, 2), at0[0:4] + [nop] * 4)
    with _scope("Vb"):
        for n in range(NC):
            bwo_cp(n).wait()
        b_halo(2, False, 16, 24)
        _interleave(sec(2, 4, 2), at0[4:8] + b_attn_fillers(1, False, z) + [nop] * 4,
                    [functools.partial(prep_bwo, n, z) for n in range(NC)])
        b_halo(3, False, 16, 24)

    def b_body(it, carry):
        with _scope("it"):
            @pl.when(it < NIT - 1)
            def _():
                for j in range(NC):
                    bx_cp(it + 1, j).start()
                aw_wait(it - 1)
            for c in range(1, 6):
                @pl.when(it == c)
                def _():
                    aw_cp(c).start()
            awo_cp(it - 1).start()
            ax_cp(it - 1).start()
            for j in range(NC):
                bx_cp(it, j).wait()
            b_iter(it, jnp.minimum(it - 1, 5))
            ob_cp(pl.multiple_of(UB * TB * (it - 1), UB * TB), UB * TB).start()
        return carry
    lax.fori_loop(1, NIT, b_body, 0)
    nb = S // TB
    with _scope("tailB"):
        z = zero()
        _interleave(b_proj_dots(nb - 4, 0) + b_proj_dots(nb - 3, 1),
                    b_attn_fillers(2, False, z) + b_attn_fillers(3, False, z))
        _interleave(b_proj_dots(nb - 2, 2) + b_proj_dots(nb - 1, 3))
        ob_cp(S - UB * TB, UB * TB).start()

    for n in range(NC):
        awo_cp(n).wait()
    for j in range(NC):
        ax_cp(j).wait()
    mem_cp.wait()

    scale_a = DH ** -0.5
    rr = lax.broadcasted_iota(i32, (2 * L, 2 * L), 0)
    cc = lax.broadcasted_iota(i32, (2 * L, 2 * L), 1)
    rb_, cb_ = rr >= L, cc >= L
    ri, ci = jnp.where(rb_, rr - L, rr), jnp.where(cb_, cc - L, cc)
    same = rb_ == cb_
    valid = same & ((ri < M) | (ri >= ci))
    fill = jnp.where(same, -1e9, -jnp.inf).astype(f32)

    mem_s[...] = mem_v[...].astype(f32)
    NP = H // 2

    def a_step(lhs, even):
        qkv, pp = {}, {}
        nrow = 32 if even else 48

        def do_qkv(j):
            res = []
            for wi in range(3):
                parts = []
                for hh in (2 * j, 2 * j + 1):
                    w0 = (wi * H + hh) * PITCH
                    y = jnp.dot(lhs, _b16(wa_v[w0:w0 + DM // 2, :]), preferred_element_type=f32)
                    if even:
                        stash[wi * H + hh] = y[32:40]
                        parts += [y[40:48], y[0:32]]
                    else:
                        parts += [y[0:8], stash[wi * H + hh], y[8:32]]
                res.append(jnp.concatenate(parts, axis=0).astype(bf16))
            qkv[j] = res

        def do_qk(j):
            q2, k2, _ = qkv[j]
            s = lax.dot_general(q2, k2, (((1,), (1,)), ((), ())), preferred_element_type=f32) * scale_a
            s = jnp.where(valid, s, fill)
            m = jnp.max(s, axis=1, keepdims=True)
            e = jnp.exp(s - m)
            l = jnp.sum(e, axis=1, keepdims=True)
            rc = pl.reciprocal(l, approx=True)
            rc = rc * (2.0 - l * rc)
            pp[j] = (e * rc).astype(bf16)

        def do_pv(j):
            o2 = jnp.dot(pp.pop(j), qkv.pop(j)[2], preferred_element_type=f32)
            for i, hh in enumerate((2 * j, 2 * j + 1)):
                o = o2[L * i:L * (i + 1)]
                if even:
                    o_s[hh, 0:32, :] = o[0:32].astype(bf16)
                    ostash[hh] = o[32:40]
                else:
                    o_s[hh] = jnp.concatenate([o[0:8], ostash[hh], o[8:40]], axis=0).astype(bf16)

        def wo_part(n, h0, h1):
            lo = jnp.concatenate([_b16(osu[hh, 0:nrow // 2, :]) for hh in range(h0, h1)], axis=1)
            return jnp.dot(lo, _b16(wou[n, h0 * 64:h1 * 64, :]), preferred_element_type=f32)

        for j in range(NP):
            do_qkv(j)
            if j - LQK >= 0:
                do_qk(j - LQK)
            if j - LPV >= 0:
                do_pv(j - LPV)
        ya = []
        nper = NC // (LPV + 1)
        for j in range(NP, NP + LPV):
            for _ in range(nper):
                ya.append(wo_part(len(ya), 0, 2 * KA))
            if j - LQK < NP:
                do_qk(j - LQK)
            do_pv(j - LPV)
        while len(ya) < NC:
            ya.append(wo_part(len(ya), 0, 2 * KA))
        return jnp.concatenate([wo_part(n, 2 * KA, H) + ya[n] for n in range(NC)], axis=1)

    def a_body(t, c):
        with _scope("a_it"):
            return a_pair(t, c)

    def a_pair(t, c):
        r0 = pl.multiple_of(t * 32, 32)
        X = jnp.concatenate([_b16(axu[j, pl.ds(r0, 32), :]) for j in range(NC)], axis=1)
        Xm = X[32:48].astype(f32)
        mixed = jnp.concatenate([Xm[0:8], mem_s[...]], axis=0).astype(bf16)
        ye = a_step(jnp.concatenate([X[0:32], mixed], axis=0), True)
        mixed = jnp.concatenate([ye[0:8], Xm[8:16]], axis=0).astype(bf16)
        yo = a_step(jnp.concatenate([mixed, X[48:64]], axis=0), False)
        mem_s[...] = yo[0:8]
        o0 = pl.multiple_of(t * 64, 64)
        outa_v[pl.ds(o0, 64), :] = jnp.concatenate([ye[8:32], yo[8:48]], axis=0).astype(bf16)
        oa_cp(o0, 64).start()
        return c
    lax.fori_loop(0, S // 64, a_body, 0)

    ob_cp(0, S).wait()
    oa_cp(0, S).wait()


@jax.jit
def _run(A_x, A_mem0, A_Wq, A_Wk, A_Wv, A_Wo, B_x, B_wqkv, B_wo):
    hbm = pl.BlockSpec(memory_space=pl.ANY)
    out = pl.pallas_call(
        _kernel,
        out_shape=jax.ShapeDtypeStruct((S, 2 * DM), bf16),
        in_specs=[hbm] * 9,
        out_specs=hbm,
        scratch_shapes=[
            pltpu.VMEM((NC, S, 128), bf16),
            pltpu.VMEM((M, DM), bf16),
            pltpu.VMEM((STG_ROWS, 128), bf16),
            pltpu.VMEM(((3 * H + 2) * PITCH + 12, 128), u32),
            pltpu.VMEM((NC, H * DH, 128), bf16),
            pltpu.VMEM((NC, S, 128), bf16),
            pltpu.VMEM((24, DM // 2, 128), u32),
            pltpu.VMEM((NC, DM, 128), bf16),
            pltpu.VMEM((2, T32_ROWS, 128), f32),
            pltpu.VMEM((S, DM), bf16),
            pltpu.VMEM((S, DM), bf16),
            pltpu.VMEM((UB + 1, 24, TB + HALO, 128), f32),
            pltpu.VMEM((UB, 8, TB, 128), bf16),
            pltpu.VMEM((M, DM), f32),
            pltpu.VMEM((3 * H, 8, DH), f32),
            pltpu.VMEM((H, 8, DH), f32),
            pltpu.VMEM((H, 48, DH), bf16),
            pltpu.SMEM((1,), i32),
            pltpu.SemaphoreType.DMA((NSEM,)),
        ],
        compiler_params=pltpu.CompilerParams(vmem_limit_bytes=110 * 1024 * 1024),
    )(
        A_x.reshape(S, DM), A_mem0.reshape(M, DM),
        A_Wq.reshape(DM * H, DH), A_Wk.reshape(DM * H, DH), A_Wv.reshape(DM * H, DH),
        A_Wo.reshape(H * DH, DM),
        B_x.reshape(S, DM), B_wqkv, B_wo,
    )
    return out.reshape(1, S, 2 * DM)


def pallas_concat_heads__memory_aug_recurrent_mem_tr__sliding_local_dilated__prompt_kernel(
    A_x, A_mem0, A_Wq, A_Wk, A_Wv, A_Wo, A_seg_len, B_x, B_wqkv, B_wo,
):
    if isinstance(A_seg_len, int):
        assert A_seg_len == SEG
    return _run(A_x, A_mem0, A_Wq, A_Wk, A_Wv, A_Wo, B_x, B_wqkv, B_wo)
```

```python
import contextlib
import functools

import jax
import jax.numpy as jnp
from jax import lax
import jax.experimental.pallas as pl
import jax.experimental.pallas.tpu as pltpu

bf16, f32, u32, i32 = jnp.bfloat16, jnp.float32, jnp.uint32, jnp.int32

S, DM = 2048, 1024
H, DH = 32, 128
M, SEG = 8, 32
L = M + SEG
DHB, WIN, DIL = 32, 8, 2
NC = DM // 128

TB = 64
UB = 4
HALO = 16
NIT = S // (TB * UB)
LQK, LPV, KA = 1, 3, 12

PITCH = DM // 2 + 2
WA_DUM = (3 * H + 2) * PITCH + 12
OPITCH = 68
HW = DM * H // 2
STG_AW, STG_BW, STG_BWO = 0, 6 * HW, 6 * HW + 24 * DM
STG_TOK = STG_BWO + NC * DM
STG_ROWS = STG_TOK + 16
NG = TB // 8
X_PART = UB * 24 * (TB + HALO)
X_PROB = X_PART + 2 * NG * WIN * 8
X_OUT = X_PROB + 2 * NG * WIN * 8
X_TMP = X_OUT + 2 * NG * 8 * 8
X_FEN = X_TMP + 8 * 256
X_ROWS = X_FEN + 8

SEM_BW, SEM_BX, SEM_BWO, SEM_AW, SEM_AWO, SEM_AX, SEM_MEM, SEM_OB, SEM_OA = 0, 6, 9, 10, 16, 17, 18, 19, 20
NSEM = 21
_SCOPES = False


def _scope(name):
    return jax.named_scope(name) if _SCOPES else contextlib.nullcontext()


def _b16(v):
    return pltpu.bitcast(v, bf16)


def _qkv_row(st, n):
    return (st * 24 + n) * (TB + HALO)


def _kernel(ax_h, mem_h, wq_h, wk_h, wv_h, wo_h, bx_h, bw_h, bwo_h, out_h,
            ax_v, mem_v, stg_v, wa_v, wo_v, bx_v, bw_v, bwo_v, outa_v, outb_v,
            x_v, ob_v, mem_s, stash, ostash, o_s, zero_s, sem):
    P = functools.partial

    def bw_cps(s, half):
        return [pltpu.make_async_copy(bw_h.at[pl.ds(half * (DM // 2), DM // 2), pl.ds(128 * n, 128)],
                                      stg_v.at[pl.ds(STG_BW + DM * n + half * (DM // 2), DM // 2), :],
                                      sem.at[SEM_BW + 2 * s + half]) for n in range(8 * s, 8 * s + 8)]

    def bx_cps(part):
        rows = (pl.ds(0, TB * UB), pl.ds(TB * UB, TB * UB), pl.ds(2 * TB * UB, S - 2 * TB * UB))[part]
        return [pltpu.make_async_copy(bx_h.at[rows, pl.ds(128 * j, 128)], bx_v.at[j, rows, :],
                                      sem.at[SEM_BX + part]) for j in range(NC)]

    def bwo_cps():
        return [pltpu.make_async_copy(bwo_h.at[:, pl.ds(128 * n, 128)], stg_v.at[pl.ds(STG_BWO + DM * n, DM), :],
                                      sem.at[SEM_BWO]) for n in range(NC)]

    def aw_cp(c):
        src = (wq_h, wk_h, wv_h)[c // 2]
        return pltpu.make_async_copy(src.at[pl.ds((c % 2) * HW, HW), :], stg_v.at[pl.ds(STG_AW + c * HW, HW), :],
                                     sem.at[SEM_AW + c])

    def awo_cp(n):
        return pltpu.make_async_copy(wo_h.at[:, pl.ds(128 * n, 128)], wo_v.at[n], sem.at[SEM_AWO])

    def ax_cp(j):
        return pltpu.make_async_copy(ax_h.at[:, pl.ds(128 * j, 128)], ax_v.at[j], sem.at[SEM_AX])

    mem_cp = pltpu.make_async_copy(mem_h, mem_v, sem.at[SEM_MEM])

    def ob_cp(r0, n):
        return pltpu.make_async_copy(outb_v.at[pl.ds(r0, n), :], out_h.at[pl.ds(r0, n), pl.ds(DM, DM)],
                                     sem.at[SEM_OB])

    def oa_cp(r0, n):
        return pltpu.make_async_copy(outa_v.at[pl.ds(r0, n), :], out_h.at[pl.ds(r0, n), pl.ds(0, DM)],
                                     sem.at[SEM_OA])

    def start(cps):
        for c in cps:
            c.start()

    def wait(cps):
        for c in cps:
            c.wait()

    start(bw_cps(0, 0) + bw_cps(0, 1) + bx_cps(0) + bw_cps(1, 0) + bw_cps(1, 1))

    bxu, stgu, obu = bx_v.bitcast(u32), stg_v.bitcast(u32), ob_v.bitcast(u32)
    wou, axu, osu = wo_v.bitcast(u32), ax_v.bitcast(u32), o_s.bitcast(u32)

    lane = lax.broadcasted_iota(i32, (8, 128), 1)
    sub = lax.broadcasted_iota(i32, (8, 128), 0)

    def xv(r):
        return x_v[r:r + 8, :]

    zero_s[0] = 0
    wa_v[WA_DUM:WA_DUM + 8, :] = jnp.zeros((8, 128), u32)

    def run(dots, fill, relayout=False):
        z = pl.multiple_of(zero_s[0], 8)
        for n, d in enumerate(dots):
            y = d()
            if fill.get(n) or fill.get(n - 1):
                if relayout:
                    x_v[X_FEN:X_FEN + 8, :] = pltpu.bitcast(wa_v[WA_DUM:WA_DUM + 8, :], f32)
                x_v[pl.ds(z + X_FEN, 8), :] = y
                stgu[pl.ds(z + STG_TOK // 2, 8), :] = pltpu.bitcast(xv(X_FEN), u32)
            for f in fill.get(n, []):
                f()
        for n in sorted(fill):
            if n >= len(dots):
                for f in fill[n]:
                    f()

    def put(fill, n, f):
        fill.setdefault(n, []).append(f)

    def perm_select(s, half, r0, r1):
        bits = [((lane >> (b + 1)) & 1) == 1 for b in range(3)]
        for r in range(r0, r1, 8):
            src = (STG_BW + 8 * s * DM) // 2 + half * 256 + r
            zs = [stgu[src + ((-t) % 8) * (DM // 2):src + ((-t) % 8) * (DM // 2) + 8, :] for t in range(8)]
            for b in range(3):
                zs = [jnp.where(bits[b], zs[(t - (1 << b)) % 8], zs[t]) for t in range(8)]
            for u in range(8):
                x_v[X_TMP + 256 * u + r:X_TMP + 256 * u + r + 8, :] = pltpu.bitcast(zs[u], f32)

    def perm_gather(s, half, u, r0, r1):
        idx = 32 * ((lane >> 3) & 3) + 16 * (lane >> 6) + 2 * ((u + lane) & 7) + ((lane >> 5) & 1)
        for r in range(r0, r1, 8):
            bw_v[8 * s + u, half * 256 + r:half * 256 + r + 8, :] = jnp.take_along_axis(
                pltpu.bitcast(xv(X_TMP + 256 * u + r), u32), idx, axis=1)

    def perm_fill(fill, s, half, n0, ns, ng):
        for k in range(4):
            put(fill, n0 + k * ns // 4, P(perm_select, s, half, 64 * k, 64 * k + 64))
        g0 = n0 + ns // 4 + 1
        for k in range(16):
            rh, u = k // 8, k % 8
            e = max(g0 + k * ng // 16, n0 + (2 * rh + 1) * ns // 4 + 1)
            put(fill, e, P(perm_gather, s, half, u, 128 * rh, 128 * rh + 128))

    def prep_bwo(n):
        for v in range(0, 8, 2):
            for k in range(8):
                r = (STG_BWO + n * DM) // 2 + 64 * v + 8 * k
                a = stgu[r:r + 8, :]
                b = stgu[r + 64:r + 72, :]
                a = pltpu.roll(a, (8 - v) % 8, 0) if v else a
                b = pltpu.roll(b, 7 - v, 0)
                d = 32 * (k % 2) + 4 * (k // 2) + v // 2
                bwo_v[n, pl.ds(d, 8, stride=OPITCH), :] = (a & jnp.uint32(0xFFFF)) | (b << 16)
                bwo_v[n, pl.ds(d + 16, 8, stride=OPITCH), :] = (a >> 16) | (b & jnp.uint32(0xFFFF0000))

    scale_b = DHB ** -0.5

    def b_qkv_dots(i, st, n0, n1, hist=True):
        r0 = i * (TB // 2)
        if not isinstance(r0, int):
            r0 = pl.multiple_of(r0, TB // 2)

        def dot(n):
            lhs = jnp.concatenate([_b16(bxu[j, pl.ds(r0, TB // 2), :]) for j in range(NC)], axis=1)
            y = jnp.dot(lhs, _b16(bw_v[n]), preferred_element_type=f32)
            r = _qkv_row(st, n)
            x_v[r + HALO:r + HALO + TB, :] = y * scale_b if n < 8 else y
            if n >= 8 and hist:
                r = _qkv_row((st + 1) % UB, n)
                x_v[r:r + HALO, :] = y[TB - HALO:TB]
            return y[TB - 8:TB]
        return [P(dot, n) for n in range(n0, n1)]

    def b_proj_dots(i, st):
        r0 = i * TB
        if not isinstance(r0, int):
            r0 = pl.multiple_of(r0, TB)

        def dot(n):
            lhs = jnp.concatenate([_b16(obu[st, j]) for j in range(NC)], axis=1)
            w = jnp.concatenate([_b16(bwo_v[n, OPITCH * u:OPITCH * u + 64, :]) for u in range(8)], axis=0)
            y = jnp.dot(lhs, w, preferred_element_type=f32)
            outb_v[pl.ds(r0, TB), 128 * n:128 * n + 128] = y.astype(bf16)
            return y[TB - 8:TB]
        return [P(dot, n) for n in range(NC)]

    def at_qk(st, g):
        q = [xv(_qkv_row(st, u) + HALO + 8 * g) for u in range(8)]
        for w in range(WIN):
            a = HALO + 8 * g - DIL * w
            p = q[0] * xv(_qkv_row(st, 8) + a)
            for u in range(1, 8):
                p = p + q[u] * xv(_qkv_row(st, 8 + u) + a)
            r = X_PART + (((st % 2) * NG + g) * WIN + w) * 8
            x_v[r:r + 8, :] = p

    def at_softmax(st, g, first, pend):
        lg = []
        for w in range(WIN):
            p = xv(X_PART + (((st % 2) * NG + g) * WIN + w) * 8)
            p = p + pltpu.roll(p, 32, 1)
            p = p + pltpu.roll(p, 64, 1)
            if first and 8 * g - DIL * w < 0:
                p = jnp.where(sub + (8 * g - DIL * w) >= 0, p, -1e9)
            lg.append(p)
        m = functools.reduce(jnp.maximum, lg)
        e = [jnp.exp(p - m) for p in lg]
        l = functools.reduce(lambda x, y: x + y, e)
        rc = pl.reciprocal(l, approx=True)
        rc = rc * (2.0 - l * rc)
        pend[st, g] = [x * rc for x in e]

    def at_store(st, g, pend):
        for w, p in enumerate(pend.pop((st, g))):
            r = X_PROB + (((st % 2) * NG + g) * WIN + w) * 8
            x_v[r:r + 8, :] = p

    def at_pv(st, g, first):
        e = [xv(X_PROB + (((st % 2) * NG + g) * WIN + w) * 8) for w in range(WIN)]
        for u in range(8):
            acc = None
            for w in range(WIN):
                r = _qkv_row(st, 16 + u) + HALO
                vv = xv(r + 8 * g - DIL * w)
                if first and 8 * g - DIL * w < 0:
                    vv = jnp.where(sub + (8 * g - DIL * w) >= 0, vv, x_v[r:r + 1, :])
                t = e[w] * vv
                acc = t if acc is None else acc + t
            r = X_OUT + (((st % 2) * NG + g) * 8 + u) * 8
            x_v[r:r + 8, :] = acc

    def at_pack(st, g):
        for u in range(8):
            o = [xv(X_OUT + (((st % 2) * NG + k) * 8 + u) * 8) for k in (g - 1, g)]
            ob_v[st, u, 8 * g - 8:8 * g + 8, :] = jnp.concatenate(o, axis=0).astype(bf16)

    pend = {}

    def attn_fill(fill, st, first, e_qk, e_pv, head=True, tail=True):
        for g in range(NG):
            if head:
                put(fill, e_qk(g), P(at_qk, st, g))
                put(fill, e_qk(g) + 1, P(at_softmax, st, g, first, pend))
                put(fill, e_qk(g) + 3, P(at_store, st, g, pend))
            if (head and g < NG - 1) or (tail and g == NG - 1):
                put(fill, e_pv(g), P(at_pv, st, g, first))
                if g % 2 == 1:
                    put(fill, e_pv(g) + 1, P(at_pack, st, g))

    def a_relayout(src0, dst0, g, o):
        src = stgu.at[pl.ds(pl.multiple_of(src0 + 256 * g, 256), 256), :]
        dst = wa_v.at[pl.ds(pl.multiple_of(dst0 + 8 * g, 8), (H + 1) * PITCH + 14), :]
        for dp in range(8):
            a = src[32 * dp + 8 * o:32 * dp + 8 * o + 8, :]
            b = src[32 * dp + 16 + 8 * o:32 * dp + 24 + 8 * o, :]
            dst[pl.ds(16 * o * PITCH + dp, 8, stride=2 * PITCH), :] = (a & jnp.uint32(0xFFFF)) | (b << 16)
            dst[pl.ds((16 * o + 1) * PITCH + dp, 8, stride=2 * PITCH), :] = (
                (a >> 16) | (b & jnp.uint32(0xFFFF0000)))

    def sec(k0, k1, s):
        return [d for k in range(k0, k1) for d in b_qkv_dots(k, k, 8 * s, 8 * s + 8)]

    with _scope("perm_q"):
        for n in range(8, 24):
            x_v[_qkv_row(0, n):_qkv_row(0, n) + HALO, :] = jnp.zeros((HALO, 128), f32)
        for half in range(2):
            wait(bw_cps(0, half))
            if half == 0:
                start(bw_cps(2, 0) + bw_cps(2, 1) + bwo_cps() + bx_cps(1))
            perm_select(0, half, 0, 256)
            for u in range(8):
                perm_gather(0, half, u, 0, 256)
    with _scope("Q01"):
        wait(bx_cps(0))
        run(sec(0, 2, 0), {})
    with _scope("Q2"):
        wait(bw_cps(1, 0))
        fill = {}
        perm_fill(fill, 1, 0, 0, 3, 5)
        run(sec(2, 3, 0), fill)
    with _scope("Q3K0"):
        wait(bw_cps(1, 1))
        start(bx_cps(2) + [aw_cp(0), mem_cp])
        fill = {}
        perm_fill(fill, 1, 1, 0, 3, 5)
        run(sec(3, 4, 0) + sec(0, 1, 1), fill)
    with _scope("K12"):
        wait(bw_cps(2, 0))
        fill = {}
        perm_fill(fill, 2, 0, 0, 6, 10)
        run(sec(1, 3, 1), fill)
    with _scope("K3V012"):
        wait(bw_cps(2, 1))
        fill = {}
        perm_fill(fill, 2, 1, 0, 3, 5)
        attn_fill(fill, 0, True, lambda g: 7 + g, lambda g: 15 + g)
        attn_fill(fill, 1, False, lambda g: 15 + g, lambda g: 23 + g, tail=False)
        run(b_qkv_dots(3, 3, 8, 16, hist=False) + sec(0, 3, 2), fill)
    with _scope("V3"):
        wait(bwo_cps())
        fill = {}
        for n in range(NC):
            put(fill, min(n, 6), P(prep_bwo, n))
        run(sec(3, 4, 2), fill)
        for n in range(8, 16):
            r0, r3 = _qkv_row(0, n), _qkv_row(3, n)
            x_v[r0:r0 + HALO, :] = x_v[r3 + TB:r3 + TB + HALO, :]

    def b_body(it, carry):
        with _scope("it"):
            for c in range(1, NIT):
                @pl.when(it == c)
                def _():
                    if c < 6:
                        aw_cp(c).start()
                    start([awo_cp(c - 1), ax_cp(c - 1)] + ([awo_cp(NC - 1), ax_cp(NC - 1)] if c == 6 else []))
                    if c <= 2:
                        wait(bx_cps(c))
                    if c >= 2:
                        aw_cp(c - 2).wait()
            c = jnp.maximum(it - 2, 0)
            src0 = jnp.where(it == 1, STG_BW // 2, STG_AW // 2 + c * (HW // 2))
            dst0 = (c // 2) * (H * PITCH) + (c % 2) * (DM // 4)
            dots, fill = [], {}
            for k in range(UB):
                i, e0 = UB * it + k, 32 * k
                dots += b_qkv_dots(i, k, 0, 24) + b_proj_dots(i - 4, k)
                attn_fill(fill, (k - 3) % UB, False, None, lambda g: e0 + 2, head=False)
                attn_fill(fill, (k - 2) % UB, False, lambda g: e0 + 4 * g - (1 if 4 * g + e0 == 124 else 0),
                          lambda g: e0 + 4 * g + 6, tail=False)
                for g in range(8):
                    for o in range(2):
                        put(fill, min(e0 + 4 * g + 1 + 2 * o, 126), P(a_relayout, src0, dst0, 8 * k + g, o))
            run(dots, fill, relayout=True)
            ob_cp(pl.multiple_of(UB * TB * (it - 1), UB * TB), UB * TB).start()
        return carry
    lax.fori_loop(1, NIT, b_body, 0)
    nb = S // TB
    with _scope("tailB"):
        fill = {}
        attn_fill(fill, 1, False, None, lambda g: 0, head=False)
        attn_fill(fill, 2, False, lambda g: g, lambda g: 4 + g)
        attn_fill(fill, 3, False, lambda g: 8 + g, lambda g: 12 + g)
        run([d for k in range(UB) for d in b_proj_dots(nb - 4 + k, k)], fill)
        ob_cp(S - UB * TB, UB * TB).start()

    wait([awo_cp(n) for n in range(NC)] + [ax_cp(j) for j in range(NC)] + [mem_cp])

    scale_a = DH ** -0.5
    rr = lax.broadcasted_iota(i32, (2 * L, 2 * L), 0)
    cc = lax.broadcasted_iota(i32, (2 * L, 2 * L), 1)
    rb_, cb_ = rr >= L, cc >= L
    ri, ci = jnp.where(rb_, rr - L, rr), jnp.where(cb_, cc - L, cc)
    same = rb_ == cb_
    valid = same & ((ri < M) | (ri >= ci))
    fill = jnp.where(same, -1e9, -jnp.inf).astype(f32)

    mem_s[...] = mem_v[...].astype(f32)
    NP = H // 2

    def a_step(lhs, even):
        qkv, pp = {}, {}
        nrow = 32 if even else 48

        def do_qkv(j):
            res = []
            for wi in range(3):
                parts = []
                for hh in (2 * j, 2 * j + 1):
                    w0 = (wi * H + hh) * PITCH
                    y = jnp.dot(lhs, _b16(wa_v[w0:w0 + DM // 2, :]), preferred_element_type=f32)
                    if even:
                        stash[wi * H + hh] = y[32:40]
                        parts += [y[40:48], y[0:32]]
                    else:
                        parts += [y[0:8], stash[wi * H + hh], y[8:32]]
                res.append(jnp.concatenate(parts, axis=0).astype(bf16))
            qkv[j] = res

        def do_qk(j):
            q2, k2, _ = qkv[j]
            s = lax.dot_general(q2, k2, (((1,), (1,)), ((), ())), preferred_element_type=f32) * scale_a
            s = jnp.where(valid, s, fill)
            m = jnp.max(s, axis=1, keepdims=True)
            e = jnp.exp(s - m)
            l = jnp.sum(e, axis=1, keepdims=True)
            rc = pl.reciprocal(l, approx=True)
            rc = rc * (2.0 - l * rc)
            pp[j] = (e * rc).astype(bf16)

        def do_pv(j):
            o2 = jnp.dot(pp.pop(j), qkv.pop(j)[2], preferred_element_type=f32)
            for i, hh in enumerate((2 * j, 2 * j + 1)):
                o = o2[L * i:L * (i + 1)]
                if even:
                    o_s[hh, 0:32, :] = o[0:32].astype(bf16)
                    ostash[hh] = o[32:40]
                else:
                    o_s[hh] = jnp.concatenate([o[0:8], ostash[hh], o[8:40]], axis=0).astype(bf16)

        def wo_part(n, h0, h1):
            lo = jnp.concatenate([_b16(osu[hh, 0:nrow // 2, :]) for hh in range(h0, h1)], axis=1)
            return jnp.dot(lo, _b16(wou[n, h0 * 64:h1 * 64, :]), preferred_element_type=f32)

        for j in range(NP):
            do_qkv(j)
            if j - LQK >= 0:
                do_qk(j - LQK)
            if j - LPV >= 0:
                do_pv(j - LPV)
        ya = []
        nper = NC // (LPV + 1)
        for j in range(NP, NP + LPV):
            for _ in range(nper):
                ya.append(wo_part(len(ya), 0, 2 * KA))
            if j - LQK < NP:
                do_qk(j - LQK)
            do_pv(j - LPV)
        while len(ya) < NC:
            ya.append(wo_part(len(ya), 0, 2 * KA))
        return jnp.concatenate([wo_part(n, 2 * KA, H) + ya[n] for n in range(NC)], axis=1)

    def a_body(t, c):
        with _scope("a_it"):
            return a_pair(t, c)

    def a_pair(t, c):
        r0 = pl.multiple_of(t * 32, 32)
        X = jnp.concatenate([_b16(axu[j, pl.ds(r0, 32), :]) for j in range(NC)], axis=1)
        Xm = X[32:48].astype(f32)
        mixed = jnp.concatenate([Xm[0:8], mem_s[...]], axis=0).astype(bf16)
        ye = a_step(jnp.concatenate([X[0:32], mixed], axis=0), True)
        mixed = jnp.concatenate([ye[0:8], Xm[8:16]], axis=0).astype(bf16)
        yo = a_step(jnp.concatenate([mixed, X[48:64]], axis=0), False)
        mem_s[...] = yo[0:8]
        o0 = pl.multiple_of(t * 64, 64)
        outa_v[pl.ds(o0, 64), :] = jnp.concatenate([ye[8:32], yo[8:48]], axis=0).astype(bf16)
        oa_cp(o0, 64).start()
        return c
    lax.fori_loop(0, S // 64, a_body, 0)

    ob_cp(0, S).wait()
    oa_cp(0, S).wait()


@jax.jit
def _run(A_x, A_mem0, A_Wq, A_Wk, A_Wv, A_Wo, B_x, B_wqkv, B_wo):
    hbm = pl.BlockSpec(memory_space=pl.ANY)
    out = pl.pallas_call(
        _kernel,
        out_shape=jax.ShapeDtypeStruct((S, 2 * DM), bf16),
        in_specs=[hbm] * 9,
        out_specs=hbm,
        scratch_shapes=[
            pltpu.VMEM((NC, S, 128), bf16),
            pltpu.VMEM((M, DM), bf16),
            pltpu.VMEM((STG_ROWS, 128), bf16),
            pltpu.VMEM((WA_DUM + 8, 128), u32),
            pltpu.VMEM((NC, H * DH, 128), bf16),
            pltpu.VMEM((NC, S, 128), bf16),
            pltpu.VMEM((24, DM // 2, 128), u32),
            pltpu.VMEM((NC, 9 * OPITCH + 4, 128), u32),
            pltpu.VMEM((S, DM), bf16),
            pltpu.VMEM((S, DM), bf16),
            pltpu.VMEM((X_ROWS, 128), f32),
            pltpu.VMEM((UB, 8, TB, 128), bf16),
            pltpu.VMEM((M, DM), f32),
            pltpu.VMEM((3 * H, 8, DH), f32),
            pltpu.VMEM((H, 8, DH), f32),
            pltpu.VMEM((H, 48, DH), bf16),
            pltpu.SMEM((1,), i32),
            pltpu.SemaphoreType.DMA((NSEM,)),
        ],
        compiler_params=pltpu.CompilerParams(vmem_limit_bytes=110 * 1024 * 1024),
    )(
        A_x.reshape(S, DM), A_mem0.reshape(M, DM),
        A_Wq.reshape(DM * H, DH), A_Wk.reshape(DM * H, DH), A_Wv.reshape(DM * H, DH),
        A_Wo.reshape(H * DH, DM),
        B_x.reshape(S, DM), B_wqkv, B_wo,
    )
    return out.reshape(1, S, 2 * DM)


def pallas_concat_heads__memory_aug_recurrent_mem_tr__sliding_local_dilated__prompt_kernel(
    A_x, A_mem0, A_Wq, A_Wk, A_Wv, A_Wo, A_seg_len, B_x, B_wqkv, B_wo,
):
    if isinstance(A_seg_len, int):
        assert A_seg_len == SEG
    return _run(A_x, A_mem0, A_Wq, A_Wk, A_Wv, A_Wo, B_x, B_wqkv, B_wo)
```

```python
import contextlib
import functools

import jax
import jax.numpy as jnp
from jax import lax
import jax.experimental.pallas as pl
import jax.experimental.pallas.tpu as pltpu

bf16, f32, u32, i32 = jnp.bfloat16, jnp.float32, jnp.uint32, jnp.int32

S, DM = 2048, 1024
H, DH = 32, 128
M, SEG = 8, 32
L = M + SEG
DHB, WIN, DIL = 32, 8, 2
NC = DM // 128

TB = 64
UB = 4
HALO = 16
NIT = S // (TB * UB)
LQK, LPV, KA = 1, 3, 12

PITCH = DM // 2 + 2
WA_DUM = (3 * H + 2) * PITCH + 12
OPITCH = 68
HW = DM * H // 2
STG_AW, STG_BW, STG_BWO = 0, 6 * HW, 6 * HW + 24 * DM
STG_TOK = STG_BWO + NC * DM
STG_ROWS = STG_TOK + 16
NG = TB // 8
X_PART = UB * 24
X_PROB = X_PART + 2 * NG
X_OUT = X_PROB + 2 * NG
X_TMP = X_OUT + 2 * NG
X_FEN = X_TMP + 32
X_SLABS = X_FEN + 1

SEM_BW, SEM_BX, SEM_BWO, SEM_AW, SEM_AWO, SEM_AX, SEM_MEM, SEM_OB, SEM_OA = 0, 6, 9, 10, 16, 17, 18, 19, 20
NSEM = 21
_SCOPES = False


def _scope(name):
    return jax.named_scope(name) if _SCOPES else contextlib.nullcontext()


def _b16(v):
    return pltpu.bitcast(v, bf16)


def _lhs(blocks):
    return _b16(jnp.concatenate(blocks, axis=1))


def _kernel(ax_h, mem_h, wq_h, wk_h, wv_h, wo_h, bx_h, bw_h, bwo_h, out_h,
            ax_v, mem_v, stg_v, wa_v, wo_v, bx_v, bw_v, bwo_v, outa_v, outb_v,
            x_v, ob_v, mem_s, stash, ostash, o_s, zero_s, sem):
    P = functools.partial

    def bw_cps(s, half):
        return [pltpu.make_async_copy(bw_h.at[pl.ds(half * (DM // 2), DM // 2), pl.ds(128 * n, 128)],
                                      stg_v.at[pl.ds(STG_BW + DM * n + half * (DM // 2), DM // 2), :],
                                      sem.at[SEM_BW + 2 * s + half]) for n in range(8 * s, 8 * s + 8)]

    def bx_cps(part):
        rows = (pl.ds(0, TB * UB), pl.ds(TB * UB, TB * UB), pl.ds(2 * TB * UB, S - 2 * TB * UB))[part]
        return [pltpu.make_async_copy(bx_h.at[rows, pl.ds(128 * j, 128)], bx_v.at[j, rows, :],
                                      sem.at[SEM_BX + part]) for j in range(NC)]

    def bwo_cps():
        return [pltpu.make_async_copy(bwo_h.at[:, pl.ds(128 * n, 128)], stg_v.at[pl.ds(STG_BWO + DM * n, DM), :],
                                      sem.at[SEM_BWO]) for n in range(NC)]

    def aw_cp(c):
        src = (wq_h, wk_h, wv_h)[c // 2]
        return pltpu.make_async_copy(src.at[pl.ds((c % 2) * HW, HW), :], stg_v.at[pl.ds(STG_AW + c * HW, HW), :],
                                     sem.at[SEM_AW + c])

    def awo_cp(n):
        return pltpu.make_async_copy(wo_h.at[:, pl.ds(128 * n, 128)], wo_v.at[n], sem.at[SEM_AWO])

    def ax_cp(j):
        return pltpu.make_async_copy(ax_h.at[:, pl.ds(128 * j, 128)], ax_v.at[j], sem.at[SEM_AX])

    mem_cp = pltpu.make_async_copy(mem_h, mem_v, sem.at[SEM_MEM])

    def ob_cp(r0, n):
        return pltpu.make_async_copy(outb_v.at[pl.ds(r0, n), :], out_h.at[pl.ds(r0, n), pl.ds(DM, DM)],
                                     sem.at[SEM_OB])

    def oa_cp(r0, n):
        return pltpu.make_async_copy(outa_v.at[pl.ds(r0, n), :], out_h.at[pl.ds(r0, n), pl.ds(0, DM)],
                                     sem.at[SEM_OA])

    def start(cps):
        for c in cps:
            c.start()

    def wait(cps):
        for c in cps:
            c.wait()

    start(bw_cps(0, 0) + bw_cps(0, 1) + bx_cps(0) + bw_cps(1, 0) + bw_cps(1, 1))

    bxu, stgu, obu = bx_v.bitcast(u32), stg_v.bitcast(u32), ob_v.bitcast(u32)
    wou, axu, osu = wo_v.bitcast(u32), ax_v.bitcast(u32), o_s.bitcast(u32)

    zero_s[0] = 0
    wa_v[WA_DUM:WA_DUM + 8, :] = jnp.zeros((8, 128), u32)

    def run(dots, fill, relayout=False):
        z = pl.multiple_of(zero_s[0], 8)
        for n, d in enumerate(dots):
            y = d()
            if fill.get(n) or fill.get(n - 1):
                if relayout:
                    x_v[X_FEN, 0:8, :] = pltpu.bitcast(wa_v[WA_DUM:WA_DUM + 8, :], f32)
                x_v[z + X_FEN, 0:8, :] = y
                stgu[pl.ds(z + STG_TOK // 2, 8), :] = pltpu.bitcast(x_v[X_FEN, 0:8, :], u32)
            for f in fill.get(n, []):
                f()
        for n in sorted(fill):
            if n >= len(dots):
                for f in fill[n]:
                    f()

    def put(fill, n, f):
        fill.setdefault(n, []).append(f)

    lane64 = lax.broadcasted_iota(i32, (64, 128), 1)

    def perm_select(s, half, k):
        src = (STG_BW + 8 * s * DM) // 2 + half * 256 + 64 * k
        zs = [stgu[src + ((-t) % 8) * (DM // 2):src + ((-t) % 8) * (DM // 2) + 64, :] for t in range(8)]
        for b in range(3):
            bit = ((lane64 >> (b + 1)) & 1) == 1
            zs = [lax.select(bit, zs[(t - (1 << b)) % 8], zs[t]) for t in range(8)]
        for u in range(8):
            x_v[X_TMP + 4 * u + k, 0:64, :] = pltpu.bitcast(zs[u], f32)

    def perm_gather(s, half, u, k0, k1):
        n = 64 * (k1 - k0)
        lane = lax.broadcasted_iota(i32, (n, 128), 1)
        idx = 32 * ((lane >> 3) & 3) + 16 * (lane >> 6) + 2 * ((u + lane) & 7) + ((lane >> 5) & 1)
        t = pltpu.bitcast(x_v[X_TMP + 4 * u + k0:X_TMP + 4 * u + k1, 0:64, :].reshape(n, 128), u32)
        bw_v[8 * s + u, half * 256 + 64 * k0:half * 256 + 64 * k1, :] = jnp.take_along_axis(t, idx, axis=1)

    def perm_fill(fill, s, half, n0, ns, ng):
        for k in range(4):
            put(fill, n0 + k * ns // 4, P(perm_select, s, half, k))
        g0 = n0 + ns // 4 + 1
        for k in range(16):
            rh, u = k // 8, k % 8
            e = max(g0 + k * ng // 16, n0 + (2 * rh + 1) * ns // 4 + 1)
            put(fill, e, P(perm_gather, s, half, u, 2 * rh, 2 * rh + 2))

    def pack_pairs(a, b):
        return (a & jnp.uint32(0xFFFF)) | (b << 16), (a >> 16) | (b & jnp.uint32(0xFFFF0000))

    def prep_bwo(n):
        for v in range(0, 8, 2):
            r = (STG_BWO + n * DM) // 2 + 64 * v
            a = stgu[r:r + 64, :].reshape(8, 8, 128)
            b = stgu[r + 64:r + 128, :].reshape(8, 8, 128)
            a = pltpu.roll(a, 8 - v, 1) if v else a
            lo, hi = pack_pairs(a, pltpu.roll(b, 7 - v, 1))
            for k in range(8):
                d = 32 * (k % 2) + 4 * (k // 2) + v // 2
                bwo_v[n, pl.ds(d, 8, stride=OPITCH), :] = lo[k]
                bwo_v[n, pl.ds(d + 16, 8, stride=OPITCH), :] = hi[k]

    scale_b = DHB ** -0.5

    def b_qkv_dots(i, st, n0, n1, hist=True):
        r0 = i * (TB // 2)
        if not isinstance(r0, int):
            r0 = pl.multiple_of(r0, TB // 2)

        def dot(n):
            lhs = _lhs([bxu[j, pl.ds(r0, TB // 2), :] for j in range(NC)])
            y = jnp.dot(lhs, _b16(bw_v[n]), preferred_element_type=f32)
            x_v[st * 24 + n, HALO:HALO + TB, :] = y * scale_b if n < 8 else y
            if n >= 8 and hist:
                x_v[((st + 1) % UB) * 24 + n, 0:HALO, :] = y[TB - HALO:TB]
            return y[TB - 8:TB]
        return [P(dot, n) for n in range(n0, n1)]

    def b_proj_dots(i, st):
        r0 = i * TB
        if not isinstance(r0, int):
            r0 = pl.multiple_of(r0, TB)

        def dot(n):
            lhs = _lhs([obu[st, j] for j in range(NC)])
            w = _b16(jnp.concatenate([bwo_v[n, OPITCH * u:OPITCH * u + 64, :] for u in range(8)], axis=0))
            y = jnp.dot(lhs, w, preferred_element_type=f32)
            outb_v[pl.ds(r0, TB), 128 * n:128 * n + 128] = y.astype(bf16)
            return y[TB - 8:TB]
        return [P(dot, n) for n in range(NC)]

    def rows8(s0, r):
        return x_v[s0:s0 + 8, r:r + 8, :]

    def pos_ok(g, w):
        return lax.broadcasted_iota(i32, (8, 8, 128), 1) + (8 * g) - DIL * w >= 0

    def at_qk(st, g):
        q = rows8(st * 24, HALO + 8 * g)
        p = [jnp.sum(q * rows8(st * 24 + 8, HALO + 8 * g - DIL * w), axis=0) for w in range(WIN)]
        x_v[X_PART + (st % 2) * NG + g, 0:64, :] = jnp.concatenate(p, axis=0)

    def at_softmax(st, g, first, pend):
        p = x_v[X_PART + (st % 2) * NG + g, 0:64, :]
        p = p + pltpu.roll(p, 32, 1)
        p = (p + pltpu.roll(p, 64, 1)).reshape(WIN, 8, 128)
        if first and 8 * g < DIL * (WIN - 1):
            p = jnp.where(pos_ok(g, lax.broadcasted_iota(i32, (8, 8, 128), 0)), p, -1e9)
        e = jnp.exp(p - jnp.max(p, axis=0, keepdims=True))
        l = jnp.sum(e, axis=0, keepdims=True)
        rc = pl.reciprocal(l, approx=True)
        pend[st, g] = e * (rc * (2.0 - l * rc))

    def at_store(st, g, pend):
        x_v[X_PROB + (st % 2) * NG + g, 0:64, :] = pend.pop((st, g)).reshape(64, 128)

    def at_pv(st, g, first):
        acc = None
        for w in range(WIN):
            e = x_v[X_PROB + (st % 2) * NG + g:X_PROB + (st % 2) * NG + g + 1, 8 * w:8 * w + 8, :]
            vv = rows8(st * 24 + 16, HALO + 8 * g - DIL * w)
            if first and 8 * g - DIL * w < 0:
                vv = jnp.where(pos_ok(g, w), vv, x_v[st * 24 + 16:st * 24 + 24, HALO:HALO + 1, :])
            acc = e * vv if acc is None else acc + e * vv
        x_v[X_OUT + (st % 2) * NG + g, 0:64, :] = acc.reshape(64, 128)

    def at_pack(st, g):
        o = [x_v[X_OUT + (st % 2) * NG + k, 0:64, :].reshape(8, 8, 128) for k in (g - 1, g)]
        ob_v[st, :, 8 * g - 8:8 * g + 8, :] = jnp.concatenate(o, axis=1).astype(bf16)

    pend = {}

    def attn_fill(fill, st, first, e_qk, e_pv, head=True, tail=True):
        for g in range(NG):
            if head:
                put(fill, e_qk(g), P(at_qk, st, g))
                put(fill, e_qk(g) + 1, P(at_softmax, st, g, first, pend))
                put(fill, e_qk(g) + 3, P(at_store, st, g, pend))
            if (head and g < NG - 1) or (tail and g == NG - 1):
                put(fill, e_pv(g), P(at_pv, st, g, first))
                if g % 2 == 1:
                    put(fill, e_pv(g) + 1, P(at_pack, st, g))

    def a_relayout(src0, dst0, g):
        src = stgu.at[pl.ds(pl.multiple_of(src0, 256), HW // 2), :]
        dst = wa_v.at[pl.ds(pl.multiple_of(dst0, 8), (H + 1) * PITCH + DM // 4 + 6), :]
        t = src[128 * g:128 * g + 128, :].reshape(4, 4, 8, 128)
        ev, od = pack_pairs(t[:, 0:2], t[:, 2:4])
        for dp in range(4):
            for o in range(2):
                dst[pl.ds(16 * o * PITCH + 4 * g + dp, 8, stride=2 * PITCH), :] = ev[dp, o]
                dst[pl.ds((16 * o + 1) * PITCH + 4 * g + dp, 8, stride=2 * PITCH), :] = od[dp, o]

    def sec(k0, k1, s):
        return [d for k in range(k0, k1) for d in b_qkv_dots(k, k, 8 * s, 8 * s + 8)]

    with _scope("perm_q"):
        x_v[8:24, 0:HALO, :] = jnp.zeros((16, HALO, 128), f32)
        for half in range(2):
            wait(bw_cps(0, half))
            if half == 0:
                start(bw_cps(2, 0) + bw_cps(2, 1) + bwo_cps() + bx_cps(1))
            for k in range(4):
                perm_select(0, half, k)
            for u in range(8):
                perm_gather(0, half, u, 0, 4)
    with _scope("Q01"):
        wait(bx_cps(0))
        run(sec(0, 2, 0), {})
    with _scope("Q2"):
        wait(bw_cps(1, 0))
        fill = {}
        perm_fill(fill, 1, 0, 0, 3, 5)
        run(sec(2, 3, 0), fill)
    with _scope("Q3K0"):
        wait(bw_cps(1, 1))
        start(bx_cps(2) + [aw_cp(0), mem_cp])
        fill = {}
        perm_fill(fill, 1, 1, 0, 3, 5)
        run(sec(3, 4, 0) + sec(0, 1, 1), fill)
    with _scope("K12"):
        wait(bw_cps(2, 0))
        fill = {}
        perm_fill(fill, 2, 0, 0, 6, 10)
        run(sec(1, 3, 1), fill)
    with _scope("K3V012"):
        wait(bw_cps(2, 1))
        fill = {}
        perm_fill(fill, 2, 1, 0, 3, 5)
        attn_fill(fill, 0, True, lambda g: 7 + g, lambda g: 15 + g)
        attn_fill(fill, 1, False, lambda g: 15 + g, lambda g: 23 + g, tail=False)
        run(b_qkv_dots(3, 3, 8, 16, hist=False) + sec(0, 3, 2), fill)
    with _scope("V3"):
        wait(bwo_cps())
        fill = {}
        for n in range(NC):
            put(fill, min(n, 6), P(prep_bwo, n))
        run(sec(3, 4, 2), fill)
        x_v[8:16, 0:HALO, :] = x_v[3 * 24 + 8:3 * 24 + 16, TB:TB + HALO, :]

    def b_body(it, carry):
        with _scope("it"):
            for c in range(1, NIT):
                @pl.when(it == c)
                def _():
                    if c < 6:
                        aw_cp(c).start()
                    start([awo_cp(c - 1), ax_cp(c - 1)] + ([awo_cp(NC - 1), ax_cp(NC - 1)] if c == 6 else []))
                    if c <= 2:
                        wait(bx_cps(c))
                    if c >= 2:
                        aw_cp(c - 2).wait()
            c = jnp.maximum(it - 2, 0)
            src0 = jnp.where(it == 1, STG_BW // 2, STG_AW // 2 + c * (HW // 2))
            dst0 = (c // 2) * (H * PITCH) + (c % 2) * (DM // 4)
            dots, fill = [], {}
            for k in range(UB):
                i, e0 = UB * it + k, 32 * k
                dots += b_qkv_dots(i, k, 0, 24) + b_proj_dots(i - 4, k)
                attn_fill(fill, (k - 3) % UB, False, None, lambda g: e0 + 2, head=False)
                attn_fill(fill, (k - 2) % UB, False, lambda g: e0 + 4 * g - (1 if 4 * g + e0 == 124 else 0),
                          lambda g: e0 + 4 * g + 6, tail=False)
                for g in range(16):
                    put(fill, min(e0 + 2 * g + 1, 126), P(a_relayout, src0, dst0, 16 * k + g))
            run(dots, fill, relayout=True)
            ob_cp(pl.multiple_of(UB * TB * (it - 1), UB * TB), UB * TB).start()
        return carry
    lax.fori_loop(1, NIT, b_body, 0)
    nb = S // TB
    with _scope("tailB"):
        fill = {}
        attn_fill(fill, 1, False, None, lambda g: 0, head=False)
        attn_fill(fill, 2, False, lambda g: g, lambda g: 4 + g)
        attn_fill(fill, 3, False, lambda g: 8 + g, lambda g: 12 + g)
        run([d for k in range(UB) for d in b_proj_dots(nb - 4 + k, k)], fill)
        ob_cp(S - UB * TB, UB * TB).start()

    wait([awo_cp(n) for n in range(NC)] + [ax_cp(j) for j in range(NC)] + [mem_cp])

    scale_a = DH ** -0.5
    rr = lax.broadcasted_iota(i32, (2 * L, 2 * L), 0)
    cc = lax.broadcasted_iota(i32, (2 * L, 2 * L), 1)
    rb_, cb_ = rr >= L, cc >= L
    ri, ci = jnp.where(rb_, rr - L, rr), jnp.where(cb_, cc - L, cc)
    same = rb_ == cb_
    valid = same & ((ri < M) | (ri >= ci))
    fill = jnp.where(same, -1e9, -jnp.inf).astype(f32)

    mem_s[...] = mem_v[...].astype(f32)
    NP = H // 2

    def a_step(lhs, even):
        qkv, pp = {}, {}
        nrow = 32 if even else 48

        def do_qkv(j):
            res = []
            for wi in range(3):
                parts = []
                for hh in (2 * j, 2 * j + 1):
                    w0 = (wi * H + hh) * PITCH
                    y = jnp.dot(lhs, _b16(wa_v[w0:w0 + DM // 2, :]), preferred_element_type=f32)
                    if even:
                        stash[wi * H + hh] = y[32:40]
                        parts += [y[40:48], y[0:32]]
                    else:
                        parts += [y[0:8], stash[wi * H + hh], y[8:32]]
                res.append(jnp.concatenate(parts, axis=0).astype(bf16))
            qkv[j] = res

        def do_qk(j):
            q2, k2, _ = qkv[j]
            s = lax.dot_general(q2, k2, (((1,), (1,)), ((), ())), preferred_element_type=f32) * scale_a
            s = jnp.where(valid, s, fill)
            m = jnp.max(s, axis=1, keepdims=True)
            e = jnp.exp(s - m)
            l = jnp.sum(e, axis=1, keepdims=True)
            rc = pl.reciprocal(l, approx=True)
            rc = rc * (2.0 - l * rc)
            pp[j] = (e * rc).astype(bf16)

        def do_pv(j):
            o2 = jnp.dot(pp.pop(j), qkv.pop(j)[2], preferred_element_type=f32)
            for i, hh in enumerate((2 * j, 2 * j + 1)):
                o = o2[L * i:L * (i + 1)]
                if even:
                    o_s[hh, 0:32, :] = o[0:32].astype(bf16)
                    ostash[hh] = o[32:40]
                else:
                    o_s[hh] = jnp.concatenate([o[0:8], ostash[hh], o[8:40]], axis=0).astype(bf16)

        def wo_part(n, h0, h1):
            lo = _lhs([osu[hh, 0:nrow // 2, :] for hh in range(h0, h1)])
            return jnp.dot(lo, _b16(wou[n, h0 * 64:h1 * 64, :]), preferred_element_type=f32)

        for j in range(NP):
            do_qkv(j)
            if j - LQK >= 0:
                do_qk(j - LQK)
            if j - LPV >= 0:
                do_pv(j - LPV)
        ya = []
        nper = NC // (LPV + 1)
        for j in range(NP, NP + LPV):
            for _ in range(nper):
                ya.append(wo_part(len(ya), 0, 2 * KA))
            if j - LQK < NP:
                do_qk(j - LQK)
            do_pv(j - LPV)
        while len(ya) < NC:
            ya.append(wo_part(len(ya), 0, 2 * KA))
        return jnp.concatenate([wo_part(n, 2 * KA, H) + ya[n] for n in range(NC)], axis=1)

    def a_body(t, c):
        with _scope("a_it"):
            return a_pair(t, c)

    def a_pair(t, c):
        r0 = pl.multiple_of(t * 32, 32)
        X = _lhs([axu[j, pl.ds(r0, 32), :] for j in range(NC)])
        Xm = X[32:48].astype(f32)
        mixed = jnp.concatenate([Xm[0:8], mem_s[...]], axis=0).astype(bf16)
        ye = a_step(jnp.concatenate([X[0:32], mixed], axis=0), True)
        mixed = jnp.concatenate([ye[0:8], Xm[8:16]], axis=0).astype(bf16)
        yo = a_step(jnp.concatenate([mixed, X[48:64]], axis=0), False)
        mem_s[...] = yo[0:8]
        o0 = pl.multiple_of(t * 64, 64)
        outa_v[pl.ds(o0, 64), :] = jnp.concatenate([ye[8:32], yo[8:48]], axis=0).astype(bf16)
        oa_cp(o0, 64).start()
        return c
    lax.fori_loop(0, S // 64, a_body, 0)

    ob_cp(0, S).wait()
    oa_cp(0, S).wait()


@jax.jit
def _run(A_x, A_mem0, A_Wq, A_Wk, A_Wv, A_Wo, B_x, B_wqkv, B_wo):
    hbm = pl.BlockSpec(memory_space=pl.ANY)
    out = pl.pallas_call(
        _kernel,
        out_shape=jax.ShapeDtypeStruct((S, 2 * DM), bf16),
        in_specs=[hbm] * 9,
        out_specs=hbm,
        scratch_shapes=[
            pltpu.VMEM((NC, S, 128), bf16),
            pltpu.VMEM((M, DM), bf16),
            pltpu.VMEM((STG_ROWS, 128), bf16),
            pltpu.VMEM((WA_DUM + 8, 128), u32),
            pltpu.VMEM((NC, H * DH, 128), bf16),
            pltpu.VMEM((NC, S, 128), bf16),
            pltpu.VMEM((24, DM // 2, 128), u32),
            pltpu.VMEM((NC, 9 * OPITCH + 4, 128), u32),
            pltpu.VMEM((S, DM), bf16),
            pltpu.VMEM((S, DM), bf16),
            pltpu.VMEM((X_SLABS, TB + HALO, 128), f32),
            pltpu.VMEM((UB, 8, TB, 128), bf16),
            pltpu.VMEM((M, DM), f32),
            pltpu.VMEM((3 * H, 8, DH), f32),
            pltpu.VMEM((H, 8, DH), f32),
            pltpu.VMEM((H, 48, DH), bf16),
            pltpu.SMEM((1,), i32),
            pltpu.SemaphoreType.DMA((NSEM,)),
        ],
        compiler_params=pltpu.CompilerParams(vmem_limit_bytes=110 * 1024 * 1024),
    )(
        A_x.reshape(S, DM), A_mem0.reshape(M, DM),
        A_Wq.reshape(DM * H, DH), A_Wk.reshape(DM * H, DH), A_Wv.reshape(DM * H, DH),
        A_Wo.reshape(H * DH, DM),
        B_x.reshape(S, DM), B_wqkv, B_wo,
    )
    return out.reshape(1, S, 2 * DM)


def pallas_concat_heads__memory_aug_recurrent_mem_tr__sliding_local_dilated__prompt_kernel(
    A_x, A_mem0, A_Wq, A_Wk, A_Wv, A_Wo, A_seg_len, B_x, B_wqkv, B_wo,
):
    if isinstance(A_seg_len, int):
        assert A_seg_len == SEG
    return _run(A_x, A_mem0, A_Wq, A_Wk, A_Wv, A_Wo, B_x, B_wqkv, B_wo)
```

```python
import contextlib
import functools

import jax
import jax.numpy as jnp
from jax import lax
import jax.experimental.pallas as pl
import jax.experimental.pallas.tpu as pltpu

bf16, f32, u32, i32 = jnp.bfloat16, jnp.float32, jnp.uint32, jnp.int32

S, DM = 2048, 1024
H, DH = 32, 128
M, SEG = 8, 32
L = M + SEG
DHB, WIN, DIL = 32, 8, 2
NC = DM // 128

TB = 64
UB = 4
HALO = 16
NIT = S // (TB * UB)
LQK, LPV, KA = 1, 3, 12

PITCH = DM // 2 + 2
WA_DUM = (3 * H + 2) * PITCH + 12
OPITCH = 68
HW = DM * H // 2
STG_AW, STG_BW, STG_BWO = 0, 6 * HW, 6 * HW + 24 * DM
STG_TOK = STG_BWO + NC * DM
STG_ROWS = STG_TOK + 16
NG = TB // 8
X_PART = UB * 24
X_PROB = X_PART + 2 * NG
X_OUT = X_PROB + 2 * NG
X_TMP = X_OUT + 2 * NG
X_FEN = X_TMP + 32
X_SLABS = X_FEN + 1

SEM_BW, SEM_BX, SEM_BWO, SEM_AW, SEM_AWO, SEM_AX, SEM_MEM, SEM_OB, SEM_OA = 0, 6, 9, 10, 16, 17, 18, 19, 20
NSEM = 21
_SCOPES = False


def _scope(name):
    return jax.named_scope(name) if _SCOPES else contextlib.nullcontext()


def _b16(v):
    return pltpu.bitcast(v, bf16)


def _lhs(blocks):
    return _b16(jnp.concatenate(blocks, axis=1))


def _kernel(ax_h, mem_h, wq_h, wk_h, wv_h, wo_h, bx_h, bw_h, bwo_h, out_h,
            ax_v, mem_v, stg_v, wa_v, wo_v, bx_v, bw_v, bwo_v, outa_v, outb_v,
            x_v, ob_v, mem_s, stash, ostash, o_s, zero_s, sem):
    P = functools.partial

    def bw_cps(s, half):
        return [pltpu.make_async_copy(bw_h.at[pl.ds(half * (DM // 2), DM // 2), pl.ds(128 * n, 128)],
                                      stg_v.at[pl.ds(STG_BW + DM * n + half * (DM // 2), DM // 2), :],
                                      sem.at[SEM_BW + 2 * s + half]) for n in range(8 * s, 8 * s + 8)]

    def bx_cps(part):
        rows = (pl.ds(0, TB * UB), pl.ds(TB * UB, TB * UB), pl.ds(2 * TB * UB, S - 2 * TB * UB))[part]
        return [pltpu.make_async_copy(bx_h.at[rows, pl.ds(128 * j, 128)], bx_v.at[j, rows, :],
                                      sem.at[SEM_BX + part]) for j in range(NC)]

    def bwo_cps():
        return [pltpu.make_async_copy(bwo_h.at[:, pl.ds(128 * n, 128)], stg_v.at[pl.ds(STG_BWO + DM * n, DM), :],
                                      sem.at[SEM_BWO]) for n in range(NC)]

    def aw_cp(c):
        src = (wq_h, wk_h, wv_h)[c // 2]
        return pltpu.make_async_copy(src.at[pl.ds((c % 2) * HW, HW), :], stg_v.at[pl.ds(STG_AW + c * HW, HW), :],
                                     sem.at[SEM_AW + c])

    def awo_cp(n):
        return pltpu.make_async_copy(wo_h.at[:, pl.ds(128 * n, 128)], wo_v.at[n], sem.at[SEM_AWO])

    def ax_cp(j):
        return pltpu.make_async_copy(ax_h.at[:, pl.ds(128 * j, 128)], ax_v.at[j], sem.at[SEM_AX])

    mem_cp = pltpu.make_async_copy(mem_h, mem_v, sem.at[SEM_MEM])

    def ob_cp(r0, n):
        return pltpu.make_async_copy(outb_v.at[pl.ds(r0, n), :], out_h.at[pl.ds(r0, n), pl.ds(DM, DM)],
                                     sem.at[SEM_OB])

    def oa_cp(r0, n):
        return pltpu.make_async_copy(outa_v.at[pl.ds(r0, n), :], out_h.at[pl.ds(r0, n), pl.ds(0, DM)],
                                     sem.at[SEM_OA])

    def start(cps):
        for c in cps:
            c.start()

    def wait(cps):
        for c in cps:
            c.wait()

    start(bw_cps(0, 0) + bw_cps(0, 1) + bx_cps(0) + bw_cps(1, 0) + bw_cps(1, 1))

    bxu, stgu, obu = bx_v.bitcast(u32), stg_v.bitcast(u32), ob_v.bitcast(u32)
    wou, axu, osu = wo_v.bitcast(u32), ax_v.bitcast(u32), o_s.bitcast(u32)

    zero_s[0] = 0
    wa_v[WA_DUM:WA_DUM + 8, :] = jnp.zeros((8, 128), u32)

    def run(dots, fill, relayout=False):
        z = pl.multiple_of(zero_s[0], 8)
        for n, d in enumerate(dots):
            y = d()
            if fill.get(n) or fill.get(n - 1):
                if relayout:
                    x_v[X_FEN, 0:8, :] = pltpu.bitcast(wa_v[WA_DUM:WA_DUM + 8, :], f32)
                x_v[z + X_FEN, 0:8, :] = y
                stgu[pl.ds(z + STG_TOK // 2, 8), :] = pltpu.bitcast(x_v[X_FEN, 0:8, :], u32)
            for f in fill.get(n, []):
                f()
        for n in sorted(fill):
            if n >= len(dots):
                for f in fill[n]:
                    f()

    def put(fill, n, f):
        fill.setdefault(n, []).append(f)

    lane16 = lax.broadcasted_iota(i32, (16, 128), 1)

    def perm_select(s, half, k):
        bits = [((lane16 >> (b + 1)) & 1) == 1 for b in range(3)]
        for r in range(0, 64, 16):
            src = (STG_BW + 8 * s * DM) // 2 + half * 256 + 64 * k + r
            zs = [stgu[src + ((-t) % 8) * (DM // 2):src + ((-t) % 8) * (DM // 2) + 16, :] for t in range(8)]
            for b in range(3):
                zs = [lax.select(bits[b], zs[(t - (1 << b)) % 8], zs[t]) for t in range(8)]
            for u in range(8):
                x_v[X_TMP + 4 * u + k, r:r + 16, :] = pltpu.bitcast(zs[u], f32)

    def perm_gather(s, half, u, k0, k1):
        n = 64 * (k1 - k0)
        lane = lax.broadcasted_iota(i32, (n, 128), 1)
        idx = 32 * ((lane >> 3) & 3) + 16 * (lane >> 6) + 2 * ((u + lane) & 7) + ((lane >> 5) & 1)
        t = pltpu.bitcast(x_v[X_TMP + 4 * u + k0:X_TMP + 4 * u + k1, 0:64, :].reshape(n, 128), u32)
        bw_v[8 * s + u, half * 256 + 64 * k0:half * 256 + 64 * k1, :] = jnp.take_along_axis(t, idx, axis=1)

    def perm_fill(fill, s, half, n0, ns, ng):
        for k in range(4):
            put(fill, n0 + k * ns // 4, P(perm_select, s, half, k))
        g0 = n0 + ns // 4 + 1
        for k in range(16):
            rh, u = k // 8, k % 8
            e = max(g0 + k * ng // 16, n0 + (2 * rh + 1) * ns // 4 + 1)
            put(fill, e, P(perm_gather, s, half, u, 2 * rh, 2 * rh + 2))

    def pack_pairs(a, b):
        return (a & jnp.uint32(0xFFFF)) | (b << 16), (a >> 16) | (b & jnp.uint32(0xFFFF0000))

    def prep_bwo(n):
        for v in range(0, 8, 2):
            r = (STG_BWO + n * DM) // 2 + 64 * v
            a = stgu[r:r + 64, :].reshape(8, 8, 128)
            b = stgu[r + 64:r + 128, :].reshape(8, 8, 128)
            a = pltpu.roll(a, 8 - v, 1) if v else a
            lo, hi = pack_pairs(a, pltpu.roll(b, 7 - v, 1))
            for k in range(8):
                d = 32 * (k % 2) + 4 * (k // 2) + v // 2
                bwo_v[n, pl.ds(d, 8, stride=OPITCH), :] = lo[k]
                bwo_v[n, pl.ds(d + 16, 8, stride=OPITCH), :] = hi[k]

    scale_b = DHB ** -0.5

    def b_qkv_dots(i, st, n0, n1, hist=True):
        r0 = i * (TB // 2)
        if not isinstance(r0, int):
            r0 = pl.multiple_of(r0, TB // 2)

        def dot(n):
            lhs = _lhs([bxu[j, pl.ds(r0, TB // 2), :] for j in range(NC)])
            y = jnp.dot(lhs, _b16(bw_v[n]), preferred_element_type=f32)
            x_v[st * 24 + n, HALO:HALO + TB, :] = y * scale_b if n < 8 else y
            if n >= 8 and hist:
                x_v[((st + 1) % UB) * 24 + n, 0:HALO, :] = y[TB - HALO:TB]
            return y[TB - 8:TB]
        return [P(dot, n) for n in range(n0, n1)]

    def b_proj_dots(i, st):
        r0 = i * TB
        if not isinstance(r0, int):
            r0 = pl.multiple_of(r0, TB)

        def dot(n):
            lhs = _lhs([obu[st, j] for j in range(NC)])
            w = _b16(jnp.concatenate([bwo_v[n, OPITCH * u:OPITCH * u + 64, :] for u in range(8)], axis=0))
            y = jnp.dot(lhs, w, preferred_element_type=f32)
            outb_v[pl.ds(r0, TB), 128 * n:128 * n + 128] = y.astype(bf16)
            return y[TB - 8:TB]
        return [P(dot, n) for n in range(NC)]

    def rows8(s0, r):
        return x_v[s0:s0 + 8, r:r + 8, :]

    def pos_ok(g, w):
        return lax.broadcasted_iota(i32, (8, 8, 128), 1) + (8 * g) - DIL * w >= 0

    def at_qk(st, g):
        q = rows8(st * 24, HALO + 8 * g)
        p = [jnp.sum(q * rows8(st * 24 + 8, HALO + 8 * g - DIL * w), axis=0) for w in range(WIN)]
        x_v[X_PART + (st % 2) * NG + g, 0:64, :] = jnp.concatenate(p, axis=0)

    def at_softmax(st, g, first, pend):
        p = x_v[X_PART + (st % 2) * NG + g, 0:64, :]
        p = p + pltpu.roll(p, 32, 1)
        p = (p + pltpu.roll(p, 64, 1)).reshape(WIN, 8, 128)
        if first and 8 * g < DIL * (WIN - 1):
            p = jnp.where(pos_ok(g, lax.broadcasted_iota(i32, (8, 8, 128), 0)), p, -1e9)
        e = jnp.exp(p - jnp.max(p, axis=0, keepdims=True))
        l = jnp.sum(e, axis=0, keepdims=True)
        rc = pl.reciprocal(l, approx=True)
        pend[st, g] = e * (rc * (2.0 - l * rc))

    def at_store(st, g, pend):
        x_v[X_PROB + (st % 2) * NG + g, 0:64, :] = pend.pop((st, g)).reshape(64, 128)

    def at_pv(st, g, first):
        acc = None
        for w in range(WIN):
            e = x_v[X_PROB + (st % 2) * NG + g:X_PROB + (st % 2) * NG + g + 1, 8 * w:8 * w + 8, :]
            vv = rows8(st * 24 + 16, HALO + 8 * g - DIL * w)
            if first and 8 * g - DIL * w < 0:
                vv = jnp.where(pos_ok(g, w), vv, x_v[st * 24 + 16:st * 24 + 24, HALO:HALO + 1, :])
            acc = e * vv if acc is None else acc + e * vv
        x_v[X_OUT + (st % 2) * NG + g, 0:64, :] = acc.reshape(64, 128)

    def at_pack(st, g):
        o = [x_v[X_OUT + (st % 2) * NG + k, 0:64, :].reshape(8, 8, 128) for k in (g - 1, g)]
        ob_v[st, :, 8 * g - 8:8 * g + 8, :] = jnp.concatenate(o, axis=1).astype(bf16)

    pend = {}

    def attn_fill(fill, st, first, e_qk, e_pv, head=True, tail=True):
        for g in range(NG):
            if head:
                put(fill, e_qk(g), P(at_qk, st, g))
                put(fill, e_qk(g) + 1, P(at_softmax, st, g, first, pend))
                put(fill, e_qk(g) + 3, P(at_store, st, g, pend))
            if (head and g < NG - 1) or (tail and g == NG - 1):
                put(fill, e_pv(g), P(at_pv, st, g, first))
                if g % 2 == 1:
                    put(fill, e_pv(g) + 1, P(at_pack, st, g))

    def a_relayout(src0, dst0, g):
        src = stgu.at[pl.ds(pl.multiple_of(src0, 256), HW // 2), :]
        dst = wa_v.at[pl.ds(pl.multiple_of(dst0, 8), (H + 1) * PITCH + DM // 4 + 6), :]
        t = src[128 * g:128 * g + 128, :].reshape(4, 4, 8, 128)
        ev, od = pack_pairs(t[:, 0:2], t[:, 2:4])
        for dp in range(4):
            for o in range(2):
                dst[pl.ds(16 * o * PITCH + 4 * g + dp, 8, stride=2 * PITCH), :] = ev[dp, o]
                dst[pl.ds((16 * o + 1) * PITCH + 4 * g + dp, 8, stride=2 * PITCH), :] = od[dp, o]

    def sec(k0, k1, s):
        return [d for k in range(k0, k1) for d in b_qkv_dots(k, k, 8 * s, 8 * s + 8)]

    with _scope("perm_q"):
        x_v[8:24, 0:HALO, :] = jnp.zeros((16, HALO, 128), f32)
        for half in range(2):
            wait(bw_cps(0, half))
            if half == 0:
                start(bw_cps(2, 0) + bw_cps(2, 1) + bwo_cps() + bx_cps(1))
            for k in range(4):
                perm_select(0, half, k)
            for u in range(8):
                perm_gather(0, half, u, 0, 4)
    with _scope("Q01"):
        wait(bx_cps(0))
        run(sec(0, 2, 0), {})
    with _scope("Q2"):
        wait(bw_cps(1, 0))
        fill = {}
        perm_fill(fill, 1, 0, 0, 3, 5)
        run(sec(2, 3, 0), fill)
    with _scope("Q3K0"):
        wait(bw_cps(1, 1))
        start(bx_cps(2) + [aw_cp(0), mem_cp])
        fill = {}
        perm_fill(fill, 1, 1, 0, 3, 5)
        run(sec(3, 4, 0) + sec(0, 1, 1), fill)
    with _scope("K12"):
        wait(bw_cps(2, 0))
        fill = {}
        perm_fill(fill, 2, 0, 0, 6, 10)
        run(sec(1, 3, 1), fill)
    with _scope("K3V012"):
        wait(bw_cps(2, 1))
        fill = {}
        perm_fill(fill, 2, 1, 0, 3, 5)
        attn_fill(fill, 0, True, lambda g: 7 + g, lambda g: 15 + g)
        attn_fill(fill, 1, False, lambda g: 15 + g, lambda g: 23 + g, tail=False)
        run(b_qkv_dots(3, 3, 8, 16, hist=False) + sec(0, 3, 2), fill)
    with _scope("V3"):
        wait(bwo_cps())
        fill = {}
        for n in range(NC):
            put(fill, min(n, 6), P(prep_bwo, n))
        run(sec(3, 4, 2), fill)
        x_v[8:16, 0:HALO, :] = x_v[3 * 24 + 8:3 * 24 + 16, TB:TB + HALO, :]

    def b_body(it, carry):
        with _scope("it"):
            for c in range(1, NIT):
                @pl.when(it == c)
                def _():
                    if c < 6:
                        aw_cp(c).start()
                    start([awo_cp(c - 1), ax_cp(c - 1)] + ([awo_cp(NC - 1), ax_cp(NC - 1)] if c == 6 else []))
                    if c <= 2:
                        wait(bx_cps(c))
                    if c >= 2:
                        aw_cp(c - 2).wait()
            c = jnp.maximum(it - 2, 0)
            src0 = jnp.where(it == 1, STG_BW // 2, STG_AW // 2 + c * (HW // 2))
            dst0 = (c // 2) * (H * PITCH) + (c % 2) * (DM // 4)
            dots, fill = [], {}
            for k in range(UB):
                i, e0 = UB * it + k, 32 * k
                dots += b_qkv_dots(i, k, 0, 24) + b_proj_dots(i - 4, k)
                attn_fill(fill, (k - 3) % UB, False, None, lambda g: e0 + 2, head=False)
                attn_fill(fill, (k - 2) % UB, False, lambda g: e0 + 4 * g - (1 if 4 * g + e0 == 124 else 0),
                          lambda g: e0 + 4 * g + 6, tail=False)
                for g in range(16):
                    put(fill, min(e0 + 2 * g + 1, 126), P(a_relayout, src0, dst0, 16 * k + g))
            run(dots, fill, relayout=True)
            ob_cp(pl.multiple_of(UB * TB * (it - 1), UB * TB), UB * TB).start()
        return carry
    lax.fori_loop(1, NIT, b_body, 0)
    nb = S // TB
    with _scope("tailB"):
        fill = {}
        attn_fill(fill, 1, False, None, lambda g: 0, head=False)
        attn_fill(fill, 2, False, lambda g: g, lambda g: 4 + g)
        attn_fill(fill, 3, False, lambda g: 8 + g, lambda g: 12 + g)
        run([d for k in range(UB) for d in b_proj_dots(nb - 4 + k, k)], fill)
        ob_cp(S - UB * TB, UB * TB).start()

    wait([awo_cp(n) for n in range(NC)] + [ax_cp(j) for j in range(NC)] + [mem_cp])

    scale_a = DH ** -0.5
    rr = lax.broadcasted_iota(i32, (2 * L, 2 * L), 0)
    cc = lax.broadcasted_iota(i32, (2 * L, 2 * L), 1)
    rb_, cb_ = rr >= L, cc >= L
    ri, ci = jnp.where(rb_, rr - L, rr), jnp.where(cb_, cc - L, cc)
    same = rb_ == cb_
    valid = same & ((ri < M) | (ri >= ci))
    fill = jnp.where(same, -1e9, -jnp.inf).astype(f32)

    mem_s[...] = mem_v[...].astype(f32)
    NP = H // 2

    def a_step(lhs, even):
        qkv, pp = {}, {}
        nrow = 32 if even else 48

        def proj(wh, k0, k1):
            w0 = wh * PITCH
            return jnp.dot(lhs[:, k0:k1], _b16(wa_v[w0 + k0 // 2:w0 + k1 // 2, :]), preferred_element_type=f32)

        def do_qkv(j):
            split = j == 0 and not even
            lo = {wi * H + hh: proj(wi * H + hh, 0, DM // 2) for wi in range(3) for hh in (0, 1)} if split else {}
            res = []
            for wi in range(3):
                parts = []
                for hh in (2 * j, 2 * j + 1):
                    wh = wi * H + hh
                    y = proj(wh, DM // 2, DM) + lo[wh] if split else proj(wh, 0, DM)
                    if even:
                        stash[wh] = y[32:40]
                        parts += [y[40:48], y[0:32]]
                    else:
                        parts += [y[0:8], stash[wh], y[8:32]]
                res.append(jnp.concatenate(parts, axis=0).astype(bf16))
            qkv[j] = res

        def do_qk(j):
            q2, k2, _ = qkv[j]
            s = lax.dot_general(q2, k2, (((1,), (1,)), ((), ())), preferred_element_type=f32) * scale_a
            s = jnp.where(valid, s, fill)
            m = jnp.max(s, axis=1, keepdims=True)
            e = jnp.exp(s - m)
            l = jnp.sum(e, axis=1, keepdims=True)
            rc = pl.reciprocal(l, approx=True)
            rc = rc * (2.0 - l * rc)
            pp[j] = (e * rc).astype(bf16)

        def do_pv(j):
            o2 = jnp.dot(pp.pop(j), qkv.pop(j)[2], preferred_element_type=f32)
            for i, hh in enumerate((2 * j, 2 * j + 1)):
                o = o2[L * i:L * (i + 1)]
                if even:
                    o_s[hh, 0:32, :] = o[0:32].astype(bf16)
                    ostash[hh] = o[32:40]
                else:
                    o_s[hh] = jnp.concatenate([o[0:8], ostash[hh], o[8:40]], axis=0).astype(bf16)

        def wo_part(n, h0, h1):
            lo = _lhs([osu[hh, 0:nrow // 2, :] for hh in range(h0, h1)])
            return jnp.dot(lo, _b16(wou[n, h0 * 64:h1 * 64, :]), preferred_element_type=f32)

        for j in range(NP):
            do_qkv(j)
            if j - LQK >= 0:
                do_qk(j - LQK)
            if j - LPV >= 0:
                do_pv(j - LPV)
        ya = []
        nper = NC // (LPV + 1)
        for j in range(NP, NP + LPV):
            for _ in range(nper):
                ya.append(wo_part(len(ya), 0, 2 * KA))
            if j - LQK < NP:
                do_qk(j - LQK)
            do_pv(j - LPV)
        while len(ya) < NC:
            ya.append(wo_part(len(ya), 0, 2 * KA))
        return jnp.concatenate([wo_part(n, 2 * KA, H) + ya[n] for n in range(NC)], axis=1)

    def a_body(t, c):
        with _scope("a_it"):
            return a_pair(t, c)

    def a_pair(t, c):
        r0 = pl.multiple_of(t * 32, 32)
        X = _lhs([axu[j, pl.ds(r0, 32), :] for j in range(NC)])
        Xm = X[32:48].astype(f32)
        mixed = jnp.concatenate([Xm[0:8], mem_s[...]], axis=0).astype(bf16)
        ye = a_step(jnp.concatenate([X[0:32], mixed], axis=0), True)
        mixed = jnp.concatenate([ye[0:8], Xm[8:16]], axis=0).astype(bf16)
        yo = a_step(jnp.concatenate([mixed, X[48:64]], axis=0), False)
        mem_s[...] = yo[0:8]
        o0 = pl.multiple_of(t * 64, 64)
        outa_v[pl.ds(o0, 64), :] = jnp.concatenate([ye[8:32], yo[8:48]], axis=0).astype(bf16)
        oa_cp(o0, 64).start()
        return c
    lax.fori_loop(0, S // 64, a_body, 0)

    ob_cp(0, S).wait()
    oa_cp(0, S).wait()


@jax.jit
def _run(A_x, A_mem0, A_Wq, A_Wk, A_Wv, A_Wo, B_x, B_wqkv, B_wo):
    hbm = pl.BlockSpec(memory_space=pl.ANY)
    out = pl.pallas_call(
        _kernel,
        out_shape=jax.ShapeDtypeStruct((S, 2 * DM), bf16),
        in_specs=[hbm] * 9,
        out_specs=hbm,
        scratch_shapes=[
            pltpu.VMEM((NC, S, 128), bf16),
            pltpu.VMEM((M, DM), bf16),
            pltpu.VMEM((STG_ROWS, 128), bf16),
            pltpu.VMEM((WA_DUM + 8, 128), u32),
            pltpu.VMEM((NC, H * DH, 128), bf16),
            pltpu.VMEM((NC, S, 128), bf16),
            pltpu.VMEM((24, DM // 2, 128), u32),
            pltpu.VMEM((NC, 9 * OPITCH + 4, 128), u32),
            pltpu.VMEM((S, DM), bf16),
            pltpu.VMEM((S, DM), bf16),
            pltpu.VMEM((X_SLABS, TB + HALO, 128), f32),
            pltpu.VMEM((UB, 8, TB, 128), bf16),
            pltpu.VMEM((M, DM), f32),
            pltpu.VMEM((3 * H, 8, DH), f32),
            pltpu.VMEM((H, 8, DH), f32),
            pltpu.VMEM((H, 48, DH), bf16),
            pltpu.SMEM((1,), i32),
            pltpu.SemaphoreType.DMA((NSEM,)),
        ],
        compiler_params=pltpu.CompilerParams(vmem_limit_bytes=110 * 1024 * 1024),
    )(
        A_x.reshape(S, DM), A_mem0.reshape(M, DM),
        A_Wq.reshape(DM * H, DH), A_Wk.reshape(DM * H, DH), A_Wv.reshape(DM * H, DH),
        A_Wo.reshape(H * DH, DM),
        B_x.reshape(S, DM), B_wqkv, B_wo,
    )
    return out.reshape(1, S, 2 * DM)


def pallas_concat_heads__memory_aug_recurrent_mem_tr__sliding_local_dilated__prompt_kernel(
    A_x, A_mem0, A_Wq, A_Wk, A_Wv, A_Wo, A_seg_len, B_x, B_wqkv, B_wo,
):
    if isinstance(A_seg_len, int):
        assert A_seg_len == SEG
    return _run(A_x, A_mem0, A_Wq, A_Wk, A_Wv, A_Wo, B_x, B_wqkv, B_wo)
```

```python
import contextlib
import functools

import jax
import jax.numpy as jnp
from jax import lax
import jax.experimental.pallas as pl
import jax.experimental.pallas.tpu as pltpu

bf16, f32, u32, i32 = jnp.bfloat16, jnp.float32, jnp.uint32, jnp.int32

S, DM = 2048, 1024
H, DH = 32, 128
M, SEG = 8, 32
L = M + SEG
DHB, WIN, DIL = 32, 8, 2
NC = DM // 128

TB = 64
UB = 4
HALO = 16
NIT = S // (TB * UB)
LQK, LPV, KA, NI = 1, 3, 12, 3

PITCH = DM // 2 + 2
WA_DUM = (3 * H + 2) * PITCH + 12
OPITCH = 68
HW = DM * H // 2
STG_AW, STG_BW, STG_BWO = 0, 6 * HW, 6 * HW + 24 * DM
STG_TOK = STG_BWO + NC * DM
STG_ROWS = STG_TOK + 16
NG = TB // 8
X_PART = UB * 24
X_PROB = X_PART + 2 * NG
X_OUT = X_PROB + 2 * NG
X_TMP = X_OUT + 2 * NG
X_FEN = X_TMP + 32
X_SLABS = X_FEN + 1

SEM_BW, SEM_BX, SEM_BWO, SEM_AW, SEM_AWO, SEM_AX, SEM_MEM, SEM_OB, SEM_OA = 0, 6, 9, 10, 16, 17, 18, 19, 20
NSEM = 21
_SCOPES = False


def _scope(name):
    return jax.named_scope(name) if _SCOPES else contextlib.nullcontext()


def _b16(v):
    return pltpu.bitcast(v, bf16)


def _lhs(blocks):
    return _b16(jnp.concatenate(blocks, axis=1))


def _kernel(ax_h, mem_h, wq_h, wk_h, wv_h, wo_h, bx_h, bw_h, bwo_h, out_h,
            ax_v, mem_v, stg_v, wa_v, wo_v, bx_v, bw_v, bwo_v, outa_v, outb_v,
            x_v, ob_v, mem_s, stash, ostash, o_s, zero_s, sem):
    P = functools.partial

    def bw_cps(s, half):
        return [pltpu.make_async_copy(bw_h.at[pl.ds(half * (DM // 2), DM // 2), pl.ds(128 * n, 128)],
                                      stg_v.at[pl.ds(STG_BW + DM * n + half * (DM // 2), DM // 2), :],
                                      sem.at[SEM_BW + 2 * s + half]) for n in range(8 * s, 8 * s + 8)]

    def bx_cps(part):
        rows = (pl.ds(0, TB * UB), pl.ds(TB * UB, TB * UB), pl.ds(2 * TB * UB, S - 2 * TB * UB))[part]
        return [pltpu.make_async_copy(bx_h.at[rows, pl.ds(128 * j, 128)], bx_v.at[j, rows, :],
                                      sem.at[SEM_BX + part]) for j in range(NC)]

    def bwo_cps():
        return [pltpu.make_async_copy(bwo_h.at[:, pl.ds(128 * n, 128)], stg_v.at[pl.ds(STG_BWO + DM * n, DM), :],
                                      sem.at[SEM_BWO]) for n in range(NC)]

    def aw_cp(c):
        src = (wq_h, wk_h, wv_h)[c // 2]
        return pltpu.make_async_copy(src.at[pl.ds((c % 2) * HW, HW), :], stg_v.at[pl.ds(STG_AW + c * HW, HW), :],
                                     sem.at[SEM_AW + c])

    def awo_cp(n):
        return pltpu.make_async_copy(wo_h.at[:, pl.ds(128 * n, 128)], wo_v.at[n], sem.at[SEM_AWO])

    def ax_cp(j):
        return pltpu.make_async_copy(ax_h.at[:, pl.ds(128 * j, 128)], ax_v.at[j], sem.at[SEM_AX])

    mem_cp = pltpu.make_async_copy(mem_h, mem_v, sem.at[SEM_MEM])

    def ob_cp(r0, n):
        return pltpu.make_async_copy(outb_v.at[pl.ds(r0, n), :], out_h.at[pl.ds(r0, n), pl.ds(DM, DM)],
                                     sem.at[SEM_OB])

    def oa_cp(r0, n):
        return pltpu.make_async_copy(outa_v.at[pl.ds(r0, n), :], out_h.at[pl.ds(r0, n), pl.ds(0, DM)],
                                     sem.at[SEM_OA])

    def start(cps):
        for c in cps:
            c.start()

    def wait(cps):
        for c in cps:
            c.wait()

    start(bw_cps(0, 0) + bw_cps(0, 1) + bx_cps(0) + bw_cps(1, 0) + bw_cps(1, 1))

    bxu, stgu, obu = bx_v.bitcast(u32), stg_v.bitcast(u32), ob_v.bitcast(u32)
    wou, axu, osu = wo_v.bitcast(u32), ax_v.bitcast(u32), o_s.bitcast(u32)

    zero_s[0] = 0
    wa_v[WA_DUM:WA_DUM + 8, :] = jnp.zeros((8, 128), u32)

    def run(dots, fill, relayout=False):
        z = pl.multiple_of(zero_s[0], 8)
        for n, d in enumerate(dots):
            y = d()
            if fill.get(n) or fill.get(n - 1):
                if relayout:
                    x_v[X_FEN, 0:8, :] = pltpu.bitcast(wa_v[WA_DUM:WA_DUM + 8, :], f32)
                x_v[z + X_FEN, 0:8, :] = y
                stgu[pl.ds(z + STG_TOK // 2, 8), :] = pltpu.bitcast(x_v[X_FEN, 0:8, :], u32)
            for f in fill.get(n, []):
                f()
        for n in sorted(fill):
            if n >= len(dots):
                for f in fill[n]:
                    f()

    def put(fill, n, f):
        fill.setdefault(n, []).append(f)

    lane16 = lax.broadcasted_iota(i32, (16, 128), 1)

    def perm_select(s, half, k):
        bits = [((lane16 >> (b + 1)) & 1) == 1 for b in range(3)]
        for r in range(0, 64, 16):
            src = (STG_BW + 8 * s * DM) // 2 + half * 256 + 64 * k + r
            zs = [stgu[src + ((-t) % 8) * (DM // 2):src + ((-t) % 8) * (DM // 2) + 16, :] for t in range(8)]
            for b in range(3):
                zs = [lax.select(bits[b], zs[(t - (1 << b)) % 8], zs[t]) for t in range(8)]
            for u in range(8):
                x_v[X_TMP + 4 * u + k, r:r + 16, :] = pltpu.bitcast(zs[u], f32)

    def perm_gather(s, half, u, k0, k1):
        n = 64 * (k1 - k0)
        lane = lax.broadcasted_iota(i32, (n, 128), 1)
        idx = 32 * ((lane >> 3) & 3) + 16 * (lane >> 6) + 2 * ((u + lane) & 7) + ((lane >> 5) & 1)
        t = pltpu.bitcast(x_v[X_TMP + 4 * u + k0:X_TMP + 4 * u + k1, 0:64, :].reshape(n, 128), u32)
        bw_v[8 * s + u, half * 256 + 64 * k0:half * 256 + 64 * k1, :] = jnp.take_along_axis(t, idx, axis=1)

    def perm_fill(fill, s, half, n0, ns, ng):
        for k in range(4):
            put(fill, n0 + k * ns // 4, P(perm_select, s, half, k))
        g0 = n0 + ns // 4 + 1
        for k in range(16):
            rh, u = k // 8, k % 8
            e = max(g0 + k * ng // 16, n0 + (2 * rh + 1) * ns // 4 + 1)
            put(fill, e, P(perm_gather, s, half, u, 2 * rh, 2 * rh + 2))

    def pack_pairs(a, b):
        return (a & jnp.uint32(0xFFFF)) | (b << 16), (a >> 16) | (b & jnp.uint32(0xFFFF0000))

    def prep_bwo(n):
        for v in range(0, 8, 2):
            r = (STG_BWO + n * DM) // 2 + 64 * v
            a = stgu[r:r + 64, :].reshape(8, 8, 128)
            b = stgu[r + 64:r + 128, :].reshape(8, 8, 128)
            a = pltpu.roll(a, 8 - v, 1) if v else a
            lo, hi = pack_pairs(a, pltpu.roll(b, 7 - v, 1))
            for k in range(8):
                d = 32 * (k % 2) + 4 * (k // 2) + v // 2
                bwo_v[n, pl.ds(d, 8, stride=OPITCH), :] = lo[k]
                bwo_v[n, pl.ds(d + 16, 8, stride=OPITCH), :] = hi[k]

    scale_b = DHB ** -0.5

    def b_qkv_dots(i, st, n0, n1, hist=True):
        r0 = i * (TB // 2)
        if not isinstance(r0, int):
            r0 = pl.multiple_of(r0, TB // 2)

        def dot(n):
            lhs = _lhs([bxu[j, pl.ds(r0, TB // 2), :] for j in range(NC)])
            y = jnp.dot(lhs, _b16(bw_v[n]), preferred_element_type=f32)
            x_v[st * 24 + n, HALO:HALO + TB, :] = y * scale_b if n < 8 else y
            if n >= 8 and hist:
                x_v[((st + 1) % UB) * 24 + n, 0:HALO, :] = y[TB - HALO:TB]
            return y[TB - 8:TB]
        return [P(dot, n) for n in range(n0, n1)]

    def b_proj_dots(i, st):
        r0 = i * TB
        if not isinstance(r0, int):
            r0 = pl.multiple_of(r0, TB)

        def dot(n):
            lhs = _lhs([obu[st, j] for j in range(NC)])
            w = _b16(jnp.concatenate([bwo_v[n, OPITCH * u:OPITCH * u + 64, :] for u in range(8)], axis=0))
            y = jnp.dot(lhs, w, preferred_element_type=f32)
            outb_v[pl.ds(r0, TB), 128 * n:128 * n + 128] = y.astype(bf16)
            return y[TB - 8:TB]
        return [P(dot, n) for n in range(NC)]

    def rows8(s0, r):
        return x_v[s0:s0 + 8, r:r + 8, :]

    def pos_ok(g, w):
        return lax.broadcasted_iota(i32, (8, 8, 128), 1) + (8 * g) - DIL * w >= 0

    def at_qk(st, g):
        q = rows8(st * 24, HALO + 8 * g)
        p = [jnp.sum(q * rows8(st * 24 + 8, HALO + 8 * g - DIL * w), axis=0) for w in range(WIN)]
        x_v[X_PART + (st % 2) * NG + g, 0:64, :] = jnp.concatenate(p, axis=0)

    def at_softmax(st, g, first, pend):
        p = x_v[X_PART + (st % 2) * NG + g, 0:64, :]
        p = p + pltpu.roll(p, 32, 1)
        p = (p + pltpu.roll(p, 64, 1)).reshape(WIN, 8, 128)
        if first and 8 * g < DIL * (WIN - 1):
            p = jnp.where(pos_ok(g, lax.broadcasted_iota(i32, (8, 8, 128), 0)), p, -1e9)
        e = jnp.exp(p - jnp.max(p, axis=0, keepdims=True))
        l = jnp.sum(e, axis=0, keepdims=True)
        rc = pl.reciprocal(l, approx=True)
        pend[st, g] = e * (rc * (2.0 - l * rc))

    def at_store(st, g, pend):
        x_v[X_PROB + (st % 2) * NG + g, 0:64, :] = pend.pop((st, g)).reshape(64, 128)

    def at_pv(st, g, first):
        acc = None
        for w in range(WIN):
            e = x_v[X_PROB + (st % 2) * NG + g:X_PROB + (st % 2) * NG + g + 1, 8 * w:8 * w + 8, :]
            vv = rows8(st * 24 + 16, HALO + 8 * g - DIL * w)
            if first and 8 * g - DIL * w < 0:
                vv = jnp.where(pos_ok(g, w), vv, x_v[st * 24 + 16:st * 24 + 24, HALO:HALO + 1, :])
            acc = e * vv if acc is None else acc + e * vv
        x_v[X_OUT + (st % 2) * NG + g, 0:64, :] = acc.reshape(64, 128)

    def at_pack(st, g):
        o = [x_v[X_OUT + (st % 2) * NG + k, 0:64, :].reshape(8, 8, 128) for k in (g - 1, g)]
        ob_v[st, :, 8 * g - 8:8 * g + 8, :] = jnp.concatenate(o, axis=1).astype(bf16)

    pend = {}

    def attn_fill(fill, st, first, e_qk, e_pv, head=True, tail=True):
        for g in range(NG):
            if head:
                put(fill, e_qk(g), P(at_qk, st, g))
                put(fill, e_qk(g) + 1, P(at_softmax, st, g, first, pend))
                put(fill, e_qk(g) + 3, P(at_store, st, g, pend))
            if (head and g < NG - 1) or (tail and g == NG - 1):
                put(fill, e_pv(g), P(at_pv, st, g, first))
                if g % 2 == 1:
                    put(fill, e_pv(g) + 1, P(at_pack, st, g))

    def a_relayout(src0, dst0, g):
        src = stgu.at[pl.ds(pl.multiple_of(src0, 256), HW // 2), :]
        dst = wa_v.at[pl.ds(pl.multiple_of(dst0, 8), (H + 1) * PITCH + DM // 4 + 6), :]
        t = src[128 * g:128 * g + 128, :].reshape(4, 4, 8, 128)
        ev, od = pack_pairs(t[:, 0:2], t[:, 2:4])
        for dp in range(4):
            for o in range(2):
                dst[pl.ds(16 * o * PITCH + 4 * g + dp, 8, stride=2 * PITCH), :] = ev[dp, o]
                dst[pl.ds((16 * o + 1) * PITCH + 4 * g + dp, 8, stride=2 * PITCH), :] = od[dp, o]

    def sec(k0, k1, s):
        return [d for k in range(k0, k1) for d in b_qkv_dots(k, k, 8 * s, 8 * s + 8)]

    with _scope("perm_q"):
        x_v[8:24, 0:HALO, :] = jnp.zeros((16, HALO, 128), f32)
        for half in range(2):
            wait(bw_cps(0, half))
            if half == 0:
                start(bw_cps(2, 0) + bw_cps(2, 1) + bwo_cps() + bx_cps(1))
            for k in range(4):
                perm_select(0, half, k)
            for u in range(8):
                perm_gather(0, half, u, 0, 4)
    with _scope("Q01"):
        wait(bx_cps(0))
        run(sec(0, 2, 0), {})
    with _scope("Q2"):
        wait(bw_cps(1, 0))
        fill = {}
        perm_fill(fill, 1, 0, 0, 3, 5)
        run(sec(2, 3, 0), fill)
    with _scope("Q3K0"):
        wait(bw_cps(1, 1))
        start(bx_cps(2) + [aw_cp(0), mem_cp])
        fill = {}
        perm_fill(fill, 1, 1, 0, 3, 5)
        run(sec(3, 4, 0) + sec(0, 1, 1), fill)
    with _scope("K12"):
        wait(bw_cps(2, 0))
        fill = {}
        perm_fill(fill, 2, 0, 0, 6, 10)
        run(sec(1, 3, 1), fill)
    with _scope("K3V012"):
        wait(bw_cps(2, 1))
        fill = {}
        perm_fill(fill, 2, 1, 0, 3, 5)
        attn_fill(fill, 0, True, lambda g: 7 + g, lambda g: 15 + g)
        attn_fill(fill, 1, False, lambda g: 15 + g, lambda g: 23 + g, tail=False)
        run(b_qkv_dots(3, 3, 8, 16, hist=False) + sec(0, 3, 2), fill)
    with _scope("V3"):
        wait(bwo_cps())
        fill = {}
        for n in range(NC):
            put(fill, min(n, 6), P(prep_bwo, n))
        run(sec(3, 4, 2), fill)
        x_v[8:16, 0:HALO, :] = x_v[3 * 24 + 8:3 * 24 + 16, TB:TB + HALO, :]

    def b_body(it, carry):
        with _scope("it"):
            for c in (1, 2):
                @pl.when(it == c)
                def _():
                    wait(bx_cps(c))

            @pl.when(it >= 2)
            def _():
                cw = jnp.maximum(it - 2, 0)
                dst = stg_v.at[pl.ds(pl.multiple_of(STG_AW + cw * HW, HW), HW), :]
                pltpu.make_async_copy(dst, dst, sem.at[SEM_AW + cw]).wait()

            for c in range(1, NIT):
                @pl.when(it == c)
                def _():
                    start(([ob_cp(UB * TB * (c - 2), UB * TB)] if c >= 2 else []) + ([aw_cp(c)] if c < 6 else [])
                          + [awo_cp(c - 1), ax_cp(c - 1)] + ([awo_cp(NC - 1), ax_cp(NC - 1)] if c == 6 else []))
            c = jnp.maximum(it - 2, 0)
            src0 = jnp.where(it == 1, STG_BW // 2, STG_AW // 2 + c * (HW // 2))
            dst0 = (c // 2) * (H * PITCH) + (c % 2) * (DM // 4)
            dots, fill = [], {}
            for k in range(UB):
                i, e0 = UB * it + k, 32 * k
                dots += b_qkv_dots(i, k, 0, 24) + b_proj_dots(i - 4, k)
                attn_fill(fill, (k - 3) % UB, False, None, lambda g: e0 + 2, head=False)
                attn_fill(fill, (k - 2) % UB, False, lambda g: e0 + 4 * g - (1 if 4 * g + e0 == 124 else 0),
                          lambda g: e0 + 4 * g + 6, tail=False)
                for g in range(16):
                    put(fill, min(e0 + 2 * g + 1, 126), P(a_relayout, src0, dst0, 16 * k + g))
            run(dots, fill, relayout=True)
        return carry
    lax.fori_loop(1, NIT, b_body, 0)
    nb = S // TB
    with _scope("tailB"):
        ob_cp(S - 2 * UB * TB, UB * TB).start()
        fill = {}
        attn_fill(fill, 1, False, None, lambda g: 0, head=False)
        attn_fill(fill, 2, False, lambda g: g, lambda g: 4 + g)
        attn_fill(fill, 3, False, lambda g: 8 + g, lambda g: 12 + g)
        run([d for k in range(UB) for d in b_proj_dots(nb - 4 + k, k)], fill)
        ob_cp(S - UB * TB, UB * TB).start()

    wait([awo_cp(n) for n in range(NC)] + [ax_cp(j) for j in range(NC)] + [mem_cp])

    scale_a = DH ** -0.5
    rr = lax.broadcasted_iota(i32, (2 * L, 2 * L), 0)
    cc = lax.broadcasted_iota(i32, (2 * L, 2 * L), 1)
    rb_, cb_ = rr >= L, cc >= L
    ri, ci = jnp.where(rb_, rr - L, rr), jnp.where(cb_, cc - L, cc)
    same = rb_ == cb_
    valid = same & ((ri < M) | (ri >= ci))
    fill = jnp.where(same, -1e9, -jnp.inf).astype(f32)

    mem_s[...] = mem_v[...].astype(f32)
    NP = H // 2

    def a_step(lhs, even):
        qkv, pp = {}, {}
        nrow = 32 if even else 48

        def proj(wh, k0, k1):
            w0 = wh * PITCH
            return jnp.dot(lhs[:, k0:k1], _b16(wa_v[w0 + k0 // 2:w0 + k1 // 2, :]), preferred_element_type=f32)

        def do_qkv(j, after_dot):
            split = j == 0 and not even
            lo = {wi * H + hh: proj(wi * H + hh, 0, DM // 2) for hh in (0, 1) for wi in range(3)} if split else {}
            parts = [[], [], []]
            for hh in (2 * j, 2 * j + 1):
                for wi in range(3):
                    wh = wi * H + hh
                    y = proj(wh, DM // 2, DM) + lo[wh] if split else proj(wh, 0, DM)
                    if even:
                        stash[wh] = y[32:40]
                        parts[wi] += [y[40:48], y[0:32]]
                    else:
                        parts[wi] += [y[0:8], stash[wh], y[8:32]]
                    after_dot(3 * hh + wi)
            qkv[j] = [jnp.concatenate(p, axis=0).astype(bf16) for p in parts]

        def do_qk(j):
            q2, k2, _ = qkv[j]
            s = lax.dot_general(q2, k2, (((1,), (1,)), ((), ())), preferred_element_type=f32) * scale_a
            s = jnp.where(valid, s, fill)
            m = jnp.max(s, axis=1, keepdims=True)
            e = jnp.exp(s - m)
            l = jnp.sum(e, axis=1, keepdims=True)
            rc = pl.reciprocal(l, approx=True)
            rc = rc * (2.0 - l * rc)
            pp[j] = (e * rc).astype(bf16)

        def do_pv(j):
            o2 = jnp.dot(pp.pop(j), qkv.pop(j)[2], preferred_element_type=f32)
            for i, hh in enumerate((2 * j, 2 * j + 1)):
                o = o2[L * i:L * (i + 1)]
                if even:
                    o_s[hh, 0:32, :] = o[0:32].astype(bf16)
                    ostash[hh] = o[32:40]
                else:
                    o_s[hh] = jnp.concatenate([o[0:8], ostash[hh], o[8:40]], axis=0).astype(bf16)

        ya = {}

        def wo_part(n, h0, h1):
            lo = _lhs([osu[hh, 0:nrow // 2, :] for hh in range(h0, h1)])
            r = jnp.dot(lo, _b16(wou[n, h0 * 64:h1 * 64, :]), preferred_element_type=f32)
            ya[n] = r + ya[n] if n in ya else r

        ni = 0 if even else NI
        pieces = [(n, 4 * g, 4 * g + 4) for g in range(ni) for n in range(NC)]
        d0 = 6 * (LPV + 2)
        done = []

        def after_dot(d):
            ready = NC * max(((d + 1) // 6 - LPV - 1 + (1 if (d + 1) % 6 else 0)) // 2, 0)
            while len(done) < min((d - d0 + 1) * len(pieces) // (3 * H - d0), ready):
                wo_part(*pieces[len(done)])
                done.append(0)

        for j in range(NP):
            do_qkv(j, after_dot)
            if j - LQK >= 0:
                do_qk(j - LQK)
            if j - LPV >= 0:
                do_pv(j - LPV)
        assert len(done) == len(pieces)
        nper, n = NC // (LPV + 1), 0
        for j in range(NP, NP + LPV):
            for _ in range(nper):
                wo_part(n, 4 * ni, 2 * KA)
                n += 1
            if j - LQK < NP:
                do_qk(j - LQK)
            do_pv(j - LPV)
        for n in range(n, NC):
            wo_part(n, 4 * ni, 2 * KA)
        for n in range(NC):
            wo_part(n, 2 * KA, H)
        return jnp.concatenate([ya[n] for n in range(NC)], axis=1)

    def a_body(t, c):
        with _scope("a_it"):
            return a_pair(t, c)

    def a_pair(t, c):
        @pl.when(t > 0)
        def _():
            oa_cp(pl.multiple_of(jnp.maximum(t - 1, 0) * 64, 64), 64).start()
        r0 = pl.multiple_of(t * 32, 32)
        X = _lhs([axu[j, pl.ds(r0, 32), :] for j in range(NC)])
        Xm = X[32:48].astype(f32)
        mixed = jnp.concatenate([Xm[0:8], mem_s[...]], axis=0).astype(bf16)
        ye = a_step(jnp.concatenate([X[0:32], mixed], axis=0), True)
        mixed = jnp.concatenate([ye[0:8], Xm[8:16]], axis=0).astype(bf16)
        yo = a_step(jnp.concatenate([mixed, X[48:64]], axis=0), False)
        mem_s[...] = yo[0:8]
        o0 = pl.multiple_of(t * 64, 64)
        outa_v[pl.ds(o0, 64), :] = jnp.concatenate([ye[8:32], yo[8:48]], axis=0).astype(bf16)
        return c
    lax.fori_loop(0, S // 64, a_body, 0)
    oa_cp(S - 64, 64).start()

    ob_cp(0, S).wait()
    oa_cp(0, S).wait()


@jax.jit
def _run(A_x, A_mem0, A_Wq, A_Wk, A_Wv, A_Wo, B_x, B_wqkv, B_wo):
    hbm = pl.BlockSpec(memory_space=pl.ANY)
    out = pl.pallas_call(
        _kernel,
        out_shape=jax.ShapeDtypeStruct((S, 2 * DM), bf16),
        in_specs=[hbm] * 9,
        out_specs=hbm,
        scratch_shapes=[
            pltpu.VMEM((NC, S, 128), bf16),
            pltpu.VMEM((M, DM), bf16),
            pltpu.VMEM((STG_ROWS, 128), bf16),
            pltpu.VMEM((WA_DUM + 8, 128), u32),
            pltpu.VMEM((NC, H * DH, 128), bf16),
            pltpu.VMEM((NC, S, 128), bf16),
            pltpu.VMEM((24, DM // 2, 128), u32),
            pltpu.VMEM((NC, 9 * OPITCH + 4, 128), u32),
            pltpu.VMEM((S, DM), bf16),
            pltpu.VMEM((S, DM), bf16),
            pltpu.VMEM((X_SLABS, TB + HALO, 128), f32),
            pltpu.VMEM((UB, 8, TB, 128), bf16),
            pltpu.VMEM((M, DM), f32),
            pltpu.VMEM((3 * H, 8, DH), f32),
            pltpu.VMEM((H, 8, DH), f32),
            pltpu.VMEM((H, 48, DH), bf16),
            pltpu.SMEM((1,), i32),
            pltpu.SemaphoreType.DMA((NSEM,)),
        ],
        compiler_params=pltpu.CompilerParams(vmem_limit_bytes=110 * 1024 * 1024, disable_bounds_checks=True),
    )(
        A_x.reshape(S, DM), A_mem0.reshape(M, DM),
        A_Wq.reshape(DM * H, DH), A_Wk.reshape(DM * H, DH), A_Wv.reshape(DM * H, DH),
        A_Wo.reshape(H * DH, DM),
        B_x.reshape(S, DM), B_wqkv, B_wo,
    )
    return out.reshape(1, S, 2 * DM)


def pallas_concat_heads__memory_aug_recurrent_mem_tr__sliding_local_dilated__prompt_kernel(
    A_x, A_mem0, A_Wq, A_Wk, A_Wv, A_Wo, A_seg_len, B_x, B_wqkv, B_wo,
):
    if isinstance(A_seg_len, int):
        assert A_seg_len == SEG
    return _run(A_x, A_mem0, A_Wq, A_Wk, A_Wv, A_Wo, B_x, B_wqkv, B_wo)
```

```python
import contextlib
import functools

import jax
import jax.numpy as jnp
from jax import lax
import jax.experimental.pallas as pl
import jax.experimental.pallas.tpu as pltpu

bf16, f32, u32, i32 = jnp.bfloat16, jnp.float32, jnp.uint32, jnp.int32

S, DM = 2048, 1024
H, DH = 32, 128
M, SEG = 8, 32
L = M + SEG
DHB, WIN, DIL = 32, 8, 2
NC = DM // 128

TB = 64
UB = 4
HALO = 16
NIT = S // (TB * UB)
LQK, LPV, KA, NI = 1, 3, 12, 3

PITCH = 9
OPITCH = 65
HW = DM * H // 2
STG_AW, STG_BW, STG_BWO = 0, 6 * HW, 6 * HW + 24 * DM
STG_TOK = STG_BWO + NC * DM
STG_ROWS = STG_TOK + 64
NG = TB // 8
X_PART = UB * 24
X_PROB = X_PART + 2 * NG
X_OUT = X_PROB + 2 * NG
X_TMP = X_OUT + 2 * NG
X_FEN = X_TMP + 32
X_SLABS = X_FEN + 2

SEM_BW, SEM_BX, SEM_BWO, SEM_AW, SEM_AWO, SEM_AX, SEM_MEM, SEM_OB, SEM_OA = 0, 6, 9, 10, 16, 17, 18, 19, 20
NSEM = 21
_SCOPES = False


def _scope(name):
    return jax.named_scope(name) if _SCOPES else contextlib.nullcontext()


def _b16(v):
    return pltpu.bitcast(v, bf16)


def _lhs(blocks):
    return _b16(jnp.concatenate(blocks, axis=1))


def _kernel(ax_h, mem_h, wq_h, wk_h, wv_h, wo_h, bx_h, bw_h, bwo_h, out_h,
            ax_v, mem_v, stg_v, wa_v, wo_v, bx_v, bw_v, bwo_v, outa_v, outb_v,
            x_v, ob_v, mem_s, stash, ostash, o_s, zero_s, sem):
    P = functools.partial

    def bw_cps(s, half):
        return [pltpu.make_async_copy(bw_h.at[pl.ds(half * (DM // 2), DM // 2), pl.ds(128 * n, 128)],
                                      stg_v.at[pl.ds(STG_BW + DM * n + half * (DM // 2), DM // 2), :],
                                      sem.at[SEM_BW + 2 * s + half]) for n in range(8 * s, 8 * s + 8)]

    def bx_cps(part):
        rows = (pl.ds(0, TB * UB), pl.ds(TB * UB, TB * UB), pl.ds(2 * TB * UB, S - 2 * TB * UB))[part]
        return [pltpu.make_async_copy(bx_h.at[rows, pl.ds(128 * j, 128)], bx_v.at[j, rows, :],
                                      sem.at[SEM_BX + part]) for j in range(NC)]

    def bwo_cps():
        return [pltpu.make_async_copy(bwo_h.at[:, pl.ds(128 * n, 128)], stg_v.at[pl.ds(STG_BWO + DM * n, DM), :],
                                      sem.at[SEM_BWO]) for n in range(NC)]

    def aw_cp(c):
        src = (wq_h, wk_h, wv_h)[c // 2]
        return pltpu.make_async_copy(src.at[pl.ds((c % 2) * HW, HW), :], stg_v.at[pl.ds(STG_AW + c * HW, HW), :],
                                     sem.at[SEM_AW + c])

    def awo_cp(n):
        return pltpu.make_async_copy(wo_h.at[:, pl.ds(128 * n, 128)], wo_v.at[n], sem.at[SEM_AWO])

    def ax_cp(j):
        return pltpu.make_async_copy(ax_h.at[:, pl.ds(128 * j, 128)], ax_v.at[j], sem.at[SEM_AX])

    mem_cp = pltpu.make_async_copy(mem_h, mem_v, sem.at[SEM_MEM])

    def ob_cp(r0, n):
        return pltpu.make_async_copy(outb_v.at[pl.ds(r0, n), :], out_h.at[pl.ds(r0, n), pl.ds(DM, DM)],
                                     sem.at[SEM_OB])

    def oa_cp(r0, n):
        return pltpu.make_async_copy(outa_v.at[pl.ds(r0, n), :], out_h.at[pl.ds(r0, n), pl.ds(0, DM)],
                                     sem.at[SEM_OA])

    def start(cps):
        for c in cps:
            c.start()

    def wait(cps):
        for c in cps:
            c.wait()

    start(bw_cps(0, 0) + bw_cps(0, 1) + bx_cps(0) + bw_cps(1, 0) + bw_cps(1, 1))

    bxu, stgu, obu = bx_v.bitcast(u32), stg_v.bitcast(u32), ob_v.bitcast(u32)
    wou, axu, osu = wo_v.bitcast(u32), ax_v.bitcast(u32), o_s.bitcast(u32)

    zero_s[0] = 0

    def run(dots, fill):
        z = pl.multiple_of(zero_s[0], 32)
        for n, d in enumerate(dots):
            y = d()
            if fill.get(n) or fill.get(n - 1):
                x_v[z + X_FEN, 0:8, :] = y
                stgu[pl.ds(z + STG_TOK // 2, 8), :] = pltpu.bitcast(y, u32)
            for f in fill.get(n, []):
                f()
        for n in sorted(fill):
            if n >= len(dots):
                for f in fill[n]:
                    f()

    def put(fill, n, f):
        fill.setdefault(n, []).append(f)

    lane16 = lax.broadcasted_iota(i32, (16, 128), 1)

    def perm_select(s, half, k):
        bits = [((lane16 >> (b + 1)) & 1) == 1 for b in range(3)]
        for r in range(0, 64, 16):
            src = (STG_BW + 8 * s * DM) // 2 + half * 256 + 64 * k + r
            zs = [stgu[src + ((-t) % 8) * (DM // 2):src + ((-t) % 8) * (DM // 2) + 16, :] for t in range(8)]
            for b in range(3):
                zs = [lax.select(bits[b], zs[(t - (1 << b)) % 8], zs[t]) for t in range(8)]
            for u in range(8):
                x_v[X_TMP + 4 * u + k, r:r + 16, :] = pltpu.bitcast(zs[u], f32)

    def perm_gather(s, half, u, k0, k1):
        n = 64 * (k1 - k0)
        lane = lax.broadcasted_iota(i32, (n, 128), 1)
        idx = 32 * ((lane >> 3) & 3) + 16 * (lane >> 6) + 2 * ((u + lane) & 7) + ((lane >> 5) & 1)
        t = pltpu.bitcast(x_v[X_TMP + 4 * u + k0:X_TMP + 4 * u + k1, 0:64, :].reshape(n, 128), u32)
        bw_v[8 * s + u, half * 256 + 64 * k0:half * 256 + 64 * k1, :] = jnp.take_along_axis(t, idx, axis=1)

    def perm_fill(fill, s, half, n0, ns, ng):
        for k in range(4):
            put(fill, n0 + k * ns // 4, P(perm_select, s, half, k))
        g0 = n0 + ns // 4 + 1
        for k in range(16):
            rh, u = k // 8, k % 8
            e = max(g0 + k * ng // 16, n0 + (2 * rh + 1) * ns // 4 + 1)
            put(fill, e, P(perm_gather, s, half, u, 2 * rh, 2 * rh + 2))

    def pack_pairs(a, b):
        return (a & jnp.uint32(0xFFFF)) | (b << 16), (a >> 16) | (b & jnp.uint32(0xFFFF0000))

    def prep_bwo(n):
        for v in range(0, 8, 2):
            r = (STG_BWO + n * DM) // 2 + 64 * v
            a = stgu[r:r + 64, :].reshape(8, 8, 128)
            b = stgu[r + 64:r + 128, :].reshape(8, 8, 128)
            a = pltpu.roll(a, 8 - v, 1) if v else a
            lo, hi = pack_pairs(a, pltpu.roll(b, 7 - v, 1))
            for k in range(8):
                d = 32 * (k % 2) + 4 * (k // 2) + v // 2
                bwo_v[n, pl.ds(d, 8, stride=OPITCH), :] = lo[k]
                bwo_v[n, pl.ds(d + 16, 8, stride=OPITCH), :] = hi[k]

    scale_b = DHB ** -0.5

    def b_qkv_dots(i, st, n0, n1):
        r0 = i * (TB // 2)
        if not isinstance(r0, int):
            r0 = pl.multiple_of(r0, TB // 2)

        def dot(n):
            lhs = _lhs([bxu[j, pl.ds(r0, TB // 2), :] for j in range(NC)])
            y = jnp.dot(lhs, _b16(bw_v[n]), preferred_element_type=f32)
            x_v[st * 24 + n, HALO:HALO + TB, :] = y * scale_b if n < 8 else y
            if n >= 8:
                x_v[((st + 1) % UB) * 24 + n, 0:HALO, :] = y[TB - HALO:TB]
            return y[TB - 8:TB]
        return [P(dot, n) for n in range(n0, n1)]

    def b_proj_dots(i, st):
        r0 = i * TB
        if not isinstance(r0, int):
            r0 = pl.multiple_of(r0, TB)

        def dot(n):
            lhs = _lhs([obu[st, j] for j in range(NC)])
            w = _b16(jnp.concatenate([bwo_v[n, OPITCH * u:OPITCH * u + 64, :] for u in range(8)], axis=0))
            y = jnp.dot(lhs, w, preferred_element_type=f32)
            outb_v[pl.ds(r0, TB), 128 * n:128 * n + 128] = y.astype(bf16)
            return y[TB - 8:TB]
        return [P(dot, n) for n in range(NC)]

    def rows8(s0, r):
        return x_v[s0:s0 + 8, r:r + 8, :]

    def pos_ok(g, w):
        return lax.broadcasted_iota(i32, (8, 8, 128), 1) + (8 * g) - DIL * w >= 0

    def at_qk(st, g, half):
        q = rows8(st * 24, HALO + 8 * g)
        p = [jnp.sum(q * rows8(st * 24 + 8, HALO + 8 * g - DIL * w), axis=0) for w in range(4 * half, 4 * half + 4)]
        x_v[X_PART + (st % 2) * NG + g, 32 * half:32 * half + 32, :] = jnp.concatenate(p, axis=0)

    def at_softmax(st, g, first, pend):
        p = x_v[X_PART + (st % 2) * NG + g, 0:64, :]
        p = p + pltpu.roll(p, 32, 1)
        p = (p + pltpu.roll(p, 64, 1)).reshape(WIN, 8, 128)
        if first and 8 * g < DIL * (WIN - 1):
            p = jnp.where(pos_ok(g, lax.broadcasted_iota(i32, (8, 8, 128), 0)), p, -1e9)
        e = jnp.exp(p - jnp.max(p, axis=0, keepdims=True))
        l = jnp.sum(e, axis=0, keepdims=True)
        rc = pl.reciprocal(l, approx=True)
        pend[st, g] = e * (rc * (2.0 - l * rc))

    def at_store(st, g, pend):
        x_v[X_PROB + (st % 2) * NG + g, 0:64, :] = pend.pop((st, g)).reshape(64, 128)

    def at_pv(st, g, first, half):
        acc = None
        s0 = st * 24 + 16 + 4 * half
        for w in range(WIN):
            e = x_v[X_PROB + (st % 2) * NG + g:X_PROB + (st % 2) * NG + g + 1, 8 * w:8 * w + 8, :]
            r = HALO + 8 * g - DIL * w
            vv = x_v[s0:s0 + 4, r:r + 8, :]
            if first and 8 * g - DIL * w < 0:
                vv = jnp.where(pos_ok(g, w)[0:4], vv, x_v[s0:s0 + 4, HALO:HALO + 1, :])
            acc = e * vv if acc is None else acc + e * vv
        x_v[X_OUT + (st % 2) * NG + g, 32 * half:32 * half + 32, :] = acc.reshape(32, 128)

    def at_pack(st, g):
        o = [x_v[X_OUT + (st % 2) * NG + k, 0:64, :].reshape(8, 8, 128) for k in (g - 1, g)]
        ob_v[st, :, 8 * g - 8:8 * g + 8, :] = jnp.concatenate(o, axis=1).astype(bf16)

    pend = {}

    def attn_fill(fill, st, first, e_qk, e_sm, e_pv, step):
        for g, e in e_qk.items():
            put(fill, e, P(at_qk, st, g, 0))
            put(fill, e + step, P(at_qk, st, g, 1))
        for g, e in e_sm.items():
            put(fill, e, P(at_softmax, st, g, first, pend))
            put(fill, e + 2, P(at_store, st, g, pend))
        for g, e in e_pv.items():
            put(fill, e, P(at_pv, st, g, first, 0))
            put(fill, e + step, P(at_pv, st, g, first, 1))
            if g % 2 == 1:
                put(fill, e + step + 1, P(at_pack, st, g))

    def ramp(e0, per, g0=0, g1=NG):
        return {g: e0 + per * g for g in range(g0, g1)}

    def a_relayout(src0, dst0, g):
        src = stgu.at[pl.ds(pl.multiple_of(src0, 256), HW // 2), :]
        dst = wa_v.at[pl.ds(dst0, DM // 32)]
        t = src[64 * g:64 * g + 64, :].reshape(2, 4, 8, 128)
        ev, od = pack_pairs(t[:, 0:2], t[:, 2:4])
        for dp in range(2):
            r = 2 * (g % 4) + dp
            for o in range(2):
                dst[g // 4, pl.ds(8 * o * PITCH + r, 8, stride=PITCH), :] = ev[dp, o]
                dst[g // 4, pl.ds((16 + 8 * o) * PITCH + r, 8, stride=PITCH), :] = od[dp, o]

    def sec(k0, k1, s):
        return [d for k in range(k0, k1) for d in b_qkv_dots(k, k, 8 * s, 8 * s + 8)]

    with _scope("perm_q"):
        x_v[8:24, 0:HALO, :] = jnp.zeros((16, HALO, 128), f32)
        for half in range(2):
            wait(bw_cps(0, half))
            if half == 0:
                start(bw_cps(2, 0) + bw_cps(2, 1) + bwo_cps() + bx_cps(1))
            for k in range(4):
                perm_select(0, half, k)
            for u in range(8):
                perm_gather(0, half, u, 0, 4)
    with _scope("Q01"):
        wait(bx_cps(0))
        run(sec(0, 2, 0), {})
    with _scope("Q2"):
        wait(bw_cps(1, 0))
        fill = {}
        perm_fill(fill, 1, 0, 0, 3, 5)
        run(sec(2, 3, 0), fill)
    with _scope("Q3K0"):
        wait(bw_cps(1, 1))
        start(bx_cps(2) + [aw_cp(0), mem_cp])
        fill = {}
        perm_fill(fill, 1, 1, 0, 3, 5)
        run(sec(3, 4, 0) + sec(0, 1, 1), fill)
    with _scope("K12"):
        wait(bw_cps(2, 0))
        fill = {}
        perm_fill(fill, 2, 0, 0, 6, 10)
        attn_fill(fill, 0, True, ramp(7, 1), {}, {}, 0)
        run(sec(1, 3, 1), fill)
    with _scope("K3V012"):
        wait(bw_cps(2, 1))
        fill = {}
        perm_fill(fill, 2, 1, 0, 3, 5)
        attn_fill(fill, 0, True, {}, ramp(7, 1), ramp(15, 1), 0)
        attn_fill(fill, 1, False, ramp(7, 1), ramp(15, 1), ramp(23, 1, 0, NG - 1), 0)
        attn_fill(fill, 2, False, {0: 30}, {}, {}, 0)
        run(sec(3, 4, 1) + sec(0, 3, 2), fill)
    with _scope("V3"):
        wait(bwo_cps())
        fill = {}
        for n in range(NC):
            put(fill, min(n, 6), P(prep_bwo, n))
        run(sec(3, 4, 2), fill)

    def b_body(it, carry):
        with _scope("it"):
            for c in (1, 2):
                @pl.when(it == c)
                def _():
                    wait(bx_cps(c))

            @pl.when(it >= 2)
            def _():
                cw = jnp.maximum(it - 2, 0)
                dst = stg_v.at[pl.ds(pl.multiple_of(STG_AW + cw * HW, HW), HW), :]
                pltpu.make_async_copy(dst, dst, sem.at[SEM_AW + cw]).wait()

            for c in range(1, NIT):
                @pl.when(it == c)
                def _():
                    start(([ob_cp(UB * TB * (c - 2), UB * TB)] if c >= 2 else []) + ([aw_cp(c)] if c < 6 else [])
                          + [awo_cp(c - 1), ax_cp(c - 1)] + ([awo_cp(NC - 1), ax_cp(NC - 1)] if c == 6 else []))
            c = jnp.maximum(it - 2, 0)
            src0 = jnp.where(it == 1, STG_BW // 2, STG_AW // 2 + c * (HW // 2))
            dst0 = c * (DM // 32)
            dots, fill = [], {}
            for k in range(UB):
                i, e0 = UB * it + k, 32 * k
                dots += b_qkv_dots(i, k, 0, 24) + b_proj_dots(i - 4, k)
                attn_fill(fill, (k - 3) % UB, False, {}, {}, {NG - 1: e0}, 1)
                attn_fill(fill, (k - 2) % UB, False, ramp(e0 - 2, 4, 1), ramp(e0, 4), ramp(e0 + 4, 4, 0, NG - 1), 1)
                attn_fill(fill, (k - 1) % UB, False, {0: min(e0 + 30, 125)}, {}, {}, 1)
                for g in range(32):
                    put(fill, min(e0 + g, 126), P(a_relayout, src0, dst0, 32 * k + g))
            run(dots, fill)
        return carry
    lax.fori_loop(1, NIT, b_body, 0)
    nb = S // TB
    with _scope("tailB"):
        ob_cp(S - 2 * UB * TB, UB * TB).start()
        fill = {}
        attn_fill(fill, 1, False, {}, {}, {NG - 1: 0}, 1)
        attn_fill(fill, 2, False, ramp(-1, 1, 1), ramp(0, 1), ramp(6, 1), 0)
        attn_fill(fill, 3, False, ramp(7, 1), ramp(8, 1), ramp(14, 1), 0)
        run([d for k in range(UB) for d in b_proj_dots(nb - 4 + k, k)], fill)
        ob_cp(S - UB * TB, UB * TB).start()

    wait([awo_cp(n) for n in range(NC)] + [ax_cp(j) for j in range(NC)] + [mem_cp])

    scale_a = DH ** -0.5
    rr = lax.broadcasted_iota(i32, (2 * L, 2 * L), 0)
    cc = lax.broadcasted_iota(i32, (2 * L, 2 * L), 1)
    rb_, cb_ = rr >= L, cc >= L
    ri, ci = jnp.where(rb_, rr - L, rr), jnp.where(cb_, cc - L, cc)
    same = rb_ == cb_
    valid = same & ((ri < M) | (ri >= ci))
    fill = jnp.where(same, -1e9, -jnp.inf).astype(f32)

    mem_s[...] = mem_v[...].astype(f32)
    NP = H // 2

    def a_step(lhs, even):
        qkv, pp = {}, {}
        nrow = 32 if even else 48

        def proj(wh, k0, k1):
            s0, r = (wh // H) * (DM // 16), ((wh % H) // 2 + (H // 2) * (wh % 2)) * PITCH
            w = wa_v[s0 + k0 // 16:s0 + k1 // 16, r:r + 8, :].reshape((k1 - k0) // 2, 128)
            return jnp.dot(lhs[:, k0:k1], _b16(w), preferred_element_type=f32)

        def do_qkv(j, after_dot):
            split = j == 0 and not even
            lo = {wi * H + hh: proj(wi * H + hh, 0, DM // 2) for hh in (0, 1) for wi in range(3)} if split else {}
            parts = [[], [], []]
            for hh in (2 * j, 2 * j + 1):
                for wi in range(3):
                    wh = wi * H + hh
                    y = proj(wh, DM // 2, DM) + lo[wh] if split else proj(wh, 0, DM)
                    if even:
                        stash[wh] = y[32:40]
                        parts[wi] += [y[40:48], y[0:32]]
                    else:
                        parts[wi] += [y[0:8], stash[wh], y[8:32]]
                    after_dot(3 * hh + wi)
            qkv[j] = [jnp.concatenate(p, axis=0).astype(bf16) for p in parts]

        def do_qk(j):
            q2, k2, _ = qkv[j]
            s = lax.dot_general(q2, k2, (((1,), (1,)), ((), ())), preferred_element_type=f32) * scale_a
            s = jnp.where(valid, s, fill)
            m = jnp.max(s, axis=1, keepdims=True)
            e = jnp.exp(s - m)
            l = jnp.sum(e, axis=1, keepdims=True)
            rc = pl.reciprocal(l, approx=True)
            rc = rc * (2.0 - l * rc)
            pp[j] = (e * rc).astype(bf16)

        def do_pv(j):
            o2 = jnp.dot(pp.pop(j), qkv.pop(j)[2], preferred_element_type=f32)
            for i, hh in enumerate((2 * j, 2 * j + 1)):
                o = o2[L * i:L * (i + 1)]
                if even:
                    o_s[hh, 0:32, :] = o[0:32].astype(bf16)
                    ostash[hh] = o[32:40]
                else:
                    o_s[hh] = jnp.concatenate([o[0:8], ostash[hh], o[8:40]], axis=0).astype(bf16)

        ya = {}

        def wo_part(n, h0, h1):
            lo = _lhs([osu[hh, 0:nrow // 2, :] for hh in range(h0, h1)])
            r = jnp.dot(lo, _b16(wou[n, h0 * 64:h1 * 64, :]), preferred_element_type=f32)
            ya[n] = r + ya[n] if n in ya else r

        ni = 0 if even else NI
        pieces = [(n, 4 * g, 4 * g + 4) for g in range(ni) for n in range(NC)]
        d0 = 6 * (LPV + 2)
        done = []

        def after_dot(d):
            ready = NC * max(((d + 1) // 6 - LPV - 1 + (1 if (d + 1) % 6 else 0)) // 2, 0)
            while len(done) < min((d - d0 + 1) * len(pieces) // (3 * H - d0), ready):
                wo_part(*pieces[len(done)])
                done.append(0)

        for j in range(NP):
            do_qkv(j, after_dot)
            if j - LQK >= 0:
                do_qk(j - LQK)
            if j - LPV >= 0:
                do_pv(j - LPV)
        assert len(done) == len(pieces)
        nper, n = NC // (LPV + 1), 0
        for j in range(NP, NP + LPV):
            for _ in range(nper):
                wo_part(n, 4 * ni, 2 * KA)
                n += 1
            if j - LQK < NP:
                do_qk(j - LQK)
            do_pv(j - LPV)
        for n in range(n, NC):
            wo_part(n, 4 * ni, 2 * KA)
        for n in range(NC):
            wo_part(n, 2 * KA, H)
        return jnp.concatenate([ya[n] for n in range(NC)], axis=1)

    def a_body(t, c):
        with _scope("a_it"):
            return a_pair(t, c)

    def a_pair(t, c):
        @pl.when(t > 0)
        def _():
            oa_cp(pl.multiple_of(jnp.maximum(t - 1, 0) * 64, 64), 64).start()
        r0 = pl.multiple_of(t * 32, 32)
        X = _lhs([axu[j, pl.ds(r0, 32), :] for j in range(NC)])
        Xm = X[32:48].astype(f32)
        mixed = jnp.concatenate([Xm[0:8], mem_s[...]], axis=0).astype(bf16)
        ye = a_step(jnp.concatenate([X[0:32], mixed], axis=0), True)
        mixed = jnp.concatenate([ye[0:8], Xm[8:16]], axis=0).astype(bf16)
        yo = a_step(jnp.concatenate([mixed, X[48:64]], axis=0), False)
        mem_s[...] = yo[0:8]
        o0 = pl.multiple_of(t * 64, 64)
        outa_v[pl.ds(o0, 64), :] = jnp.concatenate([ye[8:32], yo[8:48]], axis=0).astype(bf16)
        return c
    lax.fori_loop(0, S // 64, a_body, 0)
    oa_cp(S - 64, 64).start()

    ob_cp(0, S).wait()
    oa_cp(0, S).wait()


@jax.jit
def _run(A_x, A_mem0, A_Wq, A_Wk, A_Wv, A_Wo, B_x, B_wqkv, B_wo):
    hbm = pl.BlockSpec(memory_space=pl.ANY)
    out = pl.pallas_call(
        _kernel,
        out_shape=jax.ShapeDtypeStruct((S, 2 * DM), bf16),
        in_specs=[hbm] * 9,
        out_specs=hbm,
        scratch_shapes=[
            pltpu.VMEM((NC, S, 128), bf16),
            pltpu.VMEM((M, DM), bf16),
            pltpu.VMEM((STG_ROWS, 128), bf16),
            pltpu.VMEM((3 * DM // 16, H * PITCH + 8, 128), u32),
            pltpu.VMEM((NC, H * DH, 128), bf16),
            pltpu.VMEM((NC, S, 128), bf16),
            pltpu.VMEM((24, DM // 2, 128), u32),
            pltpu.VMEM((NC, 9 * OPITCH - 1, 128), u32),
            pltpu.VMEM((S, DM), bf16),
            pltpu.VMEM((S, DM), bf16),
            pltpu.VMEM((X_SLABS, TB + HALO, 128), f32),
            pltpu.VMEM((UB, 8, TB, 128), bf16),
            pltpu.VMEM((M, DM), f32),
            pltpu.VMEM((3 * H, 8, DH), f32),
            pltpu.VMEM((H, 8, DH), f32),
            pltpu.VMEM((H, 48, DH), bf16),
            pltpu.SMEM((1,), i32),
            pltpu.SemaphoreType.DMA((NSEM,)),
        ],
        compiler_params=pltpu.CompilerParams(vmem_limit_bytes=110 * 1024 * 1024, disable_bounds_checks=True),
    )(
        A_x.reshape(S, DM), A_mem0.reshape(M, DM),
        A_Wq.reshape(DM * H, DH), A_Wk.reshape(DM * H, DH), A_Wv.reshape(DM * H, DH),
        A_Wo.reshape(H * DH, DM),
        B_x.reshape(S, DM), B_wqkv, B_wo,
    )
    return out.reshape(1, S, 2 * DM)


def pallas_concat_heads__memory_aug_recurrent_mem_tr__sliding_local_dilated__prompt_kernel(
    A_x, A_mem0, A_Wq, A_Wk, A_Wv, A_Wo, A_seg_len, B_x, B_wqkv, B_wo,
):
    if isinstance(A_seg_len, int):
        assert A_seg_len == SEG
    return _run(A_x, A_mem0, A_Wq, A_Wk, A_Wv, A_Wo, B_x, B_wqkv, B_wo)
```

```python
import contextlib
import functools

import jax
import jax.numpy as jnp
from jax import lax
import jax.experimental.pallas as pl
import jax.experimental.pallas.tpu as pltpu

bf16, f32, u32, i32 = jnp.bfloat16, jnp.float32, jnp.uint32, jnp.int32

S, DM = 2048, 1024
H, DH = 32, 128
M, SEG = 8, 32
L = M + SEG
DHB, WIN, DIL = 32, 8, 2
NC = DM // 128

TB = 64
UB = 4
HALO = 16
NIT = S // (TB * UB)
LQK, LPV, KA, NI = 1, 3, 12, 3

PITCH = 9
OPITCH = 65
HW = DM * H // 2
STG_AW, STG_BW, STG_BWO = 0, 6 * HW, 6 * HW + 24 * DM
STG_TOK = STG_BWO + NC * DM
STG_ROWS = STG_TOK + 64
NG = TB // 8
X_PART = UB * 24
X_PROB = X_PART + 2 * NG
X_OUT = X_PROB + 2 * NG
X_TMP = X_OUT + 2 * NG
X_FEN = X_TMP + 32
X_SLABS = X_FEN + 2

SEM_BW, SEM_BX, SEM_BWO, SEM_AW, SEM_AWO, SEM_AX, SEM_MEM, SEM_OB, SEM_OA = 0, 6, 9, 10, 16, 17, 18, 19, 20
NSEM = 21
_SCOPES = False


def _scope(name):
    return jax.named_scope(name) if _SCOPES else contextlib.nullcontext()


def _b16(v):
    return pltpu.bitcast(v, bf16)


def _lhs(blocks):
    return _b16(jnp.concatenate(blocks, axis=1))


def _kernel(ax_h, mem_h, wq_h, wk_h, wv_h, wo_h, bx_h, bw_h, bwo_h, out_h,
            ax_v, mem_v, stg_v, wa_v, wo_v, bx_v, bw_v, bwo_v, outa_v, outb_v,
            x_v, ob_v, mem_s, stash, ostash, o_s, zero_s, sem):
    P = functools.partial

    def bw_cps(s, half):
        return [pltpu.make_async_copy(bw_h.at[pl.ds(half * (DM // 2), DM // 2), pl.ds(128 * n, 128)],
                                      stg_v.at[pl.ds(STG_BW + DM * n + half * (DM // 2), DM // 2), :],
                                      sem.at[SEM_BW + 2 * s + half]) for n in range(8 * s, 8 * s + 8)]

    def bx_cps(part):
        rows = (pl.ds(0, TB * UB), pl.ds(TB * UB, TB * UB), pl.ds(2 * TB * UB, S - 2 * TB * UB))[part]
        return [pltpu.make_async_copy(bx_h.at[rows, pl.ds(128 * j, 128)], bx_v.at[j, rows, :],
                                      sem.at[SEM_BX + part]) for j in range(NC)]

    def bwo_cps():
        return [pltpu.make_async_copy(bwo_h.at[:, pl.ds(128 * n, 128)], stg_v.at[pl.ds(STG_BWO + DM * n, DM), :],
                                      sem.at[SEM_BWO]) for n in range(NC)]

    def aw_cp(c):
        src = (wq_h, wk_h, wv_h)[c // 2]
        return pltpu.make_async_copy(src.at[pl.ds((c % 2) * HW, HW), :], stg_v.at[pl.ds(STG_AW + c * HW, HW), :],
                                     sem.at[SEM_AW + c])

    def awo_cp(n):
        return pltpu.make_async_copy(wo_h.at[:, pl.ds(128 * n, 128)], wo_v.at[n], sem.at[SEM_AWO])

    def ax_cp(j):
        return pltpu.make_async_copy(ax_h.at[:, pl.ds(128 * j, 128)], ax_v.at[j], sem.at[SEM_AX])

    mem_cp = pltpu.make_async_copy(mem_h, mem_v, sem.at[SEM_MEM])

    def ob_cp(r0, n):
        return pltpu.make_async_copy(outb_v.at[pl.ds(r0, n), :], out_h.at[pl.ds(r0, n), pl.ds(DM, DM)],
                                     sem.at[SEM_OB])

    def oa_cp(r0, n):
        return pltpu.make_async_copy(outa_v.at[pl.ds(r0, n), :], out_h.at[pl.ds(r0, n), pl.ds(0, DM)],
                                     sem.at[SEM_OA])

    def start(cps):
        for c in cps:
            c.start()

    def wait(cps):
        for c in cps:
            c.wait()

    start(bw_cps(0, 0) + bw_cps(0, 1) + bx_cps(0) + bw_cps(1, 0) + bw_cps(1, 1))

    bxu, stgu, obu = bx_v.bitcast(u32), stg_v.bitcast(u32), ob_v.bitcast(u32)
    wou, axu, osu = wo_v.bitcast(u32), ax_v.bitcast(u32), o_s.bitcast(u32)

    zero_s[0] = 0
    x_v[X_FEN + 1, 0:8, :] = jnp.zeros((8, 128), f32)

    def run(dots, fill):
        z = pl.multiple_of(zero_s[0], 32)
        for n, d in enumerate(dots):
            y = d()
            if fill.get(n) or fill.get(n - 1):
                x_v[z + X_FEN, 0:8, :] = y
                stgu[pl.ds(z + STG_TOK // 2, 8), :] = pltpu.bitcast(x_v[X_FEN + 1, 0:8, :], u32)
            for f in fill.get(n, []):
                f()
        for n in sorted(fill):
            if n >= len(dots):
                for f in fill[n]:
                    f()

    def put(fill, n, f):
        fill.setdefault(n, []).append(f)

    lane16 = lax.broadcasted_iota(i32, (16, 128), 1)

    def perm_select(s, half, k):
        bits = [((lane16 >> (b + 1)) & 1) == 1 for b in range(3)]
        for r in range(0, 64, 16):
            src = (STG_BW + 8 * s * DM) // 2 + half * 256 + 64 * k + r
            zs = [stgu[src + ((-t) % 8) * (DM // 2):src + ((-t) % 8) * (DM // 2) + 16, :] for t in range(8)]
            for b in range(3):
                zs = [lax.select(bits[b], zs[(t - (1 << b)) % 8], zs[t]) for t in range(8)]
            for u in range(8):
                x_v[X_TMP + 4 * u + k, r:r + 16, :] = pltpu.bitcast(zs[u], f32)

    def perm_gather(s, half, u, k0, k1):
        n = 64 * (k1 - k0)
        lane = lax.broadcasted_iota(i32, (n, 128), 1)
        idx = 32 * ((lane >> 3) & 3) + 16 * (lane >> 6) + 2 * ((u + lane) & 7) + ((lane >> 5) & 1)
        t = pltpu.bitcast(x_v[X_TMP + 4 * u + k0:X_TMP + 4 * u + k1, 0:64, :].reshape(n, 128), u32)
        bw_v[8 * s + u, half * 256 + 64 * k0:half * 256 + 64 * k1, :] = jnp.take_along_axis(t, idx, axis=1)

    def perm_fill(fill, s, half, n0, ns, ng):
        for k in range(4):
            put(fill, n0 + k * ns // 4, P(perm_select, s, half, k))
        g0 = n0 + ns // 4 + 1
        for k in range(16):
            rh, u = k // 8, k % 8
            e = max(g0 + k * ng // 16, n0 + (2 * rh + 1) * ns // 4 + 1)
            put(fill, e, P(perm_gather, s, half, u, 2 * rh, 2 * rh + 2))

    def pack_pairs(a, b):
        return (a & jnp.uint32(0xFFFF)) | (b << 16), (a >> 16) | (b & jnp.uint32(0xFFFF0000))

    def prep_bwo(n, v):
        r = (STG_BWO + n * DM) // 2 + 64 * v
        a = stgu[r:r + 64, :].reshape(8, 8, 128)
        b = stgu[r + 64:r + 128, :].reshape(8, 8, 128)
        a = pltpu.roll(a, 8 - v, 1) if v else a
        lo, hi = pack_pairs(a, pltpu.roll(b, 7 - v, 1))
        for k in range(8):
            d = 32 * (k % 2) + 4 * (k // 2) + v // 2
            bwo_v[n, pl.ds(d, 8, stride=OPITCH), :] = lo[k]
            bwo_v[n, pl.ds(d + 16, 8, stride=OPITCH), :] = hi[k]

    scale_b = DHB ** -0.5

    def b_qkv_dots(i, st, n0, n1):
        r0 = i * (TB // 2)
        if not isinstance(r0, int):
            r0 = pl.multiple_of(r0, TB // 2)

        def dot(n):
            lhs = _lhs([bxu[j, pl.ds(r0, TB // 2), :] for j in range(NC)])
            y = jnp.dot(lhs, _b16(bw_v[n]), preferred_element_type=f32)
            x_v[st * 24 + n, HALO:HALO + TB, :] = y * scale_b if n < 8 else y
            if n >= 8:
                x_v[((st + 1) % UB) * 24 + n, 0:HALO, :] = y[TB - HALO:TB]
            return y[TB - 8:TB]
        return [P(dot, n) for n in range(n0, n1)]

    def b_proj_dots(i, st):
        r0 = i * TB
        if not isinstance(r0, int):
            r0 = pl.multiple_of(r0, TB)

        def dot(n):
            lhs = _lhs([obu[st, j] for j in range(NC)])
            w = _b16(jnp.concatenate([bwo_v[n, OPITCH * u:OPITCH * u + 64, :] for u in range(8)], axis=0))
            y = jnp.dot(lhs, w, preferred_element_type=f32)
            outb_v[pl.ds(r0, TB), 128 * n:128 * n + 128] = y.astype(bf16)
            return y[TB - 8:TB]
        return [P(dot, n) for n in range(NC)]

    def rows8(s0, r):
        return x_v[s0:s0 + 8, r:r + 8, :]

    def pos_ok(g, w):
        return lax.broadcasted_iota(i32, (8, 8, 128), 1) + (8 * g) - DIL * w >= 0

    def at_qk(st, g, half):
        q = rows8(st * 24, HALO + 8 * g)
        p = [jnp.sum(q * rows8(st * 24 + 8, HALO + 8 * g - DIL * w), axis=0) for w in range(4 * half, 4 * half + 4)]
        x_v[X_PART + (st % 2) * NG + g, 32 * half:32 * half + 32, :] = jnp.concatenate(p, axis=0)

    def at_softmax(st, g, first, pend):
        p = x_v[X_PART + (st % 2) * NG + g, 0:64, :]
        p = p + pltpu.roll(p, 32, 1)
        p = (p + pltpu.roll(p, 64, 1)).reshape(WIN, 8, 128)
        if first and 8 * g < DIL * (WIN - 1):
            p = jnp.where(pos_ok(g, lax.broadcasted_iota(i32, (8, 8, 128), 0)), p, -1e9)
        e = jnp.exp(p - jnp.max(p, axis=0, keepdims=True))
        l = jnp.sum(e, axis=0, keepdims=True)
        rc = pl.reciprocal(l, approx=True)
        pend[st, g] = e * (rc * (2.0 - l * rc))

    def at_store(st, g, pend):
        x_v[X_PROB + (st % 2) * NG + g, 0:64, :] = pend.pop((st, g)).reshape(64, 128)

    def at_pv(st, g, first, half):
        acc = None
        s0 = st * 24 + 16 + 4 * half
        for w in range(WIN):
            e = x_v[X_PROB + (st % 2) * NG + g:X_PROB + (st % 2) * NG + g + 1, 8 * w:8 * w + 8, :]
            r = HALO + 8 * g - DIL * w
            vv = x_v[s0:s0 + 4, r:r + 8, :]
            if first and 8 * g - DIL * w < 0:
                vv = jnp.where(pos_ok(g, w)[0:4], vv, x_v[s0:s0 + 4, HALO:HALO + 1, :])
            acc = e * vv if acc is None else acc + e * vv
        x_v[X_OUT + (st % 2) * NG + g, 32 * half:32 * half + 32, :] = acc.reshape(32, 128)

    def at_pack(st, g):
        o = [x_v[X_OUT + (st % 2) * NG + k, 0:64, :].reshape(8, 8, 128) for k in (g - 1, g)]
        ob_v[st, :, 8 * g - 8:8 * g + 8, :] = jnp.concatenate(o, axis=1).astype(bf16)

    pend = {}

    def attn_fill(fill, st, first, e_qk, e_sm, e_pv, step):
        for g, e in e_qk.items():
            put(fill, e, P(at_qk, st, g, 0))
            put(fill, e + step, P(at_qk, st, g, 1))
        for g, e in e_sm.items():
            put(fill, e, P(at_softmax, st, g, first, pend))
            put(fill, e + 2, P(at_store, st, g, pend))
        for g, e in e_pv.items():
            put(fill, e, P(at_pv, st, g, first, 0))
            put(fill, e + step, P(at_pv, st, g, first, 1))
            if g % 2 == 1:
                put(fill, e + step + 1, P(at_pack, st, g))

    def ramp(e0, per, g0=0, g1=NG):
        return {g: e0 + per * g for g in range(g0, g1)}

    def a_relayout(src0, dst0, g):
        src = stgu.at[pl.ds(pl.multiple_of(src0, 256), HW // 2), :]
        dst = wa_v.at[pl.ds(dst0, DM // 32)]
        t = src[64 * g:64 * g + 64, :].reshape(2, 4, 8, 128)
        ev, od = pack_pairs(t[:, 0:2], t[:, 2:4])
        for dp in range(2):
            r = 2 * (g % 4) + dp
            for o in range(2):
                dst[g // 4, pl.ds(8 * o * PITCH + r, 8, stride=PITCH), :] = ev[dp, o]
                dst[g // 4, pl.ds((16 + 8 * o) * PITCH + r, 8, stride=PITCH), :] = od[dp, o]

    def sec(k0, k1, s):
        return [d for k in range(k0, k1) for d in b_qkv_dots(k, k, 8 * s, 8 * s + 8)]

    with _scope("perm_q"):
        x_v[8:24, 0:HALO, :] = jnp.zeros((16, HALO, 128), f32)
        for half in range(2):
            wait(bw_cps(0, half))
            if half == 0:
                start(bw_cps(2, 0) + bw_cps(2, 1) + bwo_cps() + bx_cps(1))
            for k in range(4):
                perm_select(0, half, k)
            for u in range(8):
                perm_gather(0, half, u, 0, 4)
    with _scope("Q01"):
        wait(bx_cps(0))
        run(sec(0, 2, 0), {})
    with _scope("Q2"):
        wait(bw_cps(1, 0))
        fill = {}
        perm_fill(fill, 1, 0, 0, 3, 5)
        run(sec(2, 3, 0), fill)
    with _scope("Q3K0"):
        wait(bw_cps(1, 1))
        start(bx_cps(2) + [aw_cp(0), mem_cp])
        fill = {}
        perm_fill(fill, 1, 1, 0, 3, 5)
        run(sec(3, 4, 0) + sec(0, 1, 1), fill)
    with _scope("K12"):
        wait(bw_cps(2, 0))
        fill = {}
        perm_fill(fill, 2, 0, 0, 6, 10)
        attn_fill(fill, 0, True, ramp(7, 1), {}, {}, 0)
        run(sec(1, 3, 1), fill)
    with _scope("K3V01"):
        wait(bw_cps(2, 1))
        fill = {}
        perm_fill(fill, 2, 1, 0, 3, 5)
        attn_fill(fill, 0, True, {}, ramp(6, 1), ramp(15, 1, 0, NG - 1), 0)
        attn_fill(fill, 1, False, ramp(7, 1), ramp(14, 1, 0, NG - 1), {}, 0)
        run(sec(3, 4, 1) + sec(0, 2, 2), fill)
    with _scope("V23"):
        wait(bwo_cps())
        fill = {}
        attn_fill(fill, 0, True, {}, {}, {NG - 1: 0}, 0)
        attn_fill(fill, 1, False, {}, {NG - 1: 0}, ramp(1, 2, 0, NG - 1), 1)
        attn_fill(fill, 2, False, {0: 0}, {}, {}, 1)
        for n in range(4 * NC):
            put(fill, n * 15 // 32, P(prep_bwo, n // 4, 2 * (n % 4)))
        run(sec(2, 4, 2), fill)

    def b_body(it, carry):
        with _scope("it"):
            for c in (1, 2):
                @pl.when(it == c)
                def _():
                    wait(bx_cps(c))

            @pl.when(it >= 2)
            def _():
                cw = jnp.maximum(it - 2, 0)
                dst = stg_v.at[pl.ds(pl.multiple_of(STG_AW + cw * HW, HW), HW), :]
                pltpu.make_async_copy(dst, dst, sem.at[SEM_AW + cw]).wait()

            for c in range(1, NIT):
                @pl.when(it == c)
                def _():
                    cols = {6: (5, 6, 7), 7: ()}.get(c, (c - 1,))
                    start(([ob_cp(UB * TB * (c - 2), UB * TB)] if c >= 2 else []) + ([aw_cp(c)] if c < 6 else [])
                          + [cp(n) for n in cols for cp in (awo_cp, ax_cp)])
            c = jnp.maximum(it - 2, 0)
            src0 = jnp.where(it == 1, STG_BW // 2, STG_AW // 2 + c * (HW // 2))
            dst0 = c * (DM // 32)
            dots, fill = [], {}
            for k in range(UB):
                i, e0 = UB * it + k, 32 * k
                dots += b_qkv_dots(i, k, 0, 24) + b_proj_dots(i - 4, k)
                attn_fill(fill, (k - 3) % UB, False, {}, {}, {NG - 1: e0}, 1)
                attn_fill(fill, (k - 2) % UB, False, ramp(e0 - 2, 4, 1), ramp(e0, 4), ramp(e0 + 4, 4, 0, NG - 1), 1)
                attn_fill(fill, (k - 1) % UB, False, {0: min(e0 + 30, 125)}, {}, {}, 1)
                for g in range(32):
                    put(fill, min(e0 + g, 126), P(a_relayout, src0, dst0, 32 * k + g))
            run(dots, fill)
        return carry
    lax.fori_loop(1, NIT, b_body, 0)
    nb = S // TB
    wait([awo_cp(n) for n in range(NC)] + [ax_cp(j) for j in range(NC)] + [mem_cp])
    with _scope("tailB"):
        ob_cp(S - 2 * UB * TB, UB * TB).start()
        fill = {}
        attn_fill(fill, 1, False, {}, {}, {NG - 1: 0}, 1)
        attn_fill(fill, 2, False, ramp(-1, 1, 1), ramp(0, 1), ramp(6, 1), 0)
        attn_fill(fill, 3, False, ramp(7, 1), ramp(8, 1), ramp(14, 1), 0)
        run([d for k in range(UB) for d in b_proj_dots(nb - 4 + k, k)], fill)
        ob_cp(S - UB * TB, UB * TB).start()


    scale_a = DH ** -0.5
    rr = lax.broadcasted_iota(i32, (2 * L, 2 * L), 0)
    cc = lax.broadcasted_iota(i32, (2 * L, 2 * L), 1)
    rb_, cb_ = rr >= L, cc >= L
    ri, ci = jnp.where(rb_, rr - L, rr), jnp.where(cb_, cc - L, cc)
    same = rb_ == cb_
    valid = same & ((ri < M) | (ri >= ci))
    fill = jnp.where(same, -1e9, -jnp.inf).astype(f32)

    mem_s[...] = mem_v[...].astype(f32)
    NP = H // 2

    def a_step(lhs, even):
        qkv, pp = {}, {}
        nrow = 32 if even else 48

        def proj(wh, k0, k1):
            s0, r = (wh // H) * (DM // 16), ((wh % H) // 2 + (H // 2) * (wh % 2)) * PITCH
            w = wa_v[s0 + k0 // 16:s0 + k1 // 16, r:r + 8, :].reshape((k1 - k0) // 2, 128)
            return jnp.dot(lhs[:, k0:k1], _b16(w), preferred_element_type=f32)

        def do_qkv(j, after_dot):
            split = j == 0 and not even
            lo = {wi * H + hh: proj(wi * H + hh, 0, DM // 2) for hh in (0, 1) for wi in range(3)} if split else {}
            parts = [[], [], []]
            for hh in (2 * j, 2 * j + 1):
                for wi in range(3):
                    wh = wi * H + hh
                    y = proj(wh, DM // 2, DM) + lo[wh] if split else proj(wh, 0, DM)
                    if even:
                        stash[wh] = y[32:40]
                        parts[wi] += [y[40:48], y[0:32]]
                    else:
                        parts[wi] += [y[0:8], stash[wh], y[8:32]]
                    after_dot(3 * hh + wi)
            qkv[j] = [jnp.concatenate(p, axis=0).astype(bf16) for p in parts]

        def do_qk(j):
            q2, k2, _ = qkv[j]
            s = lax.dot_general(q2, k2, (((1,), (1,)), ((), ())), preferred_element_type=f32) * scale_a
            s = jnp.where(valid, s, fill)
            m = jnp.max(s, axis=1, keepdims=True)
            e = jnp.exp(s - m)
            l = jnp.sum(e, axis=1, keepdims=True)
            rc = pl.reciprocal(l, approx=True)
            rc = rc * (2.0 - l * rc)
            pp[j] = (e * rc).astype(bf16)

        def do_pv(j):
            o2 = jnp.dot(pp.pop(j), qkv.pop(j)[2], preferred_element_type=f32)
            for i, hh in enumerate((2 * j, 2 * j + 1)):
                o = o2[L * i:L * (i + 1)]
                if even:
                    o_s[hh, 0:32, :] = o[0:32].astype(bf16)
                    ostash[hh] = o[32:40]
                else:
                    o_s[hh] = jnp.concatenate([o[0:8], ostash[hh], o[8:40]], axis=0).astype(bf16)

        ya = {}

        def wo_part(n, h0, h1):
            lo = _lhs([osu[hh, 0:nrow // 2, :] for hh in range(h0, h1)])
            r = jnp.dot(lo, _b16(wou[n, h0 * 64:h1 * 64, :]), preferred_element_type=f32)
            ya[n] = r + ya[n] if n in ya else r

        ni = 0 if even else NI
        pieces = [(n, 4 * g, 4 * g + 4) for g in range(ni) for n in range(NC)]
        d0 = 6 * (LPV + 2)
        done = []

        def after_dot(d):
            ready = NC * max(((d + 1) // 6 - LPV - 1 + (1 if (d + 1) % 6 else 0)) // 2, 0)
            while len(done) < min((d - d0 + 1) * len(pieces) // (3 * H - d0), ready):
                wo_part(*pieces[len(done)])
                done.append(0)

        for j in range(NP):
            do_qkv(j, after_dot)
            if j - LQK >= 0:
                do_qk(j - LQK)
            if j - LPV >= 0:
                do_pv(j - LPV)
        assert len(done) == len(pieces)
        nper, n = NC // (LPV + 1), 0
        for j in range(NP, NP + LPV):
            for _ in range(nper):
                wo_part(n, 4 * ni, 2 * KA)
                n += 1
            if j - LQK < NP:
                do_qk(j - LQK)
            do_pv(j - LPV)
        for n in range(n, NC):
            wo_part(n, 4 * ni, 2 * KA)
        for n in range(NC):
            wo_part(n, 2 * KA, H)
        return jnp.concatenate([ya[n] for n in range(NC)], axis=1)

    def a_body(t, c):
        with _scope("a_it"):
            return a_pair(t, c)

    def a_pair(t, c):
        @pl.when(t > 0)
        def _():
            oa_cp(pl.multiple_of(jnp.maximum(t - 1, 0) * 64, 64), 64).start()
        r0 = pl.multiple_of(t * 32, 32)
        X = _lhs([axu[j, pl.ds(r0, 32), :] for j in range(NC)])
        Xm = X[32:48].astype(f32)
        mixed = jnp.concatenate([Xm[0:8], mem_s[...]], axis=0).astype(bf16)
        ye = a_step(jnp.concatenate([X[0:32], mixed], axis=0), True)
        mixed = jnp.concatenate([ye[0:8], Xm[8:16]], axis=0).astype(bf16)
        yo = a_step(jnp.concatenate([mixed, X[48:64]], axis=0), False)
        mem_s[...] = yo[0:8]
        o0 = pl.multiple_of(t * 64, 64)
        outa_v[pl.ds(o0, 64), :] = jnp.concatenate([ye[8:32], yo[8:48]], axis=0).astype(bf16)
        return c
    lax.fori_loop(0, S // 64, a_body, 0)
    oa_cp(S - 64, 64).start()

    ob_cp(0, S).wait()
    oa_cp(0, S).wait()


@jax.jit
def _run(A_x, A_mem0, A_Wq, A_Wk, A_Wv, A_Wo, B_x, B_wqkv, B_wo):
    hbm = pl.BlockSpec(memory_space=pl.ANY)
    out = pl.pallas_call(
        _kernel,
        out_shape=jax.ShapeDtypeStruct((S, 2 * DM), bf16),
        in_specs=[hbm] * 9,
        out_specs=hbm,
        scratch_shapes=[
            pltpu.VMEM((NC, S, 128), bf16),
            pltpu.VMEM((M, DM), bf16),
            pltpu.VMEM((STG_ROWS, 128), bf16),
            pltpu.VMEM((3 * DM // 16, H * PITCH + 8, 128), u32),
            pltpu.VMEM((NC, H * DH, 128), bf16),
            pltpu.VMEM((NC, S, 128), bf16),
            pltpu.VMEM((24, DM // 2, 128), u32),
            pltpu.VMEM((NC, 9 * OPITCH - 1, 128), u32),
            pltpu.VMEM((S, DM), bf16),
            pltpu.VMEM((S, DM), bf16),
            pltpu.VMEM((X_SLABS, TB + HALO, 128), f32),
            pltpu.VMEM((UB, 8, TB, 128), bf16),
            pltpu.VMEM((M, DM), f32),
            pltpu.VMEM((3 * H, 8, DH), f32),
            pltpu.VMEM((H, 8, DH), f32),
            pltpu.VMEM((H, 48, DH), bf16),
            pltpu.SMEM((1,), i32),
            pltpu.SemaphoreType.DMA((NSEM,)),
        ],
        compiler_params=pltpu.CompilerParams(vmem_limit_bytes=110 * 1024 * 1024, disable_bounds_checks=True),
    )(
        A_x.reshape(S, DM), A_mem0.reshape(M, DM),
        A_Wq.reshape(DM * H, DH), A_Wk.reshape(DM * H, DH), A_Wv.reshape(DM * H, DH),
        A_Wo.reshape(H * DH, DM),
        B_x.reshape(S, DM), B_wqkv, B_wo,
    )
    return out.reshape(1, S, 2 * DM)


def pallas_concat_heads__memory_aug_recurrent_mem_tr__sliding_local_dilated__prompt_kernel(
    A_x, A_mem0, A_Wq, A_Wk, A_Wv, A_Wo, A_seg_len, B_x, B_wqkv, B_wo,
):
    if isinstance(A_seg_len, int):
        assert A_seg_len == SEG
    return _run(A_x, A_mem0, A_Wq, A_Wk, A_Wv, A_Wo, B_x, B_wqkv, B_wo)
```

```python
import contextlib
import functools

import jax
import jax.numpy as jnp
from jax import lax
import jax.experimental.pallas as pl
import jax.experimental.pallas.tpu as pltpu

bf16, f32, u32, i32 = jnp.bfloat16, jnp.float32, jnp.uint32, jnp.int32

S, DM = 2048, 1024
H, DH = 32, 128
M, SEG = 8, 32
L = M + SEG
DHB, WIN, DIL = 32, 8, 2
NC = DM // 128

TB = 64
UB = 4
HALO = 16
NIT = S // (TB * UB)
LQK, LPV, KA, NI = 1, 3, 12, 3

PITCH = 9
OPITCH = 65
HW = DM * H // 2
STG_AW, STG_BW, STG_BWO = 0, 6 * HW, 6 * HW + 24 * DM
STG_TOK = STG_BWO + NC * DM
STG_ROWS = STG_TOK + 64
NG = TB // 8
X_PART = UB * 24
X_PROB = X_PART + 2 * NG
X_OUT = X_PROB + 2 * NG
X_TMP = X_OUT + 2 * NG
X_FEN = X_TMP + 32
X_SLABS = X_FEN + 2

SEM_BW, SEM_BX, SEM_BWO, SEM_AW, SEM_AWO, SEM_AX, SEM_MEM, SEM_OB, SEM_OA = 0, 6, 9, 10, 16, 17, 18, 19, 20
NSEM = 21
_SCOPES = False


def _scope(name):
    return jax.named_scope(name) if _SCOPES else contextlib.nullcontext()


def _b16(v):
    return pltpu.bitcast(v, bf16)


def _lhs(blocks):
    return _b16(jnp.concatenate(blocks, axis=1))


def _kernel(ax_h, mem_h, wq_h, wk_h, wv_h, wo_h, bx_h, bw_h, bwo_h, out_h,
            ax_v, mem_v, stg_v, wa_v, wo_v, bx_v, bw_v, bwo_v, outa_v, outb_v,
            x_v, ob_v, mem_s, stash, ostash, o_s, zero_s, sem):
    P = functools.partial

    def bw_cps(s, half):
        return [pltpu.make_async_copy(bw_h.at[pl.ds(half * (DM // 2), DM // 2), pl.ds(128 * n, 128)],
                                      stg_v.at[pl.ds(STG_BW + DM * n + half * (DM // 2), DM // 2), :],
                                      sem.at[SEM_BW + 2 * s + half]) for n in range(8 * s, 8 * s + 8)]

    def bx_cps(part):
        rows = (pl.ds(0, TB * UB), pl.ds(TB * UB, TB * UB), pl.ds(2 * TB * UB, S - 2 * TB * UB))[part]
        return [pltpu.make_async_copy(bx_h.at[rows, pl.ds(128 * j, 128)], bx_v.at[j, rows, :],
                                      sem.at[SEM_BX + part]) for j in range(NC)]

    def bwo_cps():
        return [pltpu.make_async_copy(bwo_h.at[:, pl.ds(128 * n, 128)], stg_v.at[pl.ds(STG_BWO + DM * n, DM), :],
                                      sem.at[SEM_BWO]) for n in range(NC)]

    def aw_cp(c):
        src = (wq_h, wk_h, wv_h)[c // 2]
        return pltpu.make_async_copy(src.at[pl.ds((c % 2) * HW, HW), :], stg_v.at[pl.ds(STG_AW + c * HW, HW), :],
                                     sem.at[SEM_AW + c])

    def awo_cp(n):
        return pltpu.make_async_copy(wo_h.at[:, pl.ds(128 * n, 128)], wo_v.at[n], sem.at[SEM_AWO])

    def ax_cp(j):
        return pltpu.make_async_copy(ax_h.at[:, pl.ds(128 * j, 128)], ax_v.at[j], sem.at[SEM_AX])

    mem_cp = pltpu.make_async_copy(mem_h, mem_v, sem.at[SEM_MEM])

    def ob_cp(r0, n):
        return pltpu.make_async_copy(outb_v.at[pl.ds(r0, n), :], out_h.at[pl.ds(r0, n), pl.ds(DM, DM)],
                                     sem.at[SEM_OB])

    def oa_cp(r0, n):
        return pltpu.make_async_copy(outa_v.at[pl.ds(r0, n), :], out_h.at[pl.ds(r0, n), pl.ds(0, DM)],
                                     sem.at[SEM_OA])

    def start(cps):
        for c in cps:
            c.start()

    def wait(cps):
        for c in cps:
            c.wait()

    start(bw_cps(0, 0) + bw_cps(0, 1) + bx_cps(0) + bw_cps(1, 0) + bw_cps(1, 1))

    bxu, stgu, obu = bx_v.bitcast(u32), stg_v.bitcast(u32), ob_v.bitcast(u32)
    wou, axu, osu = wo_v.bitcast(u32), ax_v.bitcast(u32), o_s.bitcast(u32)

    zero_s[0] = 0
    x_v[X_FEN + 1, 0:8, :] = jnp.zeros((8, 128), f32)

    def run(dots, fill):
        z = pl.multiple_of(zero_s[0], 32)
        busy = [False]

        def epoch(e, y, close):
            if y is not None and (e in fill or (close and busy[0])):
                x_v[z + X_FEN, 0:8, :] = y
                stgu[pl.ds(z + STG_TOK // 2, 8), :] = pltpu.bitcast(x_v[X_FEN + 1, 0:8, :], u32)
                busy[0] = False
            for f in fill.pop(e, []):
                f()
                busy[0] = True

        epoch(-1, None, False)
        for n, d in enumerate(dots):
            y, store = d()
            epoch(n - 0.5, y[0:8], False)
            store()
            epoch(n, y[TB - 8:TB], True)
        assert not fill, sorted(fill)

    def put(fill, n, f):
        fill.setdefault(n, []).append(f)

    lane16 = lax.broadcasted_iota(i32, (16, 128), 1)

    def perm_select(s, half, k):
        bits = [((lane16 >> (b + 1)) & 1) == 1 for b in range(3)]
        for r in range(0, 64, 16):
            src = (STG_BW + 8 * s * DM) // 2 + half * 256 + 64 * k + r
            zs = [stgu[src + ((-t) % 8) * (DM // 2):src + ((-t) % 8) * (DM // 2) + 16, :] for t in range(8)]
            for b in range(3):
                zs = [lax.select(bits[b], zs[(t - (1 << b)) % 8], zs[t]) for t in range(8)]
            for u in range(8):
                x_v[X_TMP + 4 * u + k, r:r + 16, :] = pltpu.bitcast(zs[u], f32)

    def perm_gather(s, half, u, k0, k1):
        n = 64 * (k1 - k0)
        lane = lax.broadcasted_iota(i32, (n, 128), 1)
        idx = 32 * ((lane >> 3) & 3) + 16 * (lane >> 6) + 2 * ((u + lane) & 7) + ((lane >> 5) & 1)
        t = pltpu.bitcast(x_v[X_TMP + 4 * u + k0:X_TMP + 4 * u + k1, 0:64, :].reshape(n, 128), u32)
        bw_v[8 * s + u, half * 256 + 64 * k0:half * 256 + 64 * k1, :] = jnp.take_along_axis(t, idx, axis=1)

    def perm_fill(fill, s, half, e_sel, e_gat):
        for k in range(4):
            put(fill, e_sel[k], P(perm_select, s, half, k))
        for k in range(16):
            assert e_gat(k) > e_sel[2 * (k // 8) + 1]
            put(fill, e_gat(k), P(perm_gather, s, half, k % 8, 2 * (k // 8), 2 * (k // 8) + 2))

    def pack_pairs(a, b):
        return (a & jnp.uint32(0xFFFF)) | (b << 16), (a >> 16) | (b & jnp.uint32(0xFFFF0000))

    def prep_bwo(n, v):
        r = (STG_BWO + n * DM) // 2 + 64 * v
        a = stgu[r:r + 64, :].reshape(8, 8, 128)
        b = stgu[r + 64:r + 128, :].reshape(8, 8, 128)
        a = pltpu.roll(a, 8 - v, 1) if v else a
        lo, hi = pack_pairs(a, pltpu.roll(b, 7 - v, 1))
        for k in range(8):
            d = 32 * (k % 2) + 4 * (k // 2) + v // 2
            bwo_v[n, pl.ds(d, 8, stride=OPITCH), :] = lo[k]
            bwo_v[n, pl.ds(d + 16, 8, stride=OPITCH), :] = hi[k]

    scale_b = DHB ** -0.5

    def b_qkv_dots(i, st, n0, n1):
        r0 = i * (TB // 2)
        if not isinstance(r0, int):
            r0 = pl.multiple_of(r0, TB // 2)

        def dot(n):
            lhs = _lhs([bxu[j, pl.ds(r0, TB // 2), :] for j in range(NC)])
            y = jnp.dot(lhs, _b16(bw_v[n]), preferred_element_type=f32)

            def store():
                x_v[st * 24 + n, HALO:HALO + TB, :] = y * scale_b if n < 8 else y
                if n >= 8:
                    x_v[((st + 1) % UB) * 24 + n, 0:HALO, :] = y[TB - HALO:TB]
            return y, store
        return [P(dot, n) for n in range(n0, n1)]

    def b_proj_dots(i, st):
        r0 = i * TB
        if not isinstance(r0, int):
            r0 = pl.multiple_of(r0, TB)

        def dot(n):
            lhs = _lhs([obu[st, j] for j in range(NC)])
            w = _b16(jnp.concatenate([bwo_v[n, OPITCH * u:OPITCH * u + 64, :] for u in range(8)], axis=0))
            y = jnp.dot(lhs, w, preferred_element_type=f32)

            def store():
                outb_v[pl.ds(r0, TB), 128 * n:128 * n + 128] = y.astype(bf16)
            return y, store
        return [P(dot, n) for n in range(NC)]

    def rows8(s0, r):
        return x_v[s0:s0 + 8, r:r + 8, :]

    def pos_ok(g, w):
        return lax.broadcasted_iota(i32, (8, 8, 128), 1) + (8 * g) - DIL * w >= 0

    def at_qk(st, g, half):
        q = rows8(st * 24, HALO + 8 * g)
        p = [jnp.sum(q * rows8(st * 24 + 8, HALO + 8 * g - DIL * w), axis=0) for w in range(4 * half, 4 * half + 4)]
        x_v[X_PART + (st % 2) * NG + g, 32 * half:32 * half + 32, :] = jnp.concatenate(p, axis=0)

    def at_softmax(st, g, first, pend):
        p = x_v[X_PART + (st % 2) * NG + g, 0:64, :]
        p = p + pltpu.roll(p, 32, 1)
        p = (p + pltpu.roll(p, 64, 1)).reshape(WIN, 8, 128)
        if first and 8 * g < DIL * (WIN - 1):
            p = jnp.where(pos_ok(g, lax.broadcasted_iota(i32, (8, 8, 128), 0)), p, -1e9)
        e = jnp.exp(p - jnp.max(p, axis=0, keepdims=True))
        l = jnp.sum(e, axis=0, keepdims=True)
        rc = pl.reciprocal(l, approx=True)
        pend[st, g] = e * (rc * (2.0 - l * rc))

    def at_store(st, g, pend):
        x_v[X_PROB + (st % 2) * NG + g, 0:64, :] = pend.pop((st, g)).reshape(64, 128)

    def at_pv(st, g, first, half):
        acc = None
        s0 = st * 24 + 16 + 4 * half
        for w in range(WIN):
            e = x_v[X_PROB + (st % 2) * NG + g:X_PROB + (st % 2) * NG + g + 1, 8 * w:8 * w + 8, :]
            r = HALO + 8 * g - DIL * w
            vv = x_v[s0:s0 + 4, r:r + 8, :]
            if first and 8 * g - DIL * w < 0:
                vv = jnp.where(pos_ok(g, w)[0:4], vv, x_v[s0:s0 + 4, HALO:HALO + 1, :])
            acc = e * vv if acc is None else acc + e * vv
        x_v[X_OUT + (st % 2) * NG + g, 32 * half:32 * half + 32, :] = acc.reshape(32, 128)

    def at_pack(st, g):
        o = [x_v[X_OUT + (st % 2) * NG + k, 0:64, :].reshape(8, 8, 128) for k in (g - 1, g)]
        ob_v[st, :, 8 * g - 8:8 * g + 8, :] = jnp.concatenate(o, axis=1).astype(bf16)

    pend = {}

    def attn_fill(fill, st, first, e_qk, e_sm, e_pv, step):
        for g, e in e_qk.items():
            put(fill, e, P(at_qk, st, g, 0))
            put(fill, e + step, P(at_qk, st, g, 1))
        for g, e in e_sm.items():
            put(fill, e, P(at_softmax, st, g, first, pend))
            put(fill, e + 3, P(at_store, st, g, pend))
        for g, e in e_pv.items():
            put(fill, e, P(at_pv, st, g, first, 0))
            put(fill, e + step, P(at_pv, st, g, first, 1))
            if g % 2 == 1:
                put(fill, e + 2 * step, P(at_pack, st, g))

    def ramp(e0, per, g0=0, g1=NG):
        return {g: e0 + per * g for g in range(g0, g1)}

    def a_relayout(src0, dst0, g):
        src = stgu.at[pl.ds(pl.multiple_of(src0, 256), HW // 2), :]
        dst = wa_v.at[pl.ds(dst0, DM // 32)]
        t = src[64 * g:64 * g + 64, :].reshape(2, 4, 8, 128)
        ev, od = pack_pairs(t[:, 0:2], t[:, 2:4])
        for dp in range(2):
            r = 2 * (g % 4) + dp
            for o in range(2):
                dst[g // 4, pl.ds(8 * o * PITCH + r, 8, stride=PITCH), :] = ev[dp, o]
                dst[g // 4, pl.ds((16 + 8 * o) * PITCH + r, 8, stride=PITCH), :] = od[dp, o]

    def sec(k0, k1, s):
        return [d for k in range(k0, k1) for d in b_qkv_dots(k, k, 8 * s, 8 * s + 8)]

    with _scope("perm_q"):
        x_v[8:24, 0:HALO, :] = jnp.zeros((16, HALO, 128), f32)
        for half in range(2):
            wait(bw_cps(0, half))
            if half == 0:
                start(bw_cps(2, 0) + bw_cps(2, 1) + bwo_cps() + bx_cps(1))
            for k in range(4):
                perm_select(0, half, k)
            for u in range(8):
                perm_gather(0, half, u, 0, 4)
    with _scope("Q01"):
        wait(bx_cps(0))
        run(sec(0, 2, 0), {})
    with _scope("Q2"):
        wait(bw_cps(1, 0))
        fill = {}
        perm_fill(fill, 1, 0, (-1, -1, -0.5, 0.5), lambda k: (2 * k // 3 - 1) / 2)
        run(sec(2, 3, 0), fill)
    with _scope("Q3K0"):
        wait(bw_cps(1, 1))
        start(bx_cps(2) + [aw_cp(0), mem_cp])
        fill = {}
        perm_fill(fill, 1, 1, (-1, -1, -0.5, 0.5), lambda k: (2 * k // 3 - 1) / 2)
        run(sec(3, 4, 0) + sec(0, 1, 1), fill)
    with _scope("K12"):
        wait(bw_cps(2, 0))
        fill = {}
        perm_fill(fill, 2, 0, (-1, -1, 0, 1), lambda k: 3 * k // 4 + 1)
        attn_fill(fill, 0, True, ramp(2, 1.5), {}, {}, 0.5)
        run(sec(1, 3, 1), fill)
    with _scope("K3V01"):
        wait(bw_cps(2, 1))
        fill = {}
        perm_fill(fill, 2, 1, (-1, -1, -0.5, 0.5), lambda k: (2 * k // 3 - 1) / 2)
        attn_fill(fill, 0, True, {}, ramp(5, 1), ramp(15, 1, 0, NG - 1), 0.5)
        attn_fill(fill, 1, False, ramp(2, 1.5), ramp(12, 1), {}, 0.5)
        run(sec(3, 4, 1) + sec(0, 2, 2), fill)
    with _scope("V23"):
        wait(bwo_cps())
        fill = {}
        attn_fill(fill, 0, True, {}, {}, {NG - 1: -1}, 0.5)
        attn_fill(fill, 1, False, {}, {}, ramp(0.5, 2, 0, NG - 1), 1)
        attn_fill(fill, 2, False, {0: -1}, {}, {}, 0)
        for n in range(4 * NC):
            put(fill, (n * 30 // 32 - 1) / 2, P(prep_bwo, n // 4, 2 * (n % 4)))
        run(sec(2, 4, 2), fill)

    def b_body(it, carry):
        with _scope("it"):
            for c in (1, 2):
                @pl.when(it == c)
                def _():
                    wait(bx_cps(c))

            @pl.when(it >= 2)
            def _():
                cw = jnp.maximum(it - 2, 0)
                dst = stg_v.at[pl.ds(pl.multiple_of(STG_AW + cw * HW, HW), HW), :]
                pltpu.make_async_copy(dst, dst, sem.at[SEM_AW + cw]).wait()

            for c in range(1, NIT):
                @pl.when(it == c)
                def _():
                    cols = {6: (5, 6, 7), 7: ()}.get(c, (c - 1,))
                    start(([ob_cp(UB * TB * (c - 2), UB * TB)] if c >= 2 else []) + ([aw_cp(c)] if c < 6 else [])
                          + [cp(n) for n in cols for cp in (awo_cp, ax_cp)])
            c = jnp.maximum(it - 2, 0)
            src0 = jnp.where(it == 1, STG_BW // 2, STG_AW // 2 + c * (HW // 2))
            dst0 = c * (DM // 32)
            dots, fill = [], {}
            for k in range(UB):
                i, e0 = UB * it + k, 32 * k
                dots += b_qkv_dots(i, k, 0, 24) + b_proj_dots(i - 4, k)
                e0 -= 1
                attn_fill(fill, (k - 3) % UB, False, {}, {}, {NG - 1: e0}, 1)
                attn_fill(fill, (k - 2) % UB, False, ramp(e0 - 2, 4, 1), ramp(e0, 4), ramp(e0 + 4, 4, 0, NG - 1), 1)
                attn_fill(fill, (k - 1) % UB, False, {0: e0 + 30}, {}, {}, 1)
                for g in range(32):
                    put(fill, e0 + g + 0.5, P(a_relayout, src0, dst0, 32 * k + g))
            run(dots, fill)
        return carry
    lax.fori_loop(1, NIT, b_body, 0)
    nb = S // TB
    wait([awo_cp(n) for n in range(NC)] + [ax_cp(j) for j in range(NC)] + [mem_cp])
    with _scope("tailB"):
        ob_cp(S - 2 * UB * TB, UB * TB).start()
        fill = {}
        attn_fill(fill, 1, False, {}, {}, {NG - 1: -1}, 0.5)
        attn_fill(fill, 2, False, ramp(-2, 1, 1), ramp(-1, 1), ramp(6, 1), 0.5)
        attn_fill(fill, 3, False, ramp(1, 2), {}, {}, 1)
        attn_fill(fill, 3, False, {}, ramp(10, 1), ramp(14, 1), 0.5)
        run([d for k in range(UB) for d in b_proj_dots(nb - 4 + k, k)], fill)
        ob_cp(S - UB * TB, UB * TB).start()


    scale_a = DH ** -0.5
    rr = lax.broadcasted_iota(i32, (2 * L, 2 * L), 0)
    cc = lax.broadcasted_iota(i32, (2 * L, 2 * L), 1)
    rb_, cb_ = rr >= L, cc >= L
    ri, ci = jnp.where(rb_, rr - L, rr), jnp.where(cb_, cc - L, cc)
    same = rb_ == cb_
    valid = same & ((ri < M) | (ri >= ci))
    fill = jnp.where(same, -1e9, -jnp.inf).astype(f32)

    mem_s[...] = mem_v[...].astype(f32)
    NP = H // 2

    def a_step(lhs, even):
        qkv, pp = {}, {}
        nrow = 32 if even else 48

        def proj(wh, k0, k1):
            s0, r = (wh // H) * (DM // 16), ((wh % H) // 2 + (H // 2) * (wh % 2)) * PITCH
            w = wa_v[s0 + k0 // 16:s0 + k1 // 16, r:r + 8, :].reshape((k1 - k0) // 2, 128)
            return jnp.dot(lhs[:, k0:k1], _b16(w), preferred_element_type=f32)

        def do_qkv(j, after_dot):
            split = j == 0 and not even
            lo = {wi * H + hh: proj(wi * H + hh, 0, DM // 2) for hh in (0, 1) for wi in range(3)} if split else {}
            parts = [[], [], []]
            for hh in (2 * j, 2 * j + 1):
                for wi in range(3):
                    wh = wi * H + hh
                    y = proj(wh, DM // 2, DM) + lo[wh] if split else proj(wh, 0, DM)
                    if even:
                        stash[wh] = y[32:40]
                        parts[wi] += [y[40:48], y[0:32]]
                    else:
                        parts[wi] += [y[0:8], stash[wh], y[8:32]]
                    after_dot(3 * hh + wi)
            qkv[j] = [jnp.concatenate(p, axis=0).astype(bf16) for p in parts]

        def do_qk(j):
            q2, k2, _ = qkv[j]
            s = lax.dot_general(q2, k2, (((1,), (1,)), ((), ())), preferred_element_type=f32) * scale_a
            s = jnp.where(valid, s, fill)
            m = jnp.max(s, axis=1, keepdims=True)
            e = jnp.exp(s - m)
            l = jnp.sum(e, axis=1, keepdims=True)
            rc = pl.reciprocal(l, approx=True)
            rc = rc * (2.0 - l * rc)
            pp[j] = (e * rc).astype(bf16)

        def do_pv(j):
            o2 = jnp.dot(pp.pop(j), qkv.pop(j)[2], preferred_element_type=f32)
            for i, hh in enumerate((2 * j, 2 * j + 1)):
                o = o2[L * i:L * (i + 1)]
                if even:
                    o_s[hh, 0:32, :] = o[0:32].astype(bf16)
                    ostash[hh] = o[32:40]
                else:
                    o_s[hh] = jnp.concatenate([o[0:8], ostash[hh], o[8:40]], axis=0).astype(bf16)

        ya = {}

        def wo_part(n, h0, h1):
            lo = _lhs([osu[hh, 0:nrow // 2, :] for hh in range(h0, h1)])
            r = jnp.dot(lo, _b16(wou[n, h0 * 64:h1 * 64, :]), preferred_element_type=f32)
            ya[n] = r + ya[n] if n in ya else r

        ni = 0 if even else NI
        pieces = [(n, 4 * g, 4 * g + 4) for g in range(ni) for n in range(NC)]
        d0 = 6 * (LPV + 2)
        done = []

        def after_dot(d):
            ready = NC * max(((d + 1) // 6 - LPV - 1 + (1 if (d + 1) % 6 else 0)) // 2, 0)
            while len(done) < min((d - d0 + 1) * len(pieces) // (3 * H - d0), ready):
                wo_part(*pieces[len(done)])
                done.append(0)

        for j in range(NP):
            do_qkv(j, after_dot)
            if j - LQK >= 0:
                do_qk(j - LQK)
            if j - LPV >= 0:
                do_pv(j - LPV)
        assert len(done) == len(pieces)
        nper, n = NC // (LPV + 1), 0
        for j in range(NP, NP + LPV):
            for _ in range(nper):
                wo_part(n, 4 * ni, 2 * KA)
                n += 1
            if j - LQK < NP:
                do_qk(j - LQK)
            do_pv(j - LPV)
        for n in range(n, NC):
            wo_part(n, 4 * ni, 2 * KA)
        for n in range(NC):
            wo_part(n, 2 * KA, H)
        return jnp.concatenate([ya[n] for n in range(NC)], axis=1)

    def a_body(t, c):
        with _scope("a_it"):
            return a_pair(t, c)

    def a_pair(t, c):
        @pl.when(t > 0)
        def _():
            oa_cp(pl.multiple_of(jnp.maximum(t - 1, 0) * 64, 64), 64).start()
        r0 = pl.multiple_of(t * 32, 32)
        X = _lhs([axu[j, pl.ds(r0, 32), :] for j in range(NC)])
        Xm = X[32:48].astype(f32)
        mixed = jnp.concatenate([Xm[0:8], mem_s[...]], axis=0).astype(bf16)
        ye = a_step(jnp.concatenate([X[0:32], mixed], axis=0), True)
        mixed = jnp.concatenate([ye[0:8], Xm[8:16]], axis=0).astype(bf16)
        yo = a_step(jnp.concatenate([mixed, X[48:64]], axis=0), False)
        mem_s[...] = yo[0:8]
        o0 = pl.multiple_of(t * 64, 64)
        outa_v[pl.ds(o0, 64), :] = jnp.concatenate([ye[8:32], yo[8:48]], axis=0).astype(bf16)
        return c
    lax.fori_loop(0, S // 64, a_body, 0)
    oa_cp(S - 64, 64).start()

    ob_cp(0, S).wait()
    oa_cp(0, S).wait()


@jax.jit
def _run(A_x, A_mem0, A_Wq, A_Wk, A_Wv, A_Wo, B_x, B_wqkv, B_wo):
    hbm = pl.BlockSpec(memory_space=pl.ANY)
    out = pl.pallas_call(
        _kernel,
        out_shape=jax.ShapeDtypeStruct((S, 2 * DM), bf16),
        in_specs=[hbm] * 9,
        out_specs=hbm,
        scratch_shapes=[
            pltpu.VMEM((NC, S, 128), bf16),
            pltpu.VMEM((M, DM), bf16),
            pltpu.VMEM((STG_ROWS, 128), bf16),
            pltpu.VMEM((3 * DM // 16, H * PITCH + 8, 128), u32),
            pltpu.VMEM((NC, H * DH, 128), bf16),
            pltpu.VMEM((NC, S, 128), bf16),
            pltpu.VMEM((24, DM // 2, 128), u32),
            pltpu.VMEM((NC, 9 * OPITCH - 1, 128), u32),
            pltpu.VMEM((S, DM), bf16),
            pltpu.VMEM((S, DM), bf16),
            pltpu.VMEM((X_SLABS, TB + HALO, 128), f32),
            pltpu.VMEM((UB, 8, TB, 128), bf16),
            pltpu.VMEM((M, DM), f32),
            pltpu.VMEM((3 * H, 8, DH), f32),
            pltpu.VMEM((H, 8, DH), f32),
            pltpu.VMEM((H, 48, DH), bf16),
            pltpu.SMEM((1,), i32),
            pltpu.SemaphoreType.DMA((NSEM,)),
        ],
        compiler_params=pltpu.CompilerParams(vmem_limit_bytes=110 * 1024 * 1024, disable_bounds_checks=True),
    )(
        A_x.reshape(S, DM), A_mem0.reshape(M, DM),
        A_Wq.reshape(DM * H, DH), A_Wk.reshape(DM * H, DH), A_Wv.reshape(DM * H, DH),
        A_Wo.reshape(H * DH, DM),
        B_x.reshape(S, DM), B_wqkv, B_wo,
    )
    return out.reshape(1, S, 2 * DM)


def pallas_concat_heads__memory_aug_recurrent_mem_tr__sliding_local_dilated__prompt_kernel(
    A_x, A_mem0, A_Wq, A_Wk, A_Wv, A_Wo, A_seg_len, B_x, B_wqkv, B_wo,
):
    if isinstance(A_seg_len, int):
        assert A_seg_len == SEG
    return _run(A_x, A_mem0, A_Wq, A_Wk, A_Wv, A_Wo, B_x, B_wqkv, B_wo)
```

```python
import contextlib
import functools

import jax
import jax.numpy as jnp
from jax import lax
import jax.experimental.pallas as pl
import jax.experimental.pallas.tpu as pltpu

bf16, f32, u32, i32 = jnp.bfloat16, jnp.float32, jnp.uint32, jnp.int32

S, DM = 2048, 1024
H, DH = 32, 128
M, SEG = 8, 32
L = M + SEG
DHB, WIN, DIL = 32, 8, 2
NC = DM // 128

TB = 64
UB = 4
HALO = 16
NIT = S // (TB * UB)
LQK, LPV, KA, NI = 1, 3, 12, 3

PITCH = 9
OPITCH = 65
HW = DM * H // 2
STG_AW, STG_BW, STG_BWO = 0, 6 * HW, 6 * HW + 24 * DM
STG_TOK = STG_BWO + NC * DM
STG_ROWS = STG_TOK + 64
NG = TB // 8
X_PART = UB * 24
X_PROB = X_PART + 2 * NG
X_OUT = X_PROB + 2 * NG
X_TMP = X_OUT + 2 * NG
X_FEN = X_TMP + 32
X_SLABS = X_FEN + 2

SEM_BW, SEM_BX, SEM_BWO, SEM_AW, SEM_AWO, SEM_AX, SEM_MEM, SEM_OB, SEM_OA = 0, 6, 9, 10, 16, 17, 18, 19, 20
NSEM = 21
_SCOPES = False


def _scope(name):
    return jax.named_scope(name) if _SCOPES else contextlib.nullcontext()


def _b16(v):
    return pltpu.bitcast(v, bf16)


def _u32(view):
    return view.bitcast(u32)[...]


def _lhs(blocks):
    return _b16(jnp.concatenate(blocks, axis=1))


def _kernel(ax_h, mem_h, wq_h, wk_h, wv_h, wo_h, bx_h, bw_h, bwo_h, out_h,
            ax_v, mem_v, stg_v, wa_v, wo_v, bx_v, bw_v, bwo_v, outa_v, outb_v,
            x_v, ob_v, mem_s, stash, ostash, o_s, zero_s, sem):
    P = functools.partial

    def bw_cps(s, half):
        return [pltpu.make_async_copy(bw_h.at[pl.ds(half * (DM // 2), DM // 2), pl.ds(128 * n, 128)],
                                      stg_v.at[pl.ds(STG_BW + DM * n + half * (DM // 2), DM // 2), :],
                                      sem.at[SEM_BW + 2 * s + half]) for n in range(8 * s, 8 * s + 8)]

    def bx_cps(part):
        rows = (pl.ds(0, TB * UB), pl.ds(TB * UB, TB * UB), pl.ds(2 * TB * UB, S - 2 * TB * UB))[part]
        return [pltpu.make_async_copy(bx_h.at[rows, pl.ds(128 * j, 128)], bx_v.at[j, rows, :],
                                      sem.at[SEM_BX + part]) for j in range(NC)]

    def bwo_cps():
        return [pltpu.make_async_copy(bwo_h.at[:, pl.ds(128 * n, 128)], stg_v.at[pl.ds(STG_BWO + DM * n, DM), :],
                                      sem.at[SEM_BWO]) for n in range(NC)]

    def aw_cp(c):
        src = (wq_h, wk_h, wv_h)[c // 2]
        return pltpu.make_async_copy(src.at[pl.ds((c % 2) * HW, HW), :], stg_v.at[pl.ds(STG_AW + c * HW, HW), :],
                                     sem.at[SEM_AW + c])

    def awo_cp(n):
        return pltpu.make_async_copy(wo_h.at[:, pl.ds(128 * n, 128)], wo_v.at[n], sem.at[SEM_AWO])

    def ax_cp(j):
        return pltpu.make_async_copy(ax_h.at[:, pl.ds(128 * j, 128)], ax_v.at[j], sem.at[SEM_AX])

    mem_cp = pltpu.make_async_copy(mem_h, mem_v, sem.at[SEM_MEM])

    def ob_cp(r0, n):
        return pltpu.make_async_copy(outb_v.at[pl.ds(r0, n), :], out_h.at[pl.ds(r0, n), pl.ds(DM, DM)],
                                     sem.at[SEM_OB])

    def oa_cp(r0, n):
        return pltpu.make_async_copy(outa_v.at[pl.ds(r0, n), :], out_h.at[pl.ds(r0, n), pl.ds(0, DM)],
                                     sem.at[SEM_OA])

    def start(cps):
        for c in cps:
            c.start()

    def wait(cps):
        for c in cps:
            c.wait()

    start(bw_cps(0, 0) + bw_cps(0, 1) + bx_cps(0) + bw_cps(1, 0) + bw_cps(1, 1))

    zero_s[0] = 0
    x_v[X_FEN + 1, 0:8, :] = jnp.zeros((8, 128), f32)

    def run(dots, fill):
        z = pl.multiple_of(zero_s[0], 64)
        busy = [False]

        def epoch(e, y, close):
            if y is not None and (e in fill or (close and busy[0])):
                x_v[z + X_FEN, 0:8, :] = y
                stg_v.at[pl.ds(z + STG_TOK, 16), :].bitcast(f32)[...] = x_v[X_FEN + 1, 0:8, :]
                busy[0] = False
            for f in fill.pop(e, []):
                f()
                busy[0] = True

        epoch(-1, None, False)
        for n, d in enumerate(dots):
            y, store = d()
            epoch(n - 0.5, y[0:8], False)
            store()
            epoch(n, y[TB - 8:TB], True)
        assert not fill, sorted(fill)

    def put(fill, n, f):
        fill.setdefault(n, []).append(f)

    lane16 = lax.broadcasted_iota(i32, (16, 128), 1)

    def perm_select(s, half, k):
        bits = [((lane16 >> (b + 1)) & 1) == 1 for b in range(3)]
        for r in range(0, 64, 16):
            src = STG_BW + 8 * s * DM + 2 * (half * 256 + 64 * k + r)
            zs = [_u32(stg_v.at[pl.ds(src + ((-t) % 8) * DM, 32), :]) for t in range(8)]
            for b in range(3):
                zs = [lax.select(bits[b], zs[(t - (1 << b)) % 8], zs[t]) for t in range(8)]
            for u in range(8):
                x_v[X_TMP + 4 * u + k, r:r + 16, :] = pltpu.bitcast(zs[u], f32)

    def perm_gather(s, half, u, k0, k1):
        n = 64 * (k1 - k0)
        lane = lax.broadcasted_iota(i32, (n, 128), 1)
        idx = 32 * ((lane >> 3) & 3) + 16 * (lane >> 6) + 2 * ((u + lane) & 7) + ((lane >> 5) & 1)
        t = pltpu.bitcast(x_v[X_TMP + 4 * u + k0:X_TMP + 4 * u + k1, 0:64, :].reshape(n, 128), u32)
        bw_v[8 * s + u, half * 256 + 64 * k0:half * 256 + 64 * k1, :] = jnp.take_along_axis(t, idx, axis=1)

    def perm_fill(fill, s, half, e_sel, e_gat):
        for k in range(4):
            put(fill, e_sel[k], P(perm_select, s, half, k))
        for k in range(16):
            assert e_gat(k) > e_sel[2 * (k // 8) + 1]
            put(fill, e_gat(k), P(perm_gather, s, half, k % 8, 2 * (k // 8), 2 * (k // 8) + 2))

    def pack_pairs(a, b):
        return (a & jnp.uint32(0xFFFF)) | (b << 16), (a >> 16) | (b & jnp.uint32(0xFFFF0000))

    def prep_bwo(n, v):
        r = STG_BWO + n * DM + 128 * v
        a = _u32(stg_v.at[pl.ds(r, 128), :]).reshape(8, 8, 128)
        b = _u32(stg_v.at[pl.ds(r + 128, 128), :]).reshape(8, 8, 128)
        a = pltpu.roll(a, 8 - v, 1) if v else a
        lo, hi = pack_pairs(a, pltpu.roll(b, 7 - v, 1))
        for k in range(8):
            d = 32 * (k % 2) + 4 * (k // 2) + v // 2
            bwo_v[n, pl.ds(d, 8, stride=OPITCH), :] = lo[k]
            bwo_v[n, pl.ds(d + 16, 8, stride=OPITCH), :] = hi[k]

    scale_b = DHB ** -0.5

    def b_qkv_dots(i, st, n0, n1):
        r0 = i * TB
        if not isinstance(r0, int):
            r0 = pl.multiple_of(r0, TB)

        def dot(n):
            lhs = _lhs([_u32(bx_v.at[j, pl.ds(r0, TB), :]) for j in range(NC)])
            y = jnp.dot(lhs, _b16(bw_v[n]), preferred_element_type=f32)

            def store():
                x_v[st * 24 + n, HALO:HALO + TB, :] = y * scale_b if n < 8 else y
                if n >= 8:
                    x_v[((st + 1) % UB) * 24 + n, 0:HALO, :] = y[TB - HALO:TB]
            return y, store
        return [P(dot, n) for n in range(n0, n1)]

    def b_proj_dots(i, st):
        r0 = i * TB
        if not isinstance(r0, int):
            r0 = pl.multiple_of(r0, TB)

        def dot(n):
            lhs = _lhs([_u32(ob_v.at[st, j]) for j in range(NC)])
            w = _b16(jnp.concatenate([bwo_v[n, OPITCH * u:OPITCH * u + 64, :] for u in range(8)], axis=0))
            y = jnp.dot(lhs, w, preferred_element_type=f32)

            def store():
                outb_v[pl.ds(r0, TB), 128 * n:128 * n + 128] = y.astype(bf16)
            return y, store
        return [P(dot, n) for n in range(NC)]

    def rows8(s0, r):
        return x_v[s0:s0 + 8, r:r + 8, :]

    def pos_ok(g, w):
        return lax.broadcasted_iota(i32, (8, 8, 128), 1) + (8 * g) - DIL * w >= 0

    def at_qk(st, g, half):
        q = rows8(st * 24, HALO + 8 * g)
        p = [jnp.sum(q * rows8(st * 24 + 8, HALO + 8 * g - DIL * w), axis=0) for w in range(4 * half, 4 * half + 4)]
        x_v[X_PART + (st % 2) * NG + g, 32 * half:32 * half + 32, :] = jnp.concatenate(p, axis=0)

    def at_softmax(st, g, first, pend):
        p = x_v[X_PART + (st % 2) * NG + g, 0:64, :]
        p = p + pltpu.roll(p, 32, 1)
        p = (p + pltpu.roll(p, 64, 1)).reshape(WIN, 8, 128)
        if first and 8 * g < DIL * (WIN - 1):
            p = jnp.where(pos_ok(g, lax.broadcasted_iota(i32, (8, 8, 128), 0)), p, -1e9)
        e = jnp.exp(p - jnp.max(p, axis=0, keepdims=True))
        l = jnp.sum(e, axis=0, keepdims=True)
        rc = pl.reciprocal(l, approx=True)
        pend[st, g] = e * (rc * (2.0 - l * rc))

    def at_store(st, g, pend):
        x_v[X_PROB + (st % 2) * NG + g, 0:64, :] = pend.pop((st, g)).reshape(64, 128)

    def at_pv(st, g, first, half):
        acc = None
        s0 = st * 24 + 16 + 4 * half
        for w in range(WIN):
            e = x_v[X_PROB + (st % 2) * NG + g:X_PROB + (st % 2) * NG + g + 1, 8 * w:8 * w + 8, :]
            r = HALO + 8 * g - DIL * w
            vv = x_v[s0:s0 + 4, r:r + 8, :]
            if first and 8 * g - DIL * w < 0:
                vv = jnp.where(pos_ok(g, w)[0:4], vv, x_v[s0:s0 + 4, HALO:HALO + 1, :])
            acc = e * vv if acc is None else acc + e * vv
        x_v[X_OUT + (st % 2) * NG + g, 32 * half:32 * half + 32, :] = acc.reshape(32, 128)

    def at_pack(st, g):
        o = [x_v[X_OUT + (st % 2) * NG + k, 0:64, :].reshape(8, 8, 128) for k in (g - 1, g)]
        ob_v[st, :, 8 * g - 8:8 * g + 8, :] = jnp.concatenate(o, axis=1).astype(bf16)

    pend = {}

    def attn_fill(fill, st, first, e_qk, e_sm, e_pv, step):
        for g, e in e_qk.items():
            put(fill, e, P(at_qk, st, g, 0))
            put(fill, e + step, P(at_qk, st, g, 1))
        for g, e in e_sm.items():
            put(fill, e, P(at_softmax, st, g, first, pend))
            put(fill, e + 3, P(at_store, st, g, pend))
        for g, e in e_pv.items():
            put(fill, e, P(at_pv, st, g, first, 0))
            put(fill, e + step, P(at_pv, st, g, first, 1))
            if g % 2 == 1:
                put(fill, e + 2 * step, P(at_pack, st, g))

    def ramp(e0, per, g0=0, g1=NG):
        return {g: e0 + per * g for g in range(g0, g1)}

    def a_relayout(src0, dst0, g):
        src = stg_v.at[pl.ds(pl.multiple_of(src0, 512), HW), :].bitcast(u32)
        dst = wa_v.at[pl.ds(dst0, DM // 32)]
        t = src[64 * g:64 * g + 64, :].reshape(2, 4, 8, 128)
        ev, od = pack_pairs(t[:, 0:2], t[:, 2:4])
        for dp in range(2):
            r = 2 * (g % 4) + dp
            for o in range(2):
                dst[g // 4, pl.ds(8 * o * PITCH + r, 8, stride=PITCH), :] = ev[dp, o]
                dst[g // 4, pl.ds((16 + 8 * o) * PITCH + r, 8, stride=PITCH), :] = od[dp, o]

    def sec(k0, k1, s):
        return [d for k in range(k0, k1) for d in b_qkv_dots(k, k, 8 * s, 8 * s + 8)]

    with _scope("perm_q"):
        x_v[8:24, 0:HALO, :] = jnp.zeros((16, HALO, 128), f32)
        for half in range(2):
            wait(bw_cps(0, half))
            if half == 0:
                start(bw_cps(2, 0) + bw_cps(2, 1) + bwo_cps() + bx_cps(1))
            for k in range(4):
                perm_select(0, half, k)
            for u in range(8):
                perm_gather(0, half, u, 0, 4)
    with _scope("Q01"):
        wait(bx_cps(0))
        run(sec(0, 2, 0), {})
    with _scope("Q2"):
        wait(bw_cps(1, 0))
        fill = {}
        perm_fill(fill, 1, 0, (-1, -1, -0.5, 0.5), lambda k: (2 * k // 3 - 1) / 2)
        run(sec(2, 3, 0), fill)
    with _scope("Q3K0"):
        wait(bw_cps(1, 1))
        start(bx_cps(2) + [aw_cp(0), mem_cp])
        fill = {}
        perm_fill(fill, 1, 1, (-1, -1, -0.5, 0.5), lambda k: (2 * k // 3 - 1) / 2)
        run(sec(3, 4, 0) + sec(0, 1, 1), fill)
    with _scope("K12"):
        wait(bw_cps(2, 0))
        fill = {}
        perm_fill(fill, 2, 0, (-1, -1, 0, 1), lambda k: 3 * k // 4 + 1)
        attn_fill(fill, 0, True, ramp(2, 1.5), {}, {}, 0.5)
        run(sec(1, 3, 1), fill)
    with _scope("K3V01"):
        wait(bw_cps(2, 1))
        fill = {}
        perm_fill(fill, 2, 1, (-1, -1, -0.5, 0.5), lambda k: (2 * k // 3 - 1) / 2)
        attn_fill(fill, 0, True, {}, ramp(5, 1), ramp(15, 1, 0, NG - 1), 0.5)
        attn_fill(fill, 1, False, ramp(2, 1.5), ramp(12, 1), {}, 0.5)
        run(sec(3, 4, 1) + sec(0, 2, 2), fill)
    with _scope("V23"):
        wait(bwo_cps())
        fill = {}
        attn_fill(fill, 0, True, {}, {}, {NG - 1: -1}, 0.5)
        attn_fill(fill, 1, False, {}, {}, ramp(0.5, 2, 0, NG - 1), 1)
        attn_fill(fill, 2, False, {0: -1}, {}, {}, 0)
        for n in range(4 * NC):
            put(fill, (n * 30 // 32 - 1) / 2, P(prep_bwo, n // 4, 2 * (n % 4)))
        run(sec(2, 4, 2), fill)

    def b_body(it, carry):
        with _scope("it"):
            for c in (1, 2):
                @pl.when(it == c)
                def _():
                    wait(bx_cps(c))

            @pl.when(it >= 2)
            def _():
                cw = jnp.maximum(it - 2, 0)
                dst = stg_v.at[pl.ds(pl.multiple_of(STG_AW + cw * HW, HW), HW), :]
                pltpu.make_async_copy(dst, dst, sem.at[SEM_AW + cw]).wait()

            for c in range(1, NIT):
                @pl.when(it == c)
                def _():
                    cols = {6: (5, 6, 7), 7: ()}.get(c, (c - 1,))
                    start(([ob_cp(UB * TB * (c - 2), UB * TB)] if c >= 2 else []) + ([aw_cp(c)] if c < 6 else [])
                          + [cp(n) for n in cols for cp in (awo_cp, ax_cp)])
            c = jnp.maximum(it - 2, 0)
            src0 = jnp.where(it == 1, STG_BW, STG_AW + c * HW)
            dst0 = c * (DM // 32)
            dots, fill = [], {}
            for k in range(UB):
                i, e0 = UB * it + k, 32 * k
                dots += b_qkv_dots(i, k, 0, 24) + b_proj_dots(i - 4, k)
                e0 -= 1
                attn_fill(fill, (k - 3) % UB, False, {}, {}, {NG - 1: e0}, 1)
                attn_fill(fill, (k - 2) % UB, False, ramp(e0 - 2, 4, 1), ramp(e0, 4), ramp(e0 + 4, 4, 0, NG - 1), 1)
                attn_fill(fill, (k - 1) % UB, False, {0: e0 + 30}, {}, {}, 1)
                for g in range(32):
                    put(fill, e0 + g + 0.5, P(a_relayout, src0, dst0, 32 * k + g))
            run(dots, fill)
        return carry
    lax.fori_loop(1, NIT, b_body, 0)
    nb = S // TB
    wait([awo_cp(n) for n in range(NC)] + [ax_cp(j) for j in range(NC)] + [mem_cp])
    with _scope("tailB"):
        ob_cp(S - 2 * UB * TB, UB * TB).start()
        fill = {}
        attn_fill(fill, 1, False, {}, {}, {NG - 1: -1}, 0.5)
        attn_fill(fill, 2, False, ramp(-2, 1, 1), ramp(-1, 1), ramp(6, 1), 0.5)
        attn_fill(fill, 3, False, ramp(1, 2), {}, {}, 1)
        attn_fill(fill, 3, False, {}, ramp(10, 1), ramp(14, 1), 0.5)
        run([d for k in range(UB) for d in b_proj_dots(nb - 4 + k, k)], fill)
        ob_cp(S - UB * TB, UB * TB).start()


    scale_a = DH ** -0.5
    rr = lax.broadcasted_iota(i32, (2 * L, 2 * L), 0)
    cc = lax.broadcasted_iota(i32, (2 * L, 2 * L), 1)
    rb_, cb_ = rr >= L, cc >= L
    ri, ci = jnp.where(rb_, rr - L, rr), jnp.where(cb_, cc - L, cc)
    same = rb_ == cb_
    valid = same & ((ri < M) | (ri >= ci))
    fill = jnp.where(same, -1e9, -jnp.inf).astype(f32)

    mem_s[...] = mem_v[...].astype(f32)
    NP = H // 2

    def a_step(lhs, even):
        qkv, pp = {}, {}
        nrow = 32 if even else 48

        def proj(wh, k0, k1):
            s0, r = (wh // H) * (DM // 16), ((wh % H) // 2 + (H // 2) * (wh % 2)) * PITCH
            w = wa_v[s0 + k0 // 16:s0 + k1 // 16, r:r + 8, :].reshape((k1 - k0) // 2, 128)
            return jnp.dot(lhs[:, k0:k1], _b16(w), preferred_element_type=f32)

        def do_qkv(j, after_dot):
            split = j == 0 and not even
            lo = {wi * H + hh: proj(wi * H + hh, 0, DM // 2) for hh in (0, 1) for wi in range(3)} if split else {}
            parts = [[], [], []]
            for hh in (2 * j, 2 * j + 1):
                for wi in range(3):
                    wh = wi * H + hh
                    y = proj(wh, DM // 2, DM) + lo[wh] if split else proj(wh, 0, DM)
                    if even:
                        stash[wh] = y[32:40]
                        parts[wi] += [y[40:48], y[0:32]]
                    else:
                        parts[wi] += [y[0:8], stash[wh], y[8:32]]
                    after_dot(3 * hh + wi)
            qkv[j] = [jnp.concatenate(p, axis=0).astype(bf16) for p in parts]

        def do_qk(j):
            q2, k2, _ = qkv[j]
            s = lax.dot_general(q2, k2, (((1,), (1,)), ((), ())), preferred_element_type=f32) * scale_a
            s = jnp.where(valid, s, fill)
            m = jnp.max(s, axis=1, keepdims=True)
            e = jnp.exp(s - m)
            l = jnp.sum(e, axis=1, keepdims=True)
            rc = pl.reciprocal(l, approx=True)
            rc = rc * (2.0 - l * rc)
            pp[j] = (e * rc).astype(bf16)

        def do_pv(j):
            o2 = jnp.dot(pp.pop(j), qkv.pop(j)[2], preferred_element_type=f32)
            for i, hh in enumerate((2 * j, 2 * j + 1)):
                o = o2[L * i:L * (i + 1)]
                if even:
                    o_s[hh, 0:32, :] = o[0:32].astype(bf16)
                    ostash[hh] = o[32:40]
                else:
                    o_s[hh] = jnp.concatenate([o[0:8], ostash[hh], o[8:40]], axis=0).astype(bf16)

        ya = {}

        def wo_part(n, h0, h1):
            lo = _lhs([_u32(o_s.at[hh, pl.ds(0, nrow), :]) for hh in range(h0, h1)])
            w = _u32(wo_v.at[n, pl.ds(h0 * DH, (h1 - h0) * DH), :])
            r = jnp.dot(lo, _b16(w), preferred_element_type=f32)
            ya[n] = r + ya[n] if n in ya else r

        ni = 0 if even else NI
        pieces = [(n, 4 * g, 4 * g + 4) for g in range(ni) for n in range(NC)]
        d0 = 6 * (LPV + 2)
        done = []

        def after_dot(d):
            ready = NC * max(((d + 1) // 6 - LPV - 1 + (1 if (d + 1) % 6 else 0)) // 2, 0)
            while len(done) < min((d - d0 + 1) * len(pieces) // (3 * H - d0), ready):
                wo_part(*pieces[len(done)])
                done.append(0)

        for j in range(NP):
            do_qkv(j, after_dot)
            if j - LQK >= 0:
                do_qk(j - LQK)
            if j - LPV >= 0:
                do_pv(j - LPV)
        assert len(done) == len(pieces)
        nper, n = NC // (LPV + 1), 0
        for j in range(NP, NP + LPV):
            for _ in range(nper):
                wo_part(n, 4 * ni, 2 * KA)
                n += 1
            if j - LQK < NP:
                do_qk(j - LQK)
            do_pv(j - LPV)
        for n in range(n, NC):
            wo_part(n, 4 * ni, 2 * KA)
        for n in range(NC):
            wo_part(n, 2 * KA, H)
        return jnp.concatenate([ya[n] for n in range(NC)], axis=1)

    def a_body(t, c):
        with _scope("a_it"):
            return a_pair(t, c)

    def a_pair(t, c):
        @pl.when(t > 0)
        def _():
            oa_cp(pl.multiple_of(jnp.maximum(t - 1, 0) * 64, 64), 64).start()
        o0 = pl.multiple_of(t * 64, 64)
        X = _lhs([_u32(ax_v.at[j, pl.ds(o0, 64), :]) for j in range(NC)])
        Xm = X[32:48].astype(f32)
        mixed = jnp.concatenate([Xm[0:8], mem_s[...]], axis=0).astype(bf16)
        ye = a_step(jnp.concatenate([X[0:32], mixed], axis=0), True)
        mixed = jnp.concatenate([ye[0:8], Xm[8:16]], axis=0).astype(bf16)
        yo = a_step(jnp.concatenate([mixed, X[48:64]], axis=0), False)
        mem_s[...] = yo[0:8]
        outa_v[pl.ds(o0, 64), :] = jnp.concatenate([ye[8:32], yo[8:48]], axis=0).astype(bf16)
        return c
    lax.fori_loop(0, S // 64, a_body, 0)
    oa_cp(S - 64, 64).start()

    ob_cp(0, S).wait()
    oa_cp(0, S).wait()


@jax.jit
def _run(A_x, A_mem0, A_Wq, A_Wk, A_Wv, A_Wo, B_x, B_wqkv, B_wo):
    hbm = pl.BlockSpec(memory_space=pl.ANY)
    out = pl.pallas_call(
        _kernel,
        out_shape=jax.ShapeDtypeStruct((S, 2 * DM), bf16),
        in_specs=[hbm] * 9,
        out_specs=hbm,
        scratch_shapes=[
            pltpu.VMEM((NC, S, 128), bf16),
            pltpu.VMEM((M, DM), bf16),
            pltpu.VMEM((STG_ROWS, 128), bf16),
            pltpu.VMEM((3 * DM // 16, H * PITCH + 8, 128), u32),
            pltpu.VMEM((NC, H * DH, 128), bf16),
            pltpu.VMEM((NC, S, 128), bf16),
            pltpu.VMEM((24, DM // 2, 128), u32),
            pltpu.VMEM((NC, 9 * OPITCH - 1, 128), u32),
            pltpu.VMEM((S, DM), bf16),
            pltpu.VMEM((S, DM), bf16),
            pltpu.VMEM((X_SLABS, TB + HALO, 128), f32),
            pltpu.VMEM((UB, 8, TB, 128), bf16),
            pltpu.VMEM((M, DM), f32),
            pltpu.VMEM((3 * H, 8, DH), f32),
            pltpu.VMEM((H, 8, DH), f32),
            pltpu.VMEM((H, 48, DH), bf16),
            pltpu.SMEM((1,), i32),
            pltpu.SemaphoreType.DMA((NSEM,)),
        ],
        compiler_params=pltpu.CompilerParams(vmem_limit_bytes=110 * 1024 * 1024, disable_bounds_checks=True),
    )(
        A_x.reshape(S, DM), A_mem0.reshape(M, DM),
        A_Wq.reshape(DM * H, DH), A_Wk.reshape(DM * H, DH), A_Wv.reshape(DM * H, DH),
        A_Wo.reshape(H * DH, DM),
        B_x.reshape(S, DM), B_wqkv, B_wo,
    )
    return out.reshape(1, S, 2 * DM)


def pallas_concat_heads__memory_aug_recurrent_mem_tr__sliding_local_dilated__prompt_kernel(
    A_x, A_mem0, A_Wq, A_Wk, A_Wv, A_Wo, A_seg_len, B_x, B_wqkv, B_wo,
):
    if isinstance(A_seg_len, int):
        assert A_seg_len == SEG
    return _run(A_x, A_mem0, A_Wq, A_Wk, A_Wv, A_Wo, B_x, B_wqkv, B_wo)
```

```python
import contextlib
import dataclasses
import functools

import jax
import jax.numpy as jnp
from jax import lax
import jax.experimental.pallas as pl
import jax.experimental.pallas.tpu as pltpu

bf16, f32, u32, i32 = jnp.bfloat16, jnp.float32, jnp.uint32, jnp.int32

S, DM = 2048, 1024
H, DH = 32, 128
M, SEG = 8, 32
L = M + SEG
DHB, WIN, DIL = 32, 8, 2
NC = DM // 128

TB = 64
UB = 4
HALO = 16
NIT = S // (TB * UB)
LQK, LPV, KA, NI = 1, 3, 12, 3

PITCH = 9
OPITCH = 65
HW = DM * H // 2
STG_AW, STG_BW, STG_BWO = 0, 6 * HW, 6 * HW + 24 * DM
STG_TOK = STG_BWO + NC * DM
STG_ROWS = STG_TOK + 64
NG = TB // 8
X_PART = UB * 24
X_PROB = X_PART + 2 * NG
X_OUT = X_PROB + 2 * NG
X_TMP = X_OUT + 2 * NG
X_FEN = X_TMP + 32
X_SLABS = X_FEN + 2

SEM_BW, SEM_BX, SEM_BWO, SEM_AW, SEM_AWO, SEM_AX, SEM_MEM, SEM_OB, SEM_OA = 0, 6, 9, 10, 16, 17, 18, 19, 20
NSEM = 21
_SCOPES = False


def _scope(name):
    return jax.named_scope(name) if _SCOPES else contextlib.nullcontext()


def _b16(v):
    return pltpu.bitcast(v, bf16)


def _u32(view):
    return view.bitcast(u32)[...]


def _lhs(blocks):
    return _b16(jnp.concatenate(blocks, axis=1))


def _kernel(ax_h, mem_h, wq_h, wk_h, wv_h, wo_h, bx_h, bw_h, bwo_h, out_h,
            ax_v, mem_v, stg_v, wa_v, wo_v, bx_v, bw_v, bwo_v, outa_v, outb_v,
            x_v, ob_v, mem_s, stash, ostash, o_s, zero_s, sem):
    P = functools.partial

    def bw_cps(s, half):
        return [pltpu.make_async_copy(bw_h.at[pl.ds(half * (DM // 2), DM // 2), pl.ds(128 * n, 128)],
                                      stg_v.at[pl.ds(STG_BW + DM * n + half * (DM // 2), DM // 2), :],
                                      sem.at[SEM_BW + 2 * s + half]) for n in range(8 * s, 8 * s + 8)]

    def bx_cps(part):
        rows = (pl.ds(0, TB * UB), pl.ds(TB * UB, TB * UB), pl.ds(2 * TB * UB, S - 2 * TB * UB))[part]
        return [pltpu.make_async_copy(bx_h.at[rows, pl.ds(128 * j, 128)], bx_v.at[j, rows, :],
                                      sem.at[SEM_BX + part]) for j in range(NC)]

    def bwo_cps():
        return [pltpu.make_async_copy(bwo_h.at[:, pl.ds(128 * n, 128)], stg_v.at[pl.ds(STG_BWO + DM * n, DM), :],
                                      sem.at[SEM_BWO]) for n in range(NC)]

    def aw_cp(c):
        src = (wq_h, wk_h, wv_h)[c // 2]
        return pltpu.make_async_copy(src.at[pl.ds((c % 2) * HW, HW), :], stg_v.at[pl.ds(STG_AW + c * HW, HW), :],
                                     sem.at[SEM_AW + c])

    def awo_cp(n):
        return pltpu.make_async_copy(wo_h.at[:, pl.ds(128 * n, 128)], wo_v.at[n], sem.at[SEM_AWO])

    def ax_cp(j):
        return pltpu.make_async_copy(ax_h.at[:, pl.ds(128 * j, 128)], ax_v.at[j], sem.at[SEM_AX])

    mem_cp = pltpu.make_async_copy(mem_h, mem_v, sem.at[SEM_MEM])

    def ob_cp(r0, n):
        return pltpu.make_async_copy(outb_v.at[pl.ds(r0, n), :], out_h.at[pl.ds(r0, n), pl.ds(DM, DM)],
                                     sem.at[SEM_OB])

    def oa_cp(r0, n):
        return pltpu.make_async_copy(outa_v.at[pl.ds(r0, n), :], out_h.at[pl.ds(r0, n), pl.ds(0, DM)],
                                     sem.at[SEM_OA])

    def start(cps):
        for c in cps:
            c.start()

    def wait(cps):
        for c in cps:
            c.wait()

    start(bw_cps(0, 0) + bw_cps(0, 1) + bx_cps(0) + bw_cps(1, 0) + bw_cps(1, 1))

    zero_s[0] = 0
    x_v[X_FEN + 1, 0:8, :] = jnp.zeros((8, 128), f32)

    def run(dots, fill):
        z = pl.multiple_of(zero_s[0], 64)
        busy = [False]

        def epoch(e, y, close):
            if y is not None and (e in fill or (close and busy[0])):
                x_v[z + X_FEN, 0:8, :] = y
                stg_v.at[pl.ds(z + STG_TOK, 16), :].bitcast(f32)[...] = x_v[X_FEN + 1, 0:8, :]
                busy[0] = False
            for f in fill.pop(e, []):
                f()
                busy[0] = True

        epoch(-1, None, False)
        for n, d in enumerate(dots):
            y, store = d()
            epoch(n - 0.5, y[0:8], False)
            store()
            epoch(n, y[TB - 8:TB], n < len(dots) - 1)
        assert not fill, sorted(fill)

    def put(fill, n, f):
        fill.setdefault(n, []).append(f)

    lane16 = lax.broadcasted_iota(i32, (16, 128), 1)

    def perm_select(s, half, k):
        bits = [((lane16 >> (b + 1)) & 1) == 1 for b in range(3)]
        for r in range(0, 64, 16):
            src = STG_BW + 8 * s * DM + 2 * (half * 256 + 64 * k + r)
            zs = [_u32(stg_v.at[pl.ds(src + ((-t) % 8) * DM, 32), :]) for t in range(8)]
            for b in range(3):
                zs = [lax.select(bits[b], zs[(t - (1 << b)) % 8], zs[t]) for t in range(8)]
            for u in range(8):
                x_v[X_TMP + 4 * u + k, r:r + 16, :] = pltpu.bitcast(zs[u], f32)

    def perm_gather(s, half, u, k0, k1):
        n = 64 * (k1 - k0)
        lane = lax.broadcasted_iota(i32, (n, 128), 1)
        idx = 32 * ((lane >> 3) & 3) + 16 * (lane >> 6) + 2 * ((u + lane) & 7) + ((lane >> 5) & 1)
        t = pltpu.bitcast(x_v[X_TMP + 4 * u + k0:X_TMP + 4 * u + k1, 0:64, :].reshape(n, 128), u32)
        bw_v[8 * s + u, half * 256 + 64 * k0:half * 256 + 64 * k1, :] = jnp.take_along_axis(t, idx, axis=1)

    def perm_fill(fill, s, half, e_sel, e_gat):
        for k in range(4):
            put(fill, e_sel[k], P(perm_select, s, half, k))
        for k in range(16):
            assert e_gat(k) > e_sel[2 * (k // 8) + 1]
            put(fill, e_gat(k), P(perm_gather, s, half, k % 8, 2 * (k // 8), 2 * (k // 8) + 2))

    def pack_pairs(a, b):
        return (a & jnp.uint32(0xFFFF)) | (b << 16), (a >> 16) | (b & jnp.uint32(0xFFFF0000))

    def prep_bwo(n, v):
        r = STG_BWO + n * DM + 128 * v
        a = _u32(stg_v.at[pl.ds(r, 128), :]).reshape(8, 8, 128)
        b = _u32(stg_v.at[pl.ds(r + 128, 128), :]).reshape(8, 8, 128)
        a = pltpu.roll(a, 8 - v, 1) if v else a
        lo, hi = pack_pairs(a, pltpu.roll(b, 7 - v, 1))
        for k in range(8):
            d = 32 * (k % 2) + 4 * (k // 2) + v // 2
            bwo_v[n, pl.ds(d, 8, stride=OPITCH), :] = lo[k]
            bwo_v[n, pl.ds(d + 16, 8, stride=OPITCH), :] = hi[k]

    scale_b = DHB ** -0.5

    def b_qkv_dots(i, st, n0, n1):
        r0 = i * TB
        if not isinstance(r0, int):
            r0 = pl.multiple_of(r0, TB)

        def dot(n):
            lhs = _lhs([_u32(bx_v.at[j, pl.ds(r0, TB), :]) for j in range(NC)])
            y = jnp.dot(lhs, _b16(bw_v[n]), preferred_element_type=f32)

            def store():
                x_v[st * 24 + n, HALO:HALO + TB, :] = y * scale_b if n < 8 else y
                if n >= 8:
                    x_v[((st + 1) % UB) * 24 + n, 0:HALO, :] = y[TB - HALO:TB]
            return y, store
        return [P(dot, n) for n in range(n0, n1)]

    def b_proj_dots(i, st):
        r0 = i * TB
        if not isinstance(r0, int):
            r0 = pl.multiple_of(r0, TB)

        def dot(n):
            lhs = _lhs([_u32(ob_v.at[st, j]) for j in range(NC)])
            w = _b16(jnp.concatenate([bwo_v[n, OPITCH * u:OPITCH * u + 64, :] for u in range(8)], axis=0))
            y = jnp.dot(lhs, w, preferred_element_type=f32)

            def store():
                outb_v[pl.ds(r0, TB), 128 * n:128 * n + 128] = y.astype(bf16)
            return y, store
        return [P(dot, n) for n in range(NC)]

    def rows8(s0, r):
        return x_v[s0:s0 + 8, r:r + 8, :]

    def pos_ok(g, w):
        return lax.broadcasted_iota(i32, (8, 8, 128), 1) + (8 * g) - DIL * w >= 0

    def at_qk(st, g, half):
        q = rows8(st * 24, HALO + 8 * g)
        p = [jnp.sum(q * rows8(st * 24 + 8, HALO + 8 * g - DIL * w), axis=0) for w in range(4 * half, 4 * half + 4)]
        x_v[X_PART + (st % 2) * NG + g, 32 * half:32 * half + 32, :] = jnp.concatenate(p, axis=0)

    def at_softmax(st, g, first, pend):
        p = x_v[X_PART + (st % 2) * NG + g, 0:64, :]
        p = p + pltpu.roll(p, 32, 1)
        p = (p + pltpu.roll(p, 64, 1)).reshape(WIN, 8, 128)
        if first and 8 * g < DIL * (WIN - 1):
            p = jnp.where(pos_ok(g, lax.broadcasted_iota(i32, (8, 8, 128), 0)), p, -1e9)
        e = jnp.exp(p - jnp.max(p, axis=0, keepdims=True))
        l = jnp.sum(e, axis=0, keepdims=True)
        rc = pl.reciprocal(l, approx=True)
        pend[st, g] = e * (rc * (2.0 - l * rc))

    def at_store(st, g, pend):
        x_v[X_PROB + (st % 2) * NG + g, 0:64, :] = pend.pop((st, g)).reshape(64, 128)

    def at_pv(st, g, first, half):
        acc = None
        s0 = st * 24 + 16 + 4 * half
        for w in range(WIN):
            e = x_v[X_PROB + (st % 2) * NG + g:X_PROB + (st % 2) * NG + g + 1, 8 * w:8 * w + 8, :]
            r = HALO + 8 * g - DIL * w
            vv = x_v[s0:s0 + 4, r:r + 8, :]
            if first and 8 * g - DIL * w < 0:
                vv = jnp.where(pos_ok(g, w)[0:4], vv, x_v[s0:s0 + 4, HALO:HALO + 1, :])
            acc = e * vv if acc is None else acc + e * vv
        x_v[X_OUT + (st % 2) * NG + g, 32 * half:32 * half + 32, :] = acc.reshape(32, 128)

    def at_pack(st, g):
        o = [x_v[X_OUT + (st % 2) * NG + k, 0:64, :].reshape(8, 8, 128) for k in (g - 1, g)]
        ob_v[st, :, 8 * g - 8:8 * g + 8, :] = jnp.concatenate(o, axis=1).astype(bf16)

    pend = {}

    def attn_fill(fill, st, first, e_qk, e_sm, e_pv, step):
        for g, e in e_qk.items():
            put(fill, e, P(at_qk, st, g, 0))
            put(fill, e + step, P(at_qk, st, g, 1))
        for g, e in e_sm.items():
            put(fill, e, P(at_softmax, st, g, first, pend))
            put(fill, e + 3, P(at_store, st, g, pend))
        for g, e in e_pv.items():
            put(fill, e, P(at_pv, st, g, first, 0))
            put(fill, e + step, P(at_pv, st, g, first, 1))
            if g % 2 == 1:
                put(fill, e + 2 * step, P(at_pack, st, g))

    def ramp(e0, per, g0=0, g1=NG):
        return {g: e0 + per * g for g in range(g0, g1)}

    def a_relayout(src0, dst0, g):
        src = stg_v.at[pl.ds(pl.multiple_of(src0, 512), HW), :].bitcast(u32)
        dst = wa_v.at[pl.ds(dst0, DM // 32)]
        t = src[64 * g:64 * g + 64, :].reshape(2, 4, 8, 128)
        ev, od = pack_pairs(t[:, 0:2], t[:, 2:4])
        for dp in range(2):
            r = 2 * (g % 4) + dp
            for o in range(2):
                dst[g // 4, pl.ds(8 * o * PITCH + r, 8, stride=PITCH), :] = ev[dp, o]
                dst[g // 4, pl.ds((16 + 8 * o) * PITCH + r, 8, stride=PITCH), :] = od[dp, o]

    def sec(k0, k1, s):
        return [d for k in range(k0, k1) for d in b_qkv_dots(k, k, 8 * s, 8 * s + 8)]

    with _scope("perm_q"):
        x_v[8:24, 0:HALO, :] = jnp.zeros((16, HALO, 128), f32)
        for half in range(2):
            wait(bw_cps(0, half))
            if half == 0:
                start(bw_cps(2, 0) + bw_cps(2, 1) + bwo_cps() + bx_cps(1))
            for k in range(4):
                perm_select(0, half, k)
            for u in range(8):
                perm_gather(0, half, u, 0, 4)
    with _scope("Q01"):
        wait(bx_cps(0))
        run(sec(0, 2, 0), {})
    with _scope("Q2"):
        wait(bw_cps(1, 0))
        fill = {}
        perm_fill(fill, 1, 0, (-1, -1, -0.5, 0.5), lambda k: (2 * k // 3 - 1) / 2)
        run(sec(2, 3, 0), fill)
    with _scope("Q3K0"):
        wait(bw_cps(1, 1))
        start(bx_cps(2) + [aw_cp(0), mem_cp])
        fill = {}
        perm_fill(fill, 1, 1, (-1, -1, -0.5, 0.5), lambda k: (2 * k // 3 - 1) / 2)
        run(sec(3, 4, 0) + sec(0, 1, 1), fill)
    with _scope("K12"):
        wait(bw_cps(2, 0))
        fill = {}
        perm_fill(fill, 2, 0, (-1, -1, 0, 1), lambda k: 3 * k // 4 + 1)
        attn_fill(fill, 0, True, ramp(2, 1.5), {}, {}, 0.5)
        run(sec(1, 3, 1), fill)
    with _scope("K3V01"):
        wait(bw_cps(2, 1))
        fill = {}
        perm_fill(fill, 2, 1, (-1, -1, -0.5, 0.5), lambda k: (2 * k // 3 - 1) / 2)
        attn_fill(fill, 0, True, {}, ramp(5, 1), ramp(15, 1, 0, NG - 1), 0.5)
        attn_fill(fill, 1, False, ramp(2, 1.5), ramp(12, 1), {}, 0.5)
        run(sec(3, 4, 1) + sec(0, 2, 2), fill)
    with _scope("V23"):
        wait(bwo_cps())
        fill = {}
        attn_fill(fill, 0, True, {}, {}, {NG - 1: -1}, 0.5)
        attn_fill(fill, 1, False, {}, {}, ramp(0.5, 2, 0, NG - 1), 1)
        attn_fill(fill, 2, False, {0: -1}, {}, {}, 0)
        for n in range(4 * NC):
            put(fill, (n * 30 // 32 - 1) / 2, P(prep_bwo, n // 4, 2 * (n % 4)))
        run(sec(2, 4, 2), fill)

    def b_body(it, carry):
        with _scope("it"):
            for c in (1, 2):
                @pl.when(it == c)
                def _():
                    wait(bx_cps(c))

            @pl.when(it >= 2)
            def _():
                cw = jnp.maximum(it - 2, 0)
                dst = stg_v.at[pl.ds(pl.multiple_of(STG_AW + cw * HW, HW), HW), :]
                pltpu.make_async_copy(dst, dst, sem.at[SEM_AW + cw]).wait()

            for c in range(1, NIT):
                @pl.when(it == c)
                def _():
                    cols = {6: (5, 6, 7), 7: ()}.get(c, (c - 1,))
                    start(([ob_cp(UB * TB * (c - 2), UB * TB)] if c >= 2 else []) + ([aw_cp(c)] if c < 6 else [])
                          + [cp(n) for n in cols for cp in (awo_cp, ax_cp)])
            c = jnp.maximum(it - 2, 0)
            src0 = jnp.where(it == 1, STG_BW, STG_AW + c * HW)
            dst0 = c * (DM // 32)
            dots, fill = [], {}
            for k in range(UB):
                i, e0 = UB * it + k, 32 * k
                dots += b_qkv_dots(i, k, 0, 24) + b_proj_dots(i - 4, k)
                e0 -= 1
                attn_fill(fill, (k - 3) % UB, False, {}, {}, {NG - 1: e0}, 1)
                attn_fill(fill, (k - 2) % UB, False, ramp(e0 - 2, 4, 1), ramp(e0, 4), ramp(e0 + 4, 4, 0, NG - 1), 1)
                attn_fill(fill, (k - 1) % UB, False, {0: e0 + 30}, {}, {}, 1)
                for g in range(32):
                    put(fill, e0 + g + 0.5, P(a_relayout, src0, dst0, 32 * k + g))
            run(dots, fill)
        return carry
    lax.fori_loop(1, NIT, b_body, 0)
    nb = S // TB
    wait([awo_cp(n) for n in range(NC)] + [ax_cp(j) for j in range(NC)] + [mem_cp])
    with _scope("tailB"):
        ob_cp(S - 2 * UB * TB, UB * TB).start()
        fill = {}
        attn_fill(fill, 1, False, {}, {}, {NG - 1: -1}, 0.5)
        attn_fill(fill, 2, False, ramp(-2, 1, 1), ramp(-1, 1), ramp(6, 1), 0.5)
        attn_fill(fill, 3, False, ramp(1, 2), {}, {}, 1)
        attn_fill(fill, 3, False, {}, ramp(10, 1), ramp(14, 1), 0.5)
        run([d for k in range(UB) for d in b_proj_dots(nb - 4 + k, k)], fill)
        ob_cp(S - UB * TB, UB * TB).start()


    scale_a = DH ** -0.5
    rr = lax.broadcasted_iota(i32, (2 * L, 2 * L), 0)
    cc = lax.broadcasted_iota(i32, (2 * L, 2 * L), 1)
    rb_, cb_ = rr >= L, cc >= L
    ri, ci = jnp.where(rb_, rr - L, rr), jnp.where(cb_, cc - L, cc)
    same = rb_ == cb_
    valid = same & ((ri < M) | (ri >= ci))
    fill = jnp.where(same, -1e9, -jnp.inf).astype(f32)

    mem_s[...] = mem_v[...].astype(f32)
    NP = H // 2

    def a_step(lhs, even):
        qkv, pp = {}, {}
        nrow = 32 if even else 48

        def proj(wh, k0, k1):
            s0, r = (wh // H) * (DM // 16), ((wh % H) // 2 + (H // 2) * (wh % 2)) * PITCH
            w = wa_v[s0 + k0 // 16:s0 + k1 // 16, r:r + 8, :].reshape((k1 - k0) // 2, 128)
            return jnp.dot(lhs[:, k0:k1], _b16(w), preferred_element_type=f32)

        def do_qkv(j, after_dot):
            split = j == 0 and not even
            lo = {wi * H + hh: proj(wi * H + hh, 0, DM // 2) for hh in (0, 1) for wi in range(3)} if split else {}
            parts = [[], [], []]
            for hh in (2 * j, 2 * j + 1):
                for wi in range(3):
                    wh = wi * H + hh
                    y = proj(wh, DM // 2, DM) + lo[wh] if split else proj(wh, 0, DM)
                    if even:
                        stash[wh] = y[32:40]
                        parts[wi] += [y[40:48], y[0:32]]
                    else:
                        parts[wi] += [y[0:8], stash[wh], y[8:32]]
                    after_dot(3 * hh + wi)
            qkv[j] = [jnp.concatenate(p, axis=0).astype(bf16) for p in parts]

        def do_qk(j):
            q2, k2, _ = qkv[j]
            s = lax.dot_general(q2, k2, (((1,), (1,)), ((), ())), preferred_element_type=f32) * scale_a
            s = jnp.where(valid, s, fill)
            m = jnp.max(s, axis=1, keepdims=True)
            e = jnp.exp(s - m)
            l = jnp.sum(e, axis=1, keepdims=True)
            rc = pl.reciprocal(l, approx=True)
            rc = rc * (2.0 - l * rc)
            pp[j] = (e * rc).astype(bf16)

        def do_pv(j):
            o2 = jnp.dot(pp.pop(j), qkv.pop(j)[2], preferred_element_type=f32)
            for i, hh in enumerate((2 * j, 2 * j + 1)):
                o = o2[L * i:L * (i + 1)]
                if even:
                    o_s[hh, 0:32, :] = o[0:32].astype(bf16)
                    ostash[hh] = o[32:40]
                else:
                    o_s[hh] = jnp.concatenate([o[0:8], ostash[hh], o[8:40]], axis=0).astype(bf16)

        ya = {}

        def wo_part(n, h0, h1):
            lo = _lhs([_u32(o_s.at[hh, pl.ds(0, nrow), :]) for hh in range(h0, h1)])
            w = _u32(wo_v.at[n, pl.ds(h0 * DH, (h1 - h0) * DH), :])
            r = jnp.dot(lo, _b16(w), preferred_element_type=f32)
            ya[n] = r + ya[n] if n in ya else r

        ni = 0 if even else NI
        pieces = [(n, 4 * g, 4 * g + 4) for g in range(ni) for n in range(NC)]
        d0 = 6 * (LPV + 2)
        done = []

        def after_dot(d):
            ready = NC * max(((d + 1) // 6 - LPV - 1 + (1 if (d + 1) % 6 else 0)) // 2, 0)
            while len(done) < min((d - d0 + 1) * len(pieces) // (3 * H - d0), ready):
                wo_part(*pieces[len(done)])
                done.append(0)

        for j in range(NP):
            do_qkv(j, after_dot)
            if j - LQK >= 0:
                do_qk(j - LQK)
            if j - LPV >= 0:
                do_pv(j - LPV)
        assert len(done) == len(pieces)
        nper, n = NC // (LPV + 1), 0
        for j in range(NP, NP + LPV):
            for _ in range(nper):
                wo_part(n, 4 * ni, 2 * KA)
                n += 1
            if j - LQK < NP:
                do_qk(j - LQK)
            do_pv(j - LPV)
        for n in range(n, NC):
            wo_part(n, 4 * ni, 2 * KA)
        for n in range(NC):
            wo_part(n, 2 * KA, H)
        return jnp.concatenate([ya[n] for n in range(NC)], axis=1)

    def a_body(t, c):
        with _scope("a_it"):
            return a_pair(t, c)

    def a_pair(t, c):
        @pl.when(t > 0)
        def _():
            oa_cp(pl.multiple_of(jnp.maximum(t - 1, 0) * 64, 64), 64).start()
        o0 = pl.multiple_of(t * 64, 64)
        X = _lhs([_u32(ax_v.at[j, pl.ds(o0, 64), :]) for j in range(NC)])
        Xm = X[32:48].astype(f32)
        mixed = jnp.concatenate([Xm[0:8], mem_s[...]], axis=0).astype(bf16)
        ye = a_step(jnp.concatenate([X[0:32], mixed], axis=0), True)
        mixed = jnp.concatenate([ye[0:8], Xm[8:16]], axis=0).astype(bf16)
        yo = a_step(jnp.concatenate([mixed, X[48:64]], axis=0), False)
        mem_s[...] = yo[0:8]
        outa_v[pl.ds(o0, 64), :] = jnp.concatenate([ye[8:32], yo[8:48]], axis=0).astype(bf16)
        return c
    lax.fori_loop(0, S // 64, a_body, 0)
    oa_cp(S - 64, 64).start()

    ob_cp(0, S).wait()
    oa_cp(0, S).wait()


@jax.jit
def _run(A_x, A_mem0, A_Wq, A_Wk, A_Wv, A_Wo, B_x, B_wqkv, B_wo):
    hbm = pl.BlockSpec(memory_space=pl.ANY)
    known = {f.name for f in dataclasses.fields(pltpu.CompilerParams)}
    optional = {k: True for k in ("disable_bounds_checks", "disable_semaphore_checks") if k in known}
    out = pl.pallas_call(
        _kernel,
        out_shape=jax.ShapeDtypeStruct((S, 2 * DM), bf16),
        in_specs=[hbm] * 9,
        out_specs=hbm,
        scratch_shapes=[
            pltpu.VMEM((NC, S, 128), bf16),
            pltpu.VMEM((M, DM), bf16),
            pltpu.VMEM((STG_ROWS, 128), bf16),
            pltpu.VMEM((3 * DM // 16, H * PITCH + 8, 128), u32),
            pltpu.VMEM((NC, H * DH, 128), bf16),
            pltpu.VMEM((NC, S, 128), bf16),
            pltpu.VMEM((24, DM // 2, 128), u32),
            pltpu.VMEM((NC, 9 * OPITCH - 1, 128), u32),
            pltpu.VMEM((S, DM), bf16),
            pltpu.VMEM((S, DM), bf16),
            pltpu.VMEM((X_SLABS, TB + HALO, 128), f32),
            pltpu.VMEM((UB, 8, TB, 128), bf16),
            pltpu.VMEM((M, DM), f32),
            pltpu.VMEM((3 * H, 8, DH), f32),
            pltpu.VMEM((H, 8, DH), f32),
            pltpu.VMEM((H, 48, DH), bf16),
            pltpu.SMEM((1,), i32),
            pltpu.SemaphoreType.DMA((NSEM,)),
        ],
        compiler_params=pltpu.CompilerParams(vmem_limit_bytes=110 * 1024 * 1024, **optional),
    )(
        A_x.reshape(S, DM), A_mem0.reshape(M, DM),
        A_Wq.reshape(DM * H, DH), A_Wk.reshape(DM * H, DH), A_Wv.reshape(DM * H, DH),
        A_Wo.reshape(H * DH, DM),
        B_x.reshape(S, DM), B_wqkv, B_wo,
    )
    return out.reshape(1, S, 2 * DM)


def pallas_concat_heads__memory_aug_recurrent_mem_tr__sliding_local_dilated__prompt_kernel(
    A_x, A_mem0, A_Wq, A_Wk, A_Wv, A_Wo, A_seg_len, B_x, B_wqkv, B_wo,
):
    if isinstance(A_seg_len, int):
        assert A_seg_len == SEG
    return _run(A_x, A_mem0, A_Wq, A_Wk, A_Wv, A_Wo, B_x, B_wqkv, B_wo)
```

```python
import contextlib
import dataclasses
import functools

import jax
import jax.numpy as jnp
from jax import lax
import jax.experimental.pallas as pl
import jax.experimental.pallas.tpu as pltpu

bf16, f32, u32, i32 = jnp.bfloat16, jnp.float32, jnp.uint32, jnp.int32

S, DM = 2048, 1024
H, DH = 32, 128
M, SEG = 8, 32
L = M + SEG
DHB, WIN, DIL = 32, 8, 2
NC = DM // 128

TB = 64
UB = 4
HALO = 16
NIT = S // (TB * UB)
LQK, LPV, KA = 1, 3, 12
NI = (3, 4)
NK0 = 2 * M
RM = L - 8
AQ, AK, AV, AM, AO, AROWS = 0, 16, 40, 56, 64, 96
LOG2E = 1.4426950408889634

PITCH = 9
OPITCH = 65
HW = DM * H // 2
STG_AW, STG_BW, STG_BWO = 0, 6 * HW, 6 * HW + 24 * DM
STG_TOK = STG_BWO + NC * DM
STG_ROWS = STG_TOK + 64
NG = TB // 8
X_PART = UB * 24
X_PROB = X_PART + 2 * NG
X_OUT = X_PROB + 2 * NG
X_TMP = X_OUT + 2 * NG
X_FEN = X_TMP + 32
X_SLABS = X_FEN + 2

SEM_BW, SEM_BX, SEM_BWO, SEM_AW, SEM_AWO, SEM_AX, SEM_MEM, SEM_OB, SEM_OA = 0, 6, 9, 10, 16, 17, 18, 19, 20
NSEM = 21
_SCOPES = False


def _scope(name):
    return jax.named_scope(name) if _SCOPES else contextlib.nullcontext()


def _b16(v):
    return pltpu.bitcast(v, bf16)


def _u32(view):
    return view.bitcast(u32)[...]


def _lhs(blocks):
    return _b16(jnp.concatenate(blocks, axis=1))


def _kernel(ax_h, mem_h, wq_h, wk_h, wv_h, wo_h, bx_h, bw_h, bwo_h, out_h,
            ax_v, mem_v, stg_v, wa_v, wo_v, bx_v, bw_v, bwo_v, outa_v, outb_v,
            x_v, ob_v, mem_s, stash, ostash, o_s, xa_v, sa_v, zero_s, sem):
    P = functools.partial

    def bw_cps(s, half):
        return [pltpu.make_async_copy(bw_h.at[pl.ds(half * (DM // 2), DM // 2), pl.ds(128 * n, 128)],
                                      stg_v.at[pl.ds(STG_BW + DM * n + half * (DM // 2), DM // 2), :],
                                      sem.at[SEM_BW + 2 * s + half]) for n in range(8 * s, 8 * s + 8)]

    def bx_cps(part):
        rows = (pl.ds(0, TB * UB), pl.ds(TB * UB, TB * UB), pl.ds(2 * TB * UB, S - 2 * TB * UB))[part]
        return [pltpu.make_async_copy(bx_h.at[rows, pl.ds(128 * j, 128)], bx_v.at[j, rows, :],
                                      sem.at[SEM_BX + part]) for j in range(NC)]

    def bwo_cps():
        return [pltpu.make_async_copy(bwo_h.at[:, pl.ds(128 * n, 128)], stg_v.at[pl.ds(STG_BWO + DM * n, DM), :],
                                      sem.at[SEM_BWO]) for n in range(NC)]

    def aw_cp(c):
        src = (wq_h, wk_h, wv_h)[c // 2]
        return pltpu.make_async_copy(src.at[pl.ds((c % 2) * HW, HW), :], stg_v.at[pl.ds(STG_AW + c * HW, HW), :],
                                     sem.at[SEM_AW + c])

    def awo_cp(n):
        return pltpu.make_async_copy(wo_h.at[:, pl.ds(128 * n, 128)], wo_v.at[n], sem.at[SEM_AWO])

    def ax_cp(j):
        return pltpu.make_async_copy(ax_h.at[:, pl.ds(128 * j, 128)], ax_v.at[j], sem.at[SEM_AX])

    mem_cp = pltpu.make_async_copy(mem_h, mem_v, sem.at[SEM_MEM])

    def ob_cp(r0, n):
        return pltpu.make_async_copy(outb_v.at[pl.ds(r0, n), :], out_h.at[pl.ds(r0, n), pl.ds(DM, DM)],
                                     sem.at[SEM_OB])

    def oa_cp(r0, n):
        return pltpu.make_async_copy(outa_v.at[pl.ds(r0, n), :], out_h.at[pl.ds(r0, n), pl.ds(0, DM)],
                                     sem.at[SEM_OA])

    def start(cps):
        for c in cps:
            c.start()

    def wait(cps):
        for c in cps:
            c.wait()

    start(bw_cps(0, 0) + bw_cps(0, 1) + bx_cps(0) + bw_cps(1, 0) + bw_cps(1, 1))

    zero_s[0] = 0
    x_v[X_FEN + 1, 0:8, :] = jnp.zeros((8, 128), f32)

    def run(dots, fill):
        z = pl.multiple_of(zero_s[0], 64)
        busy = [False]

        def epoch(e, y, close):
            if y is not None and (e in fill or (close and busy[0])):
                x_v[z + X_FEN, 0:8, :] = y
                stg_v.at[pl.ds(z + STG_TOK, 16), :].bitcast(f32)[...] = x_v[X_FEN + 1, 0:8, :]
                busy[0] = False
            for f in fill.pop(e, []):
                f()
                busy[0] = True

        epoch(-1, None, False)
        for n, d in enumerate(dots):
            y, store = d()
            epoch(n - 0.5, y[0:8], False)
            store()
            epoch(n, y[TB - 8:TB], n < len(dots) - 1)
        assert not fill, sorted(fill)

    def put(fill, n, f):
        fill.setdefault(n, []).append(f)

    lane16 = lax.broadcasted_iota(i32, (16, 128), 1)

    def perm_select(s, half, k):
        bits = [((lane16 >> (b + 1)) & 1) == 1 for b in range(3)]
        for r in range(0, 64, 16):
            src = STG_BW + 8 * s * DM + 2 * (half * 256 + 64 * k + r)
            zs = [_u32(stg_v.at[pl.ds(src + ((-t) % 8) * DM, 32), :]) for t in range(8)]
            for b in range(3):
                zs = [lax.select(bits[b], zs[(t - (1 << b)) % 8], zs[t]) for t in range(8)]
            for u in range(8):
                x_v[X_TMP + 4 * u + k, r:r + 16, :] = pltpu.bitcast(zs[u], f32)

    def perm_gather(s, half, u, k0, k1):
        n = 64 * (k1 - k0)
        lane = lax.broadcasted_iota(i32, (n, 128), 1)
        idx = 32 * ((lane >> 3) & 3) + 16 * (lane >> 6) + 2 * ((u + lane) & 7) + ((lane >> 5) & 1)
        t = pltpu.bitcast(x_v[X_TMP + 4 * u + k0:X_TMP + 4 * u + k1, 0:64, :].reshape(n, 128), u32)
        bw_v[8 * s + u, half * 256 + 64 * k0:half * 256 + 64 * k1, :] = jnp.take_along_axis(t, idx, axis=1)

    def perm_fill(fill, s, half, e_sel, e_gat):
        for k in range(4):
            put(fill, e_sel[k], P(perm_select, s, half, k))
        for k in range(16):
            assert e_gat(k) > e_sel[2 * (k // 8) + 1]
            put(fill, e_gat(k), P(perm_gather, s, half, k % 8, 2 * (k // 8), 2 * (k // 8) + 2))

    def pack_pairs(a, b):
        return (a & jnp.uint32(0xFFFF)) | (b << 16), (a >> 16) | (b & jnp.uint32(0xFFFF0000))

    def prep_bwo(n, v):
        r = STG_BWO + n * DM + 128 * v
        a = _u32(stg_v.at[pl.ds(r, 128), :]).reshape(8, 8, 128)
        b = _u32(stg_v.at[pl.ds(r + 128, 128), :]).reshape(8, 8, 128)
        a = pltpu.roll(a, 8 - v, 1) if v else a
        lo, hi = pack_pairs(a, pltpu.roll(b, 7 - v, 1))
        for k in range(8):
            d = 32 * (k % 2) + 4 * (k // 2) + v // 2
            bwo_v[n, pl.ds(d, 8, stride=OPITCH), :] = lo[k]
            bwo_v[n, pl.ds(d + 16, 8, stride=OPITCH), :] = hi[k]

    scale_b = DHB ** -0.5

    def b_qkv_dots(i, st, n0, n1):
        r0 = i * TB
        if not isinstance(r0, int):
            r0 = pl.multiple_of(r0, TB)

        def dot(n):
            lhs = _lhs([_u32(bx_v.at[j, pl.ds(r0, TB), :]) for j in range(NC)])
            y = jnp.dot(lhs, _b16(bw_v[n]), preferred_element_type=f32)

            def store():
                x_v[st * 24 + n, HALO:HALO + TB, :] = y * scale_b if n < 8 else y
                if n >= 8:
                    x_v[((st + 1) % UB) * 24 + n, 0:HALO, :] = y[TB - HALO:TB]
            return y, store
        return [P(dot, n) for n in range(n0, n1)]

    def b_proj_dots(i, st):
        r0 = i * TB
        if not isinstance(r0, int):
            r0 = pl.multiple_of(r0, TB)

        def dot(n):
            lhs = _lhs([_u32(ob_v.at[st, j]) for j in range(NC)])
            w = _b16(jnp.concatenate([bwo_v[n, OPITCH * u:OPITCH * u + 64, :] for u in range(8)], axis=0))
            y = jnp.dot(lhs, w, preferred_element_type=f32)

            def store():
                outb_v[pl.ds(r0, TB), 128 * n:128 * n + 128] = y.astype(bf16)
            return y, store
        return [P(dot, n) for n in range(NC)]

    def rows8(s0, r):
        return x_v[s0:s0 + 8, r:r + 8, :]

    def pos_ok(g, w):
        return lax.broadcasted_iota(i32, (8, 8, 128), 1) + (8 * g) - DIL * w >= 0

    def at_qk(st, g, half):
        q = rows8(st * 24, HALO + 8 * g)
        p = [jnp.sum(q * rows8(st * 24 + 8, HALO + 8 * g - DIL * w), axis=0) for w in range(4 * half, 4 * half + 4)]
        x_v[X_PART + (st % 2) * NG + g, 32 * half:32 * half + 32, :] = jnp.concatenate(p, axis=0)

    def at_softmax(st, g, first, pend):
        p = x_v[X_PART + (st % 2) * NG + g, 0:64, :]
        p = p + pltpu.roll(p, 32, 1)
        p = (p + pltpu.roll(p, 64, 1)).reshape(WIN, 8, 128)
        if first and 8 * g < DIL * (WIN - 1):
            p = jnp.where(pos_ok(g, lax.broadcasted_iota(i32, (8, 8, 128), 0)), p, -1e9)
        e = jnp.exp(p - jnp.max(p, axis=0, keepdims=True))
        l = jnp.sum(e, axis=0, keepdims=True)
        rc = pl.reciprocal(l, approx=True)
        pend[st, g] = e * (rc * (2.0 - l * rc))

    def at_store(st, g, pend):
        x_v[X_PROB + (st % 2) * NG + g, 0:64, :] = pend.pop((st, g)).reshape(64, 128)

    def at_pv(st, g, first, half):
        acc = None
        s0 = st * 24 + 16 + 4 * half
        for w in range(WIN):
            e = x_v[X_PROB + (st % 2) * NG + g:X_PROB + (st % 2) * NG + g + 1, 8 * w:8 * w + 8, :]
            r = HALO + 8 * g - DIL * w
            vv = x_v[s0:s0 + 4, r:r + 8, :]
            if first and 8 * g - DIL * w < 0:
                vv = jnp.where(pos_ok(g, w)[0:4], vv, x_v[s0:s0 + 4, HALO:HALO + 1, :])
            acc = e * vv if acc is None else acc + e * vv
        x_v[X_OUT + (st % 2) * NG + g, 32 * half:32 * half + 32, :] = acc.reshape(32, 128)

    def at_pack(st, g):
        o = [x_v[X_OUT + (st % 2) * NG + k, 0:64, :].reshape(8, 8, 128) for k in (g - 1, g)]
        ob_v[st, :, 8 * g - 8:8 * g + 8, :] = jnp.concatenate(o, axis=1).astype(bf16)

    pend = {}

    def attn_fill(fill, st, first, e_qk, e_sm, e_pv, step):
        for g, e in e_qk.items():
            put(fill, e, P(at_qk, st, g, 0))
            put(fill, e + step, P(at_qk, st, g, 1))
        for g, e in e_sm.items():
            put(fill, e, P(at_softmax, st, g, first, pend))
            put(fill, e + 3, P(at_store, st, g, pend))
        for g, e in e_pv.items():
            put(fill, e, P(at_pv, st, g, first, 0))
            put(fill, e + step, P(at_pv, st, g, first, 1))
            if g % 2 == 1:
                put(fill, e + 2 * step, P(at_pack, st, g))

    def ramp(e0, per, g0=0, g1=NG):
        return {g: e0 + per * g for g in range(g0, g1)}

    def a_relayout(src0, dst0, g):
        src = stg_v.at[pl.ds(pl.multiple_of(src0, 512), HW), :].bitcast(u32)
        dst = wa_v.at[pl.ds(dst0, DM // 32)]
        t = src[64 * g:64 * g + 64, :].reshape(2, 4, 8, 128)
        ev, od = pack_pairs(t[:, 0:2], t[:, 2:4])
        for dp in range(2):
            r = 2 * (g % 4) + dp
            for o in range(2):
                dst[g // 4, pl.ds(8 * o * PITCH + r, 8, stride=PITCH), :] = ev[dp, o]
                dst[g // 4, pl.ds((16 + 8 * o) * PITCH + r, 8, stride=PITCH), :] = od[dp, o]

    def a_weight(wh, k0, k1):
        s0, r = (wh // H) * (DM // 16), ((wh % H) // 2 + (H // 2) * (wh % 2)) * PITCH
        return _b16(wa_v[s0 + k0 // 16:s0 + k1 // 16, r:r + 8, :].reshape((k1 - k0) // 2, 128))

    def sec(k0, k1, s):
        return [d for k in range(k0, k1) for d in b_qkv_dots(k, k, 8 * s, 8 * s + 8)]

    with _scope("perm_q"):
        x_v[8:24, 0:HALO, :] = jnp.zeros((16, HALO, 128), f32)
        for half in range(2):
            wait(bw_cps(0, half))
            if half == 0:
                start(bw_cps(2, 0) + bw_cps(2, 1) + bwo_cps() + bx_cps(1))
            for k in range(4):
                perm_select(0, half, k)
            for u in range(8):
                perm_gather(0, half, u, 0, 4)
    with _scope("Q01"):
        wait(bx_cps(0))
        run(sec(0, 2, 0), {})
    with _scope("Q2"):
        wait(bw_cps(1, 0))
        fill = {}
        perm_fill(fill, 1, 0, (-1, -1, -0.5, 0.5), lambda k: (2 * k // 3 - 1) / 2)
        run(sec(2, 3, 0), fill)
    with _scope("Q3K0"):
        wait(bw_cps(1, 1))
        start(bx_cps(2) + [aw_cp(0), mem_cp])
        fill = {}
        perm_fill(fill, 1, 1, (-1, -1, -0.5, 0.5), lambda k: (2 * k // 3 - 1) / 2)
        run(sec(3, 4, 0) + sec(0, 1, 1), fill)
    with _scope("K12"):
        wait(bw_cps(2, 0))
        fill = {}
        perm_fill(fill, 2, 0, (-1, -1, 0, 1), lambda k: 3 * k // 4 + 1)
        attn_fill(fill, 0, True, ramp(2, 1.5), {}, {}, 0.5)
        run(sec(1, 3, 1), fill)
    with _scope("K3V01"):
        wait(bw_cps(2, 1))
        fill = {}
        perm_fill(fill, 2, 1, (-1, -1, -0.5, 0.5), lambda k: (2 * k // 3 - 1) / 2)
        attn_fill(fill, 0, True, {}, ramp(5, 1), ramp(15, 1, 0, NG - 1), 0.5)
        attn_fill(fill, 1, False, ramp(2, 1.5), ramp(12, 1), {}, 0.5)
        run(sec(3, 4, 1) + sec(0, 2, 2), fill)
    with _scope("V23"):
        wait(bwo_cps())
        fill = {}
        attn_fill(fill, 0, True, {}, {}, {NG - 1: -1}, 0.5)
        attn_fill(fill, 1, False, {}, {}, ramp(0.5, 2, 0, NG - 1), 1)
        attn_fill(fill, 2, False, {0: -1}, {}, {}, 0)
        for n in range(4 * NC):
            put(fill, (n * 30 // 32 - 1) / 2, P(prep_bwo, n // 4, 2 * (n % 4)))
        run(sec(2, 4, 2), fill)

    def b_body(it, carry):
        with _scope("it"):
            for c in (1, 2):
                @pl.when(it == c)
                def _():
                    wait(bx_cps(c))

            @pl.when(it >= 2)
            def _():
                cw = jnp.maximum(it - 2, 0)
                dst = stg_v.at[pl.ds(pl.multiple_of(STG_AW + cw * HW, HW), HW), :]
                pltpu.make_async_copy(dst, dst, sem.at[SEM_AW + cw]).wait()

            for c in range(1, NIT):
                @pl.when(it == c)
                def _():
                    cols = {6: (5, 6, 7), 7: ()}.get(c, (c - 1,))
                    start(([ob_cp(UB * TB * (c - 2), UB * TB)] if c >= 2 else []) + ([aw_cp(c)] if c < 6 else [])
                          + [cp(n) for n in cols for cp in (awo_cp, ax_cp)])
            c = jnp.maximum(it - 2, 0)
            src0 = jnp.where(it == 1, STG_BW, STG_AW + c * HW)
            dst0 = c * (DM // 32)
            dots, fill = [], {}
            for k in range(UB):
                i, e0 = UB * it + k, 32 * k
                dots += b_qkv_dots(i, k, 0, 24) + b_proj_dots(i - 4, k)
                e0 -= 1
                attn_fill(fill, (k - 3) % UB, False, {}, {}, {NG - 1: e0}, 1)
                attn_fill(fill, (k - 2) % UB, False, ramp(e0 - 2, 4, 1), ramp(e0, 4), ramp(e0 + 4, 4, 0, NG - 1), 1)
                attn_fill(fill, (k - 1) % UB, False, {0: e0 + 30}, {}, {}, 1)
                for g in range(32):
                    put(fill, e0 + g + 0.5, P(a_relayout, src0, dst0, 32 * k + g))
            run(dots, fill)
        return carry
    lax.fori_loop(1, NIT, b_body, 0)
    nb = S // TB
    wait([awo_cp(n) for n in range(NC)] + [ax_cp(j) for j in range(NC)] + [mem_cp])
    with _scope("tailB"):
        ob_cp(S - 2 * UB * TB, UB * TB).start()
        fill = {}
        attn_fill(fill, 1, False, {}, {}, {NG - 1: -1}, 0.5)
        attn_fill(fill, 2, False, ramp(-2, 1, 1), ramp(-1, 1), ramp(6, 1), 0.5)
        attn_fill(fill, 3, False, ramp(1, 2), {}, {}, 1)
        attn_fill(fill, 3, False, {}, ramp(10, 1), ramp(14, 1), 0.5)

        def with_q0(d, hh):
            y, store = d()
            x0 = _lhs([_u32(ax_v.at[j, pl.ds(0, 16), :]) for j in range(NC)])
            stash[hh] = jnp.dot(x0, a_weight(hh, 0, DM), preferred_element_type=f32)[0:8]
            return y, store
        dots = [d for k in range(UB) for d in b_proj_dots(nb - 4 + k, k)]
        run([P(with_q0, d, hh) for hh, d in enumerate(dots)], fill)
        ob_cp(S - UB * TB, UB * TB).start()


    scale_a = DH ** -0.5
    rr = lax.broadcasted_iota(i32, (2 * RM, 2 * L), 0)
    cc = lax.broadcasted_iota(i32, (2 * RM, 2 * L), 1)
    rb_, cb_ = rr >= RM, cc >= L
    ri, ci = jnp.where(rb_, rr - RM, rr), jnp.where(cb_, cc - L, cc)
    same = rb_ == cb_
    valid = same & ((ri < M) | (ri + 8 >= ci))
    fill = jnp.where(same, -1e9, -jnp.inf).astype(f32)
    slot_ok = (lax.broadcasted_iota(i32, (7, 8, 128), 0) + lax.broadcasted_iota(i32, (7, 8, 128), 1)) >= 7

    mem_s[...] = mem_v[...].astype(f32)
    xa_v[0:H, AK - 8:AK, :] = jnp.zeros((H, 8, 128), f32)
    xa_v[0:H, AV - 8:AV, :] = jnp.zeros((H, 8, 128), f32)
    NP = H // 2

    def a_step(lhs, even, z):
        qkv, pp, pend, lo, ya = {}, {}, {}, {}, {}
        nrow = 32 if even else 48

        def dot(wi, hh, k0, k1):
            rows = 48 if even != (wi == 0) else 32
            return jnp.dot(lhs[0:rows, k0:k1], a_weight(wi * H + hh, k0, k1), preferred_element_type=f32)

        def proj(wi, hh):
            y = dot(wi, hh, DM // 2, DM) + lo[wi, hh] if (wi, hh) in lo else dot(wi, hh, 0, DM)
            if y.shape[0] == 48:
                t0 = y[32:40]
                stash[wi * H + hh] = y[40:48]
            else:
                t0 = stash[wi * H + hh]
            if wi == 0:
                xa_v[hh, AQ:AQ + 8, :] = t0 * (scale_a * LOG2E)
                qkv[wi, hh] = y[0:32]
            else:
                t = jnp.concatenate([y[0:8], t0], axis=0)
                xa_v[hh, (AK, AV)[wi - 1]:(AK, AV)[wi - 1] + NK0, :] = t
                qkv[wi, hh] = jnp.concatenate([t, y[8:32]], axis=0)
            return y[0:8]

        def pair(wi, j):
            return jnp.concatenate([qkv.pop((wi, 2 * j)), qkv.pop((wi, 2 * j + 1))], axis=0).astype(bf16)

        def do_qk(j):
            q2, k2 = pair(0, j), pair(1, j)
            qkv[j] = pair(2, j)
            s = lax.dot_general(q2, k2, (((1,), (1,)), ((), ())), preferred_element_type=f32) * scale_a
            s = jnp.where(valid, s, fill)
            m = jnp.max(s, axis=1, keepdims=True)
            e = jnp.exp(s - m)
            l = jnp.sum(e, axis=1, keepdims=True)
            rc = pl.reciprocal(l, approx=True)
            rc = rc * (2.0 - l * rc)
            pp[j] = (e * rc).astype(bf16)

        def do_pv(j):
            o2 = jnp.dot(pp.pop(j), qkv.pop(j), preferred_element_type=f32)
            for i, hh in enumerate((2 * j, 2 * j + 1)):
                o, o0 = o2[RM * i:RM * (i + 1)], xa_v[hh, AO:AO + 8, :]
                if even:
                    o_s[hh, 0:32, :] = jnp.concatenate([o[0:8], o0, o[8:24]], axis=0).astype(bf16)
                    ostash[hh] = o[24:32]
                else:
                    o_s[hh] = jnp.concatenate([o[0:8], ostash[hh], o0, o[8:32]], axis=0).astype(bf16)

        def windows(hh, r):
            return jnp.concatenate([xa_v[hh:hh + 1, r + j - 7:r + j + 1, :] for j in range(NK0)], axis=0)

        def v_qk(hh):
            s = jnp.sum(xa_v[hh:hh + 1, AQ:AQ + 8, :] * windows(hh, AK), axis=2, keepdims=True)
            s = jnp.broadcast_to(s, (NK0, 8, 128))
            s = jnp.concatenate([jnp.where(slot_ok, s[0:7], -jnp.inf), s[7:]], axis=0)
            sa_v[hh % 4] = s
            pend[hh] = jnp.max(s, axis=0)

        def v_max(hh):
            xa_v[hh, AM:AM + 8, :] = pend.pop(hh)

        def v_pv(hh):
            e = jnp.exp2(sa_v[hh % 4] - xa_v[hh:hh + 1, AM:AM + 8, :])
            l = jnp.sum(e, axis=0)
            rc = pl.reciprocal(l, approx=True)
            xa_v[hh, AO:AO + 8, :] = jnp.sum(e * windows(hh, AV), axis=0) * (rc * (2.0 - l * rc))

        def epoch(d, y):
            if d > 3 * H + 4:
                return
            xa_v[z + H, 0:8, :] = y
            if d % 6 == 5 and d < 3 * H:
                qkv[1, d // 3] = jnp.concatenate([xa_v[d // 3, AK:AK + 8, :], qkv[1, d // 3][8:]], axis=0)
            for off, f in ((5, v_max), (6, v_pv), (2, v_qk)):
                if (d - off) % 3 == 0 and 0 <= (d - off) // 3 < H:
                    f((d - off) // 3)

        def wo_part(n, h0, h1):
            lo = _lhs([_u32(o_s.at[hh, pl.ds(0, nrow), :]) for hh in range(h0, h1)])
            w = _u32(wo_v.at[n, pl.ds(h0 * DH, (h1 - h0) * DH), :])
            r = jnp.dot(lo, _b16(w), preferred_element_type=f32)
            ya[n] = r + ya[n] if n in ya else r
            return ya[n][0:8]

        ni = NI[0 if even else 1]
        pieces = [(n, 4 * g, 4 * g + 4) for g in range(ni) for n in range(NC)]
        d0, done = 6 * (LPV + 2), 0
        if not even:
            lo.update({(wi, hh): dot(wi, hh, 0, DM // 2) for hh in (0, 1) for wi in range(3)})
        for d in range(3 * H):
            y = proj(d % 3, d // 3)
            ready = NC * max(((d + 1) // 6 - LPV - 1 + (1 if (d + 1) % 6 else 0)) // 2, 0)
            while done < min((d - d0 + 1) * len(pieces) // (3 * H - d0), ready):
                wo_part(*pieces[done])
                done += 1
            if d % 6 == 5:
                if d // 6 >= LQK:
                    do_qk(d // 6 - LQK)
                if d // 6 >= LPV:
                    do_pv(d // 6 - LPV)
            epoch(d, y)
        assert done == len(pieces)
        nper, n = NC // (LPV + 1), 0
        for j in range(NP, NP + LPV):
            for _ in range(nper):
                y = wo_part(n, 4 * ni, 2 * KA)
                for d in range(3 * (H + n), 3 * (H + n + 1)):
                    epoch(d, y)
                n += 1
            if j - LQK < NP:
                do_qk(j - LQK)
            do_pv(j - LPV)
        for n in range(n, NC):
            wo_part(n, 4 * ni, 2 * KA)
        for n in range(NC):
            wo_part(n, 2 * KA, H)
        return jnp.concatenate([ya[n] for n in range(NC)], axis=1)

    def a_body(t, c):
        with _scope("a_it"):
            return a_pair(t, c)

    def a_pair(t, c):
        @pl.when(t > 0)
        def _():
            oa_cp(pl.multiple_of(jnp.maximum(t - 1, 0) * 64, 64), 64).start()
        z = zero_s[0]
        o0 = pl.multiple_of(t * 64, 64)
        o1 = pl.multiple_of(jnp.minimum(t * 64 + 64, S - 64), 64)
        X = _lhs([_u32(ax_v.at[j, pl.ds(o0, 64), :]) for j in range(NC)])
        X0, X2 = X[0:16].astype(f32), X[32:48].astype(f32)
        X4 = _lhs([_u32(ax_v.at[j, pl.ds(o1, 16), :]) for j in range(NC)]).astype(f32)

        def pk(a, b):
            return jnp.concatenate([a, b], axis=0).astype(bf16)
        ye = a_step(jnp.concatenate([pk(mem_s[...], X0[8:16]), X[16:32], pk(X0[0:8], X2[0:8])], axis=0), True, z)
        yo = a_step(jnp.concatenate([pk(ye[0:8], X2[8:16]), X[48:64], pk(X2[0:8], X4[0:8])], axis=0), False, z)
        mem_s[...] = yo[0:8]
        outa_v[pl.ds(o0, 64), :] = jnp.concatenate([ye[8:32], yo[8:48]], axis=0).astype(bf16)
        return c
    lax.fori_loop(0, S // 64, a_body, 0)
    oa_cp(S - 64, 64).start()

    ob_cp(0, S).wait()
    oa_cp(0, S).wait()


@jax.jit
def _run(A_x, A_mem0, A_Wq, A_Wk, A_Wv, A_Wo, B_x, B_wqkv, B_wo):
    hbm = pl.BlockSpec(memory_space=pl.ANY)
    known = {f.name for f in dataclasses.fields(pltpu.CompilerParams)}
    optional = {k: True for k in ("disable_bounds_checks", "disable_semaphore_checks") if k in known}
    out = pl.pallas_call(
        _kernel,
        out_shape=jax.ShapeDtypeStruct((S, 2 * DM), bf16),
        in_specs=[hbm] * 9,
        out_specs=hbm,
        scratch_shapes=[
            pltpu.VMEM((NC, S, 128), bf16),
            pltpu.VMEM((M, DM), bf16),
            pltpu.VMEM((STG_ROWS, 128), bf16),
            pltpu.VMEM((3 * DM // 16, H * PITCH + 8, 128), u32),
            pltpu.VMEM((NC, H * DH, 128), bf16),
            pltpu.VMEM((NC, S, 128), bf16),
            pltpu.VMEM((24, DM // 2, 128), u32),
            pltpu.VMEM((NC, 9 * OPITCH - 1, 128), u32),
            pltpu.VMEM((S, DM), bf16),
            pltpu.VMEM((S, DM), bf16),
            pltpu.VMEM((X_SLABS, TB + HALO, 128), f32),
            pltpu.VMEM((UB, 8, TB, 128), bf16),
            pltpu.VMEM((M, DM), f32),
            pltpu.VMEM((3 * H, 8, DH), f32),
            pltpu.VMEM((H, 8, DH), f32),
            pltpu.VMEM((H, 48, DH), bf16),
            pltpu.VMEM((H + 1, AROWS, 128), f32),
            pltpu.VMEM((4, NK0, 8, 128), f32),
            pltpu.SMEM((1,), i32),
            pltpu.SemaphoreType.DMA((NSEM,)),
        ],
        compiler_params=pltpu.CompilerParams(vmem_limit_bytes=110 * 1024 * 1024, **optional),
    )(
        A_x.reshape(S, DM), A_mem0.reshape(M, DM),
        A_Wq.reshape(DM * H, DH), A_Wk.reshape(DM * H, DH), A_Wv.reshape(DM * H, DH),
        A_Wo.reshape(H * DH, DM),
        B_x.reshape(S, DM), B_wqkv, B_wo,
    )
    return out.reshape(1, S, 2 * DM)


def pallas_concat_heads__memory_aug_recurrent_mem_tr__sliding_local_dilated__prompt_kernel(
    A_x, A_mem0, A_Wq, A_Wk, A_Wv, A_Wo, A_seg_len, B_x, B_wqkv, B_wo,
):
    if isinstance(A_seg_len, int):
        assert A_seg_len == SEG
    return _run(A_x, A_mem0, A_Wq, A_Wk, A_Wv, A_Wo, B_x, B_wqkv, B_wo)
```

```python
import contextlib
import dataclasses
import functools

import jax
import jax.numpy as jnp
from jax import lax
import jax.experimental.pallas as pl
import jax.experimental.pallas.tpu as pltpu

bf16, f32, u32, i32 = jnp.bfloat16, jnp.float32, jnp.uint32, jnp.int32

S, DM = 2048, 1024
H, DH = 32, 128
M, SEG = 8, 32
L = M + SEG
DHB, WIN, DIL = 32, 8, 2
NC = DM // 128

TB = 64
UB = 4
HALO = 16
NIT = S // (TB * UB)
LQK, LPV, KA = 1, 3, 12
NI = (3, 4)
PAIRS2 = ((0, 2, 4, 6, 8, 10, 12), (0, 2, 4, 6, 8, 10, 12))
AQ, AK, AV, AM, AO, AL, AROWS = 0, 24, 56, 80, 96, 112, 128
LOG2E = 1.4426950408889634

PITCH = 9
OPITCH = 65
HW = DM * H // 2
STG_AW, STG_BW, STG_BWO = 0, 6 * HW, 6 * HW + 24 * DM
STG_TOK = STG_BWO + NC * DM
STG_ROWS = STG_TOK + 64
NG = TB // 8
X_PART = UB * 24
X_PROB = X_PART + 2 * NG
X_OUT = X_PROB + 2 * NG
X_TMP = X_OUT + 2 * NG
X_FEN = X_TMP + 32
X_SLABS = X_FEN + 2

SEM_BW, SEM_BX, SEM_BWO, SEM_AW, SEM_AWO, SEM_AX, SEM_MEM, SEM_OB, SEM_OA = 0, 6, 9, 10, 16, 17, 18, 19, 20
NSEM = 21
_SCOPES = False


def _scope(name):
    return jax.named_scope(name) if _SCOPES else contextlib.nullcontext()


def _b16(v):
    return pltpu.bitcast(v, bf16)


def _u32(view):
    return view.bitcast(u32)[...]


def _lhs(blocks):
    return _b16(jnp.concatenate(blocks, axis=1))


def _kernel(ax_h, mem_h, wq_h, wk_h, wv_h, wo_h, bx_h, bw_h, bwo_h, out_h,
            ax_v, mem_v, stg_v, wa_v, wo_v, bx_v, bw_v, bwo_v, outa_v, outb_v,
            x_v, ob_v, mem_s, stash, ostash, o_s, xa_v, sa_v, sb_v, cap_v, zero_s, sem):
    P = functools.partial

    def bw_cps(s, half):
        return [pltpu.make_async_copy(bw_h.at[pl.ds(half * (DM // 2), DM // 2), pl.ds(128 * n, 128)],
                                      stg_v.at[pl.ds(STG_BW + DM * n + half * (DM // 2), DM // 2), :],
                                      sem.at[SEM_BW + 2 * s + half]) for n in range(8 * s, 8 * s + 8)]

    def bx_cps(part):
        rows = (pl.ds(0, TB * UB), pl.ds(TB * UB, TB * UB), pl.ds(2 * TB * UB, S - 2 * TB * UB))[part]
        return [pltpu.make_async_copy(bx_h.at[rows, pl.ds(128 * j, 128)], bx_v.at[j, rows, :],
                                      sem.at[SEM_BX + part]) for j in range(NC)]

    def bwo_cps():
        return [pltpu.make_async_copy(bwo_h.at[:, pl.ds(128 * n, 128)], stg_v.at[pl.ds(STG_BWO + DM * n, DM), :],
                                      sem.at[SEM_BWO]) for n in range(NC)]

    def aw_cp(c):
        src = (wq_h, wk_h, wv_h)[c // 2]
        return pltpu.make_async_copy(src.at[pl.ds((c % 2) * HW, HW), :], stg_v.at[pl.ds(STG_AW + c * HW, HW), :],
                                     sem.at[SEM_AW + c])

    def awo_cp(n):
        return pltpu.make_async_copy(wo_h.at[:, pl.ds(128 * n, 128)], wo_v.at[n], sem.at[SEM_AWO])

    def ax_cp(j):
        return pltpu.make_async_copy(ax_h.at[:, pl.ds(128 * j, 128)], ax_v.at[j], sem.at[SEM_AX])

    mem_cp = pltpu.make_async_copy(mem_h, mem_v, sem.at[SEM_MEM])

    def ob_cp(r0, n):
        return pltpu.make_async_copy(outb_v.at[pl.ds(r0, n), :], out_h.at[pl.ds(r0, n), pl.ds(DM, DM)],
                                     sem.at[SEM_OB])

    def oa_cp(r0, n):
        return pltpu.make_async_copy(outa_v.at[pl.ds(r0, n), :], out_h.at[pl.ds(r0, n), pl.ds(0, DM)],
                                     sem.at[SEM_OA])

    def start(cps):
        for c in cps:
            c.start()

    def wait(cps):
        for c in cps:
            c.wait()

    start(bw_cps(0, 0) + bw_cps(0, 1) + bx_cps(0) + bw_cps(1, 0) + bw_cps(1, 1))

    zero_s[0] = 0
    x_v[X_FEN + 1, 0:8, :] = jnp.zeros((8, 128), f32)

    def run(dots, fill):
        z = pl.multiple_of(zero_s[0], 64)
        busy = [False]

        def epoch(e, y, close):
            if y is not None and (e in fill or (close and busy[0])):
                x_v[z + X_FEN, 0:8, :] = y
                stg_v.at[pl.ds(z + STG_TOK, 16), :].bitcast(f32)[...] = x_v[X_FEN + 1, 0:8, :]
                busy[0] = False
            for f in fill.pop(e, []):
                f()
                busy[0] = True

        epoch(-1, None, False)
        for n, d in enumerate(dots):
            y, store = d()
            epoch(n - 0.5, y[0:8], False)
            store()
            epoch(n, y[TB - 8:TB], n < len(dots) - 1)
        assert not fill, sorted(fill)

    def put(fill, n, f):
        fill.setdefault(n, []).append(f)

    lane16 = lax.broadcasted_iota(i32, (16, 128), 1)

    def perm_select(s, half, k):
        bits = [((lane16 >> (b + 1)) & 1) == 1 for b in range(3)]
        for r in range(0, 64, 16):
            src = STG_BW + 8 * s * DM + 2 * (half * 256 + 64 * k + r)
            zs = [_u32(stg_v.at[pl.ds(src + ((-t) % 8) * DM, 32), :]) for t in range(8)]
            for b in range(3):
                zs = [lax.select(bits[b], zs[(t - (1 << b)) % 8], zs[t]) for t in range(8)]
            for u in range(8):
                x_v[X_TMP + 4 * u + k, r:r + 16, :] = pltpu.bitcast(zs[u], f32)

    def perm_gather(s, half, u, k0, k1):
        n = 64 * (k1 - k0)
        lane = lax.broadcasted_iota(i32, (n, 128), 1)
        idx = 32 * ((lane >> 3) & 3) + 16 * (lane >> 6) + 2 * ((u + lane) & 7) + ((lane >> 5) & 1)
        t = pltpu.bitcast(x_v[X_TMP + 4 * u + k0:X_TMP + 4 * u + k1, 0:64, :].reshape(n, 128), u32)
        bw_v[8 * s + u, half * 256 + 64 * k0:half * 256 + 64 * k1, :] = jnp.take_along_axis(t, idx, axis=1)

    def perm_fill(fill, s, half, e_sel, e_gat):
        for k in range(4):
            put(fill, e_sel[k], P(perm_select, s, half, k))
        for k in range(16):
            assert e_gat(k) > e_sel[2 * (k // 8) + 1]
            put(fill, e_gat(k), P(perm_gather, s, half, k % 8, 2 * (k // 8), 2 * (k // 8) + 2))

    def pack_pairs(a, b):
        return (a & jnp.uint32(0xFFFF)) | (b << 16), (a >> 16) | (b & jnp.uint32(0xFFFF0000))

    def prep_bwo(n, v):
        r = STG_BWO + n * DM + 128 * v
        a = _u32(stg_v.at[pl.ds(r, 128), :]).reshape(8, 8, 128)
        b = _u32(stg_v.at[pl.ds(r + 128, 128), :]).reshape(8, 8, 128)
        a = pltpu.roll(a, 8 - v, 1) if v else a
        lo, hi = pack_pairs(a, pltpu.roll(b, 7 - v, 1))
        for k in range(8):
            d = 32 * (k % 2) + 4 * (k // 2) + v // 2
            bwo_v[n, pl.ds(d, 8, stride=OPITCH), :] = lo[k]
            bwo_v[n, pl.ds(d + 16, 8, stride=OPITCH), :] = hi[k]

    scale_b = DHB ** -0.5

    def b_qkv_dots(i, st, n0, n1):
        r0 = i * TB
        if not isinstance(r0, int):
            r0 = pl.multiple_of(r0, TB)

        def dot(n):
            lhs = _lhs([_u32(bx_v.at[j, pl.ds(r0, TB), :]) for j in range(NC)])
            y = jnp.dot(lhs, _b16(bw_v[n]), preferred_element_type=f32)

            def store():
                x_v[st * 24 + n, HALO:HALO + TB, :] = y * scale_b if n < 8 else y
                if n >= 8:
                    x_v[((st + 1) % UB) * 24 + n, 0:HALO, :] = y[TB - HALO:TB]
            return y, store
        return [P(dot, n) for n in range(n0, n1)]

    def b_proj_dots(i, st):
        r0 = i * TB
        if not isinstance(r0, int):
            r0 = pl.multiple_of(r0, TB)

        def dot(n):
            lhs = _lhs([_u32(ob_v.at[st, j]) for j in range(NC)])
            w = _b16(jnp.concatenate([bwo_v[n, OPITCH * u:OPITCH * u + 64, :] for u in range(8)], axis=0))
            y = jnp.dot(lhs, w, preferred_element_type=f32)

            def store():
                outb_v[pl.ds(r0, TB), 128 * n:128 * n + 128] = y.astype(bf16)
            return y, store
        return [P(dot, n) for n in range(NC)]

    def rows8(s0, r):
        return x_v[s0:s0 + 8, r:r + 8, :]

    def pos_ok(g, w):
        return lax.broadcasted_iota(i32, (8, 8, 128), 1) + (8 * g) - DIL * w >= 0

    def at_qk(st, g, half):
        q = rows8(st * 24, HALO + 8 * g)
        p = [jnp.sum(q * rows8(st * 24 + 8, HALO + 8 * g - DIL * w), axis=0) for w in range(4 * half, 4 * half + 4)]
        x_v[X_PART + (st % 2) * NG + g, 32 * half:32 * half + 32, :] = jnp.concatenate(p, axis=0)

    def at_softmax(st, g, first, pend):
        p = x_v[X_PART + (st % 2) * NG + g, 0:64, :]
        p = p + pltpu.roll(p, 32, 1)
        p = (p + pltpu.roll(p, 64, 1)).reshape(WIN, 8, 128)
        if first and 8 * g < DIL * (WIN - 1):
            p = jnp.where(pos_ok(g, lax.broadcasted_iota(i32, (8, 8, 128), 0)), p, -1e9)
        e = jnp.exp(p - jnp.max(p, axis=0, keepdims=True))
        l = jnp.sum(e, axis=0, keepdims=True)
        rc = pl.reciprocal(l, approx=True)
        pend[st, g] = e * (rc * (2.0 - l * rc))

    def at_store(st, g, pend):
        x_v[X_PROB + (st % 2) * NG + g, 0:64, :] = pend.pop((st, g)).reshape(64, 128)

    def at_pv(st, g, first, half):
        acc = None
        s0 = st * 24 + 16 + 4 * half
        for w in range(WIN):
            e = x_v[X_PROB + (st % 2) * NG + g:X_PROB + (st % 2) * NG + g + 1, 8 * w:8 * w + 8, :]
            r = HALO + 8 * g - DIL * w
            vv = x_v[s0:s0 + 4, r:r + 8, :]
            if first and 8 * g - DIL * w < 0:
                vv = jnp.where(pos_ok(g, w)[0:4], vv, x_v[s0:s0 + 4, HALO:HALO + 1, :])
            acc = e * vv if acc is None else acc + e * vv
        x_v[X_OUT + (st % 2) * NG + g, 32 * half:32 * half + 32, :] = acc.reshape(32, 128)

    def at_pack(st, g):
        o = [x_v[X_OUT + (st % 2) * NG + k, 0:64, :].reshape(8, 8, 128) for k in (g - 1, g)]
        ob_v[st, :, 8 * g - 8:8 * g + 8, :] = jnp.concatenate(o, axis=1).astype(bf16)

    pend = {}

    def attn_fill(fill, st, first, e_qk, e_sm, e_pv, step):
        for g, e in e_qk.items():
            put(fill, e, P(at_qk, st, g, 0))
            put(fill, e + step, P(at_qk, st, g, 1))
        for g, e in e_sm.items():
            put(fill, e, P(at_softmax, st, g, first, pend))
            put(fill, e + 3, P(at_store, st, g, pend))
        for g, e in e_pv.items():
            put(fill, e, P(at_pv, st, g, first, 0))
            put(fill, e + step, P(at_pv, st, g, first, 1))
            if g % 2 == 1:
                put(fill, e + 2 * step, P(at_pack, st, g))

    def ramp(e0, per, g0=0, g1=NG):
        return {g: e0 + per * g for g in range(g0, g1)}

    def a_relayout(src0, dst0, g):
        src = stg_v.at[pl.ds(pl.multiple_of(src0, 512), HW), :].bitcast(u32)
        dst = wa_v.at[pl.ds(dst0, DM // 32)]
        t = src[64 * g:64 * g + 64, :].reshape(2, 4, 8, 128)
        ev, od = pack_pairs(t[:, 0:2], t[:, 2:4])
        for dp in range(2):
            r = 2 * (g % 4) + dp
            for o in range(2):
                dst[g // 4, pl.ds(8 * o * PITCH + r, 8, stride=PITCH), :] = ev[dp, o]
                dst[g // 4, pl.ds((16 + 8 * o) * PITCH + r, 8, stride=PITCH), :] = od[dp, o]

    def a_weight(wh, k0, k1):
        s0, r = (wh // H) * (DM // 16), ((wh % H) // 2 + (H // 2) * (wh % 2)) * PITCH
        return _b16(wa_v[s0 + k0 // 16:s0 + k1 // 16, r:r + 8, :].reshape((k1 - k0) // 2, 128))

    def sec(k0, k1, s):
        return [d for k in range(k0, k1) for d in b_qkv_dots(k, k, 8 * s, 8 * s + 8)]

    with _scope("perm_q"):
        x_v[8:24, 0:HALO, :] = jnp.zeros((16, HALO, 128), f32)
        for half in range(2):
            wait(bw_cps(0, half))
            if half == 0:
                start(bw_cps(2, 0) + bw_cps(2, 1) + bwo_cps() + bx_cps(1))
            for k in range(4):
                perm_select(0, half, k)
            for u in range(8):
                perm_gather(0, half, u, 0, 4)
    with _scope("Q01"):
        wait(bx_cps(0))
        run(sec(0, 2, 0), {})
    with _scope("Q2"):
        wait(bw_cps(1, 0))
        fill = {}
        perm_fill(fill, 1, 0, (-1, -1, -0.5, 0.5), lambda k: (2 * k // 3 - 1) / 2)
        run(sec(2, 3, 0), fill)
    with _scope("Q3K0"):
        wait(bw_cps(1, 1))
        start(bx_cps(2) + [aw_cp(0), mem_cp])
        fill = {}
        perm_fill(fill, 1, 1, (-1, -1, -0.5, 0.5), lambda k: (2 * k // 3 - 1) / 2)
        run(sec(3, 4, 0) + sec(0, 1, 1), fill)
    with _scope("K12"):
        wait(bw_cps(2, 0))
        fill = {}
        perm_fill(fill, 2, 0, (-1, -1, 0, 1), lambda k: 3 * k // 4 + 1)
        attn_fill(fill, 0, True, ramp(2, 1.5), {}, {}, 0.5)
        run(sec(1, 3, 1), fill)
    with _scope("K3V01"):
        wait(bw_cps(2, 1))
        fill = {}
        perm_fill(fill, 2, 1, (-1, -1, -0.5, 0.5), lambda k: (2 * k // 3 - 1) / 2)
        attn_fill(fill, 0, True, {}, ramp(5, 1), ramp(15, 1, 0, NG - 1), 0.5)
        attn_fill(fill, 1, False, ramp(2, 1.5), ramp(12, 1), {}, 0.5)
        run(sec(3, 4, 1) + sec(0, 2, 2), fill)
    with _scope("V23"):
        wait(bwo_cps())
        fill = {}
        attn_fill(fill, 0, True, {}, {}, {NG - 1: -1}, 0.5)
        attn_fill(fill, 1, False, {}, {}, ramp(0.5, 2, 0, NG - 1), 1)
        attn_fill(fill, 2, False, {0: -1}, {}, {}, 0)
        for n in range(4 * NC):
            put(fill, (n * 30 // 32 - 1) / 2, P(prep_bwo, n // 4, 2 * (n % 4)))
        run(sec(2, 4, 2), fill)

    def b_body(it, carry):
        with _scope("it"):
            for c in (1, 2):
                @pl.when(it == c)
                def _():
                    wait(bx_cps(c))

            @pl.when(it >= 2)
            def _():
                cw = jnp.maximum(it - 2, 0)
                dst = stg_v.at[pl.ds(pl.multiple_of(STG_AW + cw * HW, HW), HW), :]
                pltpu.make_async_copy(dst, dst, sem.at[SEM_AW + cw]).wait()

            for c in range(1, NIT):
                @pl.when(it == c)
                def _():
                    cols = {6: (5, 6, 7), 7: ()}.get(c, (c - 1,))
                    start(([ob_cp(UB * TB * (c - 2), UB * TB)] if c >= 2 else []) + ([aw_cp(c)] if c < 6 else [])
                          + [cp(n) for n in cols for cp in (awo_cp, ax_cp)])
            c = jnp.maximum(it - 2, 0)
            src0 = jnp.where(it == 1, STG_BW, STG_AW + c * HW)
            dst0 = c * (DM // 32)
            dots, fill = [], {}
            for k in range(UB):
                i, e0 = UB * it + k, 32 * k
                dots += b_qkv_dots(i, k, 0, 24) + b_proj_dots(i - 4, k)
                e0 -= 1
                attn_fill(fill, (k - 3) % UB, False, {}, {}, {NG - 1: e0}, 1)
                attn_fill(fill, (k - 2) % UB, False, ramp(e0 - 2, 4, 1), ramp(e0, 4), ramp(e0 + 4, 4, 0, NG - 1), 1)
                attn_fill(fill, (k - 1) % UB, False, {0: e0 + 30}, {}, {}, 1)
                for g in range(32):
                    put(fill, e0 + g + 0.5, P(a_relayout, src0, dst0, 32 * k + g))
            run(dots, fill)
        return carry
    lax.fori_loop(1, NIT, b_body, 0)
    nb = S // TB
    wait([awo_cp(n) for n in range(NC)] + [ax_cp(j) for j in range(NC)] + [mem_cp])
    with _scope("tailB"):
        ob_cp(S - 2 * UB * TB, UB * TB).start()
        fill = {}
        attn_fill(fill, 1, False, {}, {}, {NG - 1: -1}, 0.5)
        attn_fill(fill, 2, False, ramp(-2, 1, 1), ramp(-1, 1), ramp(6, 1), 0.5)
        attn_fill(fill, 3, False, ramp(1, 2), {}, {}, 1)
        attn_fill(fill, 3, False, {}, ramp(10, 1), ramp(14, 1), 0.5)

        def with_q0(d, hh):
            y, store = d()
            x0 = _lhs([_u32(ax_v.at[j, pl.ds(0, 16), :]) for j in range(NC)])
            stash[hh] = jnp.dot(x0, a_weight(hh, 0, DM), preferred_element_type=f32)[0:8]
            return y, store
        dots = [d for k in range(UB) for d in b_proj_dots(nb - 4 + k, k)]
        run([P(with_q0, d, hh) for hh, d in enumerate(dots)], fill)
        ob_cp(S - UB * TB, UB * TB).start()


    scale_a = DH ** -0.5
    for nv in (1, 2):
        rm = L - 8 * nv
        rr = lax.broadcasted_iota(i32, (2 * rm, 2 * L), 0)
        cc = lax.broadcasted_iota(i32, (2 * rm, 2 * L), 1)
        rb_, cb_ = rr >= rm, cc >= L
        ri, ci = jnp.where(rb_, rr - rm, rr), jnp.where(cb_, cc - L, cc)
        same = rb_ == cb_
        cap_v[nv - 1, 0:2 * rm, :] = jnp.where(same & ((ri < M) | (ri + 8 * nv >= ci)), 1.0,
                                               jnp.where(same, -1e9, -jnp.inf)).astype(f32)
    slot_ok = (lax.broadcasted_iota(i32, (7, 8, 128), 0) + lax.broadcasted_iota(i32, (7, 8, 128), 1)) >= 7

    mem_s[...] = mem_v[...].astype(f32)
    xa_v[0:H, AK - 8:AK, :] = jnp.zeros((H, 8, 128), f32)
    xa_v[0:H, AV - 8:AV, :] = jnp.zeros((H, 8, 128), f32)
    NP = H // 2

    def a_step(lhs, even, z):
        qkv, pp, pend, lo, ya = {}, {}, {}, {}, {}
        nrow = 32 if even else 48

        def nv(hh):
            return 2 if hh // 2 in PAIRS2[0 if even else 1] else 1

        def dot(wi, hh, k0, k1):
            rows = 48 if even != (wi == 0) else 32
            return jnp.dot(lhs[0:rows, k0:k1], a_weight(wi * H + hh, k0, k1), preferred_element_type=f32)

        def proj(wi, hh):
            y = dot(wi, hh, DM // 2, DM) + lo[wi, hh] if (wi, hh) in lo else dot(wi, hh, 0, DM)
            if y.shape[0] == 48:
                t0 = y[32:40]
                stash[wi * H + hh] = y[40:48]
            else:
                t0 = stash[wi * H + hh]
            t, n = jnp.concatenate([y[0:8], t0, y[8:32]], axis=0), 8 * nv(hh)
            if wi == 0:
                xa_v[hh, AQ:AQ + n, :] = t[8:8 + n] * (scale_a * LOG2E)
                qkv[wi, hh] = jnp.concatenate([y[0:8], y[n:32]], axis=0)
            else:
                xa_v[hh, (AK, AV)[wi - 1]:(AK, AV)[wi - 1] + 8 + n, :] = t[0:8 + n]
                qkv[wi, hh] = t
            return y[y.shape[0] - 8:]

        def pair(wi, j):
            return jnp.concatenate([qkv.pop((wi, 2 * j)), qkv.pop((wi, 2 * j + 1))], axis=0).astype(bf16)

        def do_qk(j):
            q2, k2 = pair(0, j), pair(1, j)
            qkv[j] = pair(2, j)
            s = lax.dot_general(q2, k2, (((1,), (1,)), ((), ())), preferred_element_type=f32) * scale_a
            cap = cap_v[nv(2 * j) - 1, 0:s.shape[0], :]
            s = jnp.where(cap > 0, s, cap)
            m = jnp.max(s, axis=1, keepdims=True)
            e = jnp.exp(s - m)
            l = jnp.sum(e, axis=1, keepdims=True)
            rc = pl.reciprocal(l, approx=True)
            rc = rc * (2.0 - l * rc)
            pp[j] = (e * rc).astype(bf16)

        def do_pv(j):
            o2 = jnp.dot(pp.pop(j), qkv.pop(j), preferred_element_type=f32)
            for i, hh in enumerate((2 * j, 2 * j + 1)):
                rm = L - 8 * nv(hh)
                o = jnp.concatenate([o2[rm * i:rm * i + 8], xa_v[hh, AO:AO + 8 * nv(hh), :],
                                     o2[rm * i + 8:rm * (i + 1)]], axis=0)
                if even:
                    o_s[hh, 0:32, :] = o[0:32].astype(bf16)
                    ostash[hh] = o[32:40]
                else:
                    o_s[hh] = jnp.concatenate([o[0:8], ostash[hh], o[8:40]], axis=0).astype(bf16)

        def windows(hh, r, j0, j1):
            return jnp.concatenate([xa_v[hh:hh + 1, r + j - 7:r + j + 1, :] for j in range(j0, j1)], axis=0)

        def scores(hh, g):
            return sa_v.at[hh % 4] if g == 0 else sb_v.at[hh % 2]

        def v_qk(hh, g, j0, j1):
            q = xa_v[hh:hh + 1, AQ + 8 * g:AQ + 8 * g + 8, :]
            s = jnp.sum(q * windows(hh, AK, j0, j1), axis=2, keepdims=True)
            s = jnp.broadcast_to(s, (j1 - j0, 8, 128))
            if j0 == 0:
                s = jnp.concatenate([jnp.where(slot_ok, s[0:7], -jnp.inf), s[7:]], axis=0)
            scores(hh, g)[j0:j1] = s
            m = jnp.max(s, axis=0)
            pend[hh, g] = m if j0 == 0 else jnp.maximum(m, pend[hh, g])

        def v_max(hh, g):
            xa_v[hh, AM + 8 * g:AM + 8 * g + 8, :] = pend.pop((hh, g))

        def v_pv(hh, g, j0, j1):
            e = jnp.exp2(scores(hh, g)[j0:j1] - xa_v[hh:hh + 1, AM + 8 * g:AM + 8 * g + 8, :])
            l, o = jnp.sum(e, axis=0), jnp.sum(e * windows(hh, AV, j0, j1), axis=0)
            if j0 > 0:
                l, o = l + xa_v[hh, AL:AL + 8, :], o + xa_v[hh, AO + 8 * g:AO + 8 * g + 8, :]
            if j1 == 16 + 8 * g:
                rc = pl.reciprocal(l, approx=True)
                o = o * (rc * (2.0 - l * rc))
            else:
                xa_v[hh, AL:AL + 8, :] = l
            xa_v[hh, AO + 8 * g:AO + 8 * g + 8, :] = o

        work = {}
        for hh in range(H):
            d = 3 * hh
            put(work, d + 5, P(v_max, hh, 0))
            put(work, d + 6, P(v_pv, hh, 0, 0, 16))
            put(work, d + 2, P(v_qk, hh, 0, 0, 16))
            if nv(hh) == 2:
                d += 3 * (hh % 2)
                put(work, d + 2, P(v_qk, hh, 1, 0, 12))
                put(work, d + 5, P(v_qk, hh, 1, 12, 24))
                put(work, d + 8, P(v_max, hh, 1))
                put(work, d + 10, P(v_pv, hh, 1, 0, 12))
                put(work, d + 13, P(v_pv, hh, 1, 12, 24))

        def epoch(d, y):
            if not work and d > 3 * H + 4:
                return
            xa_v[z + H, 0:8, :] = y
            if d % 6 == 5 and d < 3 * H:
                qkv[1, d // 3] = jnp.concatenate([xa_v[d // 3, AK:AK + 8, :], qkv[1, d // 3][8:]], axis=0)
            for f in work.pop(d, []):
                f()

        def wo_part(n, h0, h1):
            lo = _lhs([_u32(o_s.at[hh, pl.ds(0, nrow), :]) for hh in range(h0, h1)])
            w = _u32(wo_v.at[n, pl.ds(h0 * DH, (h1 - h0) * DH), :])
            r = jnp.dot(lo, _b16(w), preferred_element_type=f32)
            ya[n] = r + ya[n] if n in ya else r
            return ya[n][0:8]

        ni = NI[0 if even else 1]
        pieces = [(n, 4 * g, 4 * g + 4) for g in range(ni) for n in range(NC)]
        d0, done = 6 * (LPV + 2), 0
        if not even:
            lo.update({(wi, hh): dot(wi, hh, 0, DM // 2) for hh in (0, 1) for wi in range(3)})
        for d in range(3 * H):
            y = proj(d % 3, d // 3)
            ready = NC * max(((d + 1) // 6 - LPV - 1 + (1 if (d + 1) % 6 else 0)) // 2, 0)
            while done < min((d - d0 + 1) * len(pieces) // (3 * H - d0), ready):
                wo_part(*pieces[done])
                done += 1
            if d % 6 == 5:
                if d // 6 >= LQK:
                    do_qk(d // 6 - LQK)
                if d // 6 >= LPV:
                    do_pv(d // 6 - LPV)
            epoch(d, y)
        assert done == len(pieces)
        nper, n = NC // (LPV + 1), 0
        for j in range(NP, NP + LPV):
            for _ in range(nper):
                y = wo_part(n, 4 * ni, 2 * KA)
                for d in range(3 * (H + n), 3 * (H + n + 1)):
                    epoch(d, y)
                n += 1
            if j - LQK < NP:
                do_qk(j - LQK)
            do_pv(j - LPV)
        for n in range(n, NC):
            wo_part(n, 4 * ni, 2 * KA)
        for n in range(NC):
            wo_part(n, 2 * KA, H)
        assert not work
        return jnp.concatenate([ya[n] for n in range(NC)], axis=1)

    def a_body(t, c):
        with _scope("a_it"):
            return a_pair(t, c)

    def a_pair(t, c):
        @pl.when(t > 0)
        def _():
            oa_cp(pl.multiple_of(jnp.maximum(t - 1, 0) * 64, 64), 64).start()
        z = zero_s[0]
        o0 = pl.multiple_of(t * 64, 64)
        o1 = pl.multiple_of(jnp.minimum(t * 64 + 64, S - 64), 64)
        X = _lhs([_u32(ax_v.at[j, pl.ds(o0, 64), :]) for j in range(NC)])
        X0, X2 = X[0:16].astype(f32), X[32:48].astype(f32)
        X4 = _lhs([_u32(ax_v.at[j, pl.ds(o1, 16), :]) for j in range(NC)]).astype(f32)

        def pk(a, b):
            return jnp.concatenate([a, b], axis=0).astype(bf16)
        ye = a_step(jnp.concatenate([pk(mem_s[...], X0[8:16]), X[16:32], pk(X0[0:8], X2[0:8])], axis=0), True, z)
        yo = a_step(jnp.concatenate([pk(ye[0:8], X2[8:16]), X[48:64], pk(X2[0:8], X4[0:8])], axis=0), False, z)
        mem_s[...] = yo[0:8]
        outa_v[pl.ds(o0, 64), :] = jnp.concatenate([ye[8:32], yo[8:48]], axis=0).astype(bf16)
        return c
    lax.fori_loop(0, S // 64, a_body, 0)
    oa_cp(S - 64, 64).start()

    ob_cp(0, S).wait()
    oa_cp(0, S).wait()


@jax.jit
def _run(A_x, A_mem0, A_Wq, A_Wk, A_Wv, A_Wo, B_x, B_wqkv, B_wo):
    hbm = pl.BlockSpec(memory_space=pl.ANY)
    known = {f.name for f in dataclasses.fields(pltpu.CompilerParams)}
    optional = {k: True for k in ("disable_bounds_checks", "disable_semaphore_checks") if k in known}
    out = pl.pallas_call(
        _kernel,
        out_shape=jax.ShapeDtypeStruct((S, 2 * DM), bf16),
        in_specs=[hbm] * 9,
        out_specs=hbm,
        scratch_shapes=[
            pltpu.VMEM((NC, S, 128), bf16),
            pltpu.VMEM((M, DM), bf16),
            pltpu.VMEM((STG_ROWS, 128), bf16),
            pltpu.VMEM((3 * DM // 16, H * PITCH + 8, 128), u32),
            pltpu.VMEM((NC, H * DH, 128), bf16),
            pltpu.VMEM((NC, S, 128), bf16),
            pltpu.VMEM((24, DM // 2, 128), u32),
            pltpu.VMEM((NC, 9 * OPITCH - 1, 128), u32),
            pltpu.VMEM((S, DM), bf16),
            pltpu.VMEM((S, DM), bf16),
            pltpu.VMEM((X_SLABS, TB + HALO, 128), f32),
            pltpu.VMEM((UB, 8, TB, 128), bf16),
            pltpu.VMEM((M, DM), f32),
            pltpu.VMEM((3 * H, 8, DH), f32),
            pltpu.VMEM((H, 8, DH), f32),
            pltpu.VMEM((H, 48, DH), bf16),
            pltpu.VMEM((H + 1, AROWS, 128), f32),
            pltpu.VMEM((4, 16, 8, 128), f32),
            pltpu.VMEM((2, 24, 8, 128), f32),
            pltpu.VMEM((2, 64, 2 * L), f32),
            pltpu.SMEM((1,), i32),
            pltpu.SemaphoreType.DMA((NSEM,)),
        ],
        compiler_params=pltpu.CompilerParams(vmem_limit_bytes=110 * 1024 * 1024, **optional),
    )(
        A_x.reshape(S, DM), A_mem0.reshape(M, DM),
        A_Wq.reshape(DM * H, DH), A_Wk.reshape(DM * H, DH), A_Wv.reshape(DM * H, DH),
        A_Wo.reshape(H * DH, DM),
        B_x.reshape(S, DM), B_wqkv, B_wo,
    )
    return out.reshape(1, S, 2 * DM)


def pallas_concat_heads__memory_aug_recurrent_mem_tr__sliding_local_dilated__prompt_kernel(
    A_x, A_mem0, A_Wq, A_Wk, A_Wv, A_Wo, A_seg_len, B_x, B_wqkv, B_wo,
):
    if isinstance(A_seg_len, int):
        assert A_seg_len == SEG
    return _run(A_x, A_mem0, A_Wq, A_Wk, A_Wv, A_Wo, B_x, B_wqkv, B_wo)
```

```python
import contextlib
import dataclasses
import functools

import jax
import jax.numpy as jnp
from jax import lax
import jax.experimental.pallas as pl
import jax.experimental.pallas.tpu as pltpu

bf16, f32, u32, i32 = jnp.bfloat16, jnp.float32, jnp.uint32, jnp.int32

S, DM = 2048, 1024
H, DH = 32, 128
M, SEG = 8, 32
L = M + SEG
DHB, WIN, DIL = 32, 8, 2
NC = DM // 128

TB = 64
UB = 4
HALO = 16
NIT = S // (TB * UB)
GC = 3
LQK, LPV, KA = 1, 3, 12
NI = (3, 4)
PAIRS2 = ((0, 2, 4, 6, 8, 10, 12), (0, 2, 4, 6, 8, 10, 12))
AQ, AK, AV, AM, AO, AL, AROWS = 0, 24, 56, 80, 96, 112, 128
LOG2E = 1.4426950408889634

PITCH = 9
OPITCH = 65
HW = DM * H // 2
STG_AW, STG_BW, STG_BWO = 0, 6 * HW, 6 * HW + 24 * DM
STG_TOK = STG_BWO + NC * DM
STG_ROWS = STG_TOK + 64
NG = TB // 8
X_PART = UB * 24
X_PROB = X_PART + 2 * NG
X_OUT = X_PROB + 2 * NG
X_TMP = X_OUT + 2 * NG
X_FEN = X_TMP + 32
X_SLABS = X_FEN + 2

SEM_BW, SEM_BX, SEM_BWO, SEM_AW, SEM_AWO, SEM_AX, SEM_MEM, SEM_OB, SEM_OA = 0, 6, 9, 10, 16, 17, 18, 19, 20
NSEM = 21
_SCOPES = False


def _scope(name):
    return jax.named_scope(name) if _SCOPES else contextlib.nullcontext()


def _b16(v):
    return pltpu.bitcast(v, bf16)


def _u32(view):
    return view.bitcast(u32)[...]


def _lhs(blocks):
    return _b16(jnp.concatenate(blocks, axis=1))


def _kernel(ax_h, mem_h, wq_h, wk_h, wv_h, wo_h, bx_h, bw_h, bwo_h, out_h,
            ax_v, mem_v, stg_v, wa_v, wo_v, bx_v, bw_v, bwo_v, outa_v, outb_v,
            x_v, ob_v, mem_s, stash, ostash, o_s, xa_v, sa_v, sb_v, cap_v, zero_s, sem):
    P = functools.partial

    def bw_cps(s, half):
        return [pltpu.make_async_copy(bw_h.at[pl.ds(half * (DM // 2), DM // 2), pl.ds(128 * n, 128)],
                                      stg_v.at[pl.ds(STG_BW + DM * n + half * (DM // 2), DM // 2), :],
                                      sem.at[SEM_BW + 2 * s + half]) for n in range(8 * s, 8 * s + 8)]

    def bx_cps(part):
        rows = (pl.ds(0, TB * UB), pl.ds(TB * UB, TB * UB), pl.ds(2 * TB * UB, S - 2 * TB * UB))[part]
        return [pltpu.make_async_copy(bx_h.at[rows, pl.ds(128 * j, 128)], bx_v.at[j, rows, :],
                                      sem.at[SEM_BX + part]) for j in range(NC)]

    def bwo_cps():
        return [pltpu.make_async_copy(bwo_h.at[:, pl.ds(128 * n, 128)], stg_v.at[pl.ds(STG_BWO + DM * n, DM), :],
                                      sem.at[SEM_BWO]) for n in range(NC)]

    def aw_cp(c):
        src = (wq_h, wk_h, wv_h)[c // 2]
        return pltpu.make_async_copy(src.at[pl.ds((c % 2) * HW, HW), :], stg_v.at[pl.ds(STG_AW + c * HW, HW), :],
                                     sem.at[SEM_AW + c])

    def awo_cp(n):
        return pltpu.make_async_copy(wo_h.at[:, pl.ds(128 * n, 128)], wo_v.at[n], sem.at[SEM_AWO])

    def ax_cp(j):
        return pltpu.make_async_copy(ax_h.at[:, pl.ds(128 * j, 128)], ax_v.at[j], sem.at[SEM_AX])

    mem_cp = pltpu.make_async_copy(mem_h, mem_v, sem.at[SEM_MEM])

    def ob_cp(r0, n):
        return pltpu.make_async_copy(outb_v.at[pl.ds(r0, n), :], out_h.at[pl.ds(r0, n), pl.ds(DM, DM)],
                                     sem.at[SEM_OB])

    def oa_cp(r0, n):
        return pltpu.make_async_copy(outa_v.at[pl.ds(r0, n), :], out_h.at[pl.ds(r0, n), pl.ds(0, DM)],
                                     sem.at[SEM_OA])

    def start(cps):
        for c in cps:
            c.start()

    def wait(cps):
        for c in cps:
            c.wait()

    start(bx_cps(0) + bw_cps(0, 0) + bw_cps(0, 1) + bw_cps(1, 0) + bw_cps(1, 1))

    zero_s[0] = 0
    x_v[X_FEN + 1, 0:8, :] = jnp.zeros((8, 128), f32)

    def run(dots, fill):
        z = pl.multiple_of(zero_s[0], 64)
        busy = [False]

        def epoch(e, y, close):
            if y is not None and (e in fill or (close and busy[0])):
                x_v[z + X_FEN, 0:8, :] = y
                stg_v.at[pl.ds(z + STG_TOK, 16), :].bitcast(f32)[...] = x_v[X_FEN + 1, 0:8, :]
                busy[0] = False
            for f in fill.pop(e, []):
                f()
                busy[0] = True

        epoch(-1, None, False)
        for n, d in enumerate(dots):
            y, store = d()
            epoch(n - 0.5, y[0:8], False)
            store()
            epoch(n, y[TB - 8:TB], n < len(dots) - 1)
        assert not fill, sorted(fill)

    def put(fill, n, f):
        fill.setdefault(n, []).append(f)

    lane16 = lax.broadcasted_iota(i32, (16, 128), 1)

    def perm_select(s, half, k, r0=0, r1=64):
        bits = [((lane16 >> (b + 1)) & 1) == 1 for b in range(3)]
        for r in range(r0, r1, 16):
            src = STG_BW + 8 * s * DM + 2 * (half * 256 + 64 * k + r)
            zs = [_u32(stg_v.at[pl.ds(src + ((-t) % 8) * DM, 32), :]) for t in range(8)]
            for b in range(3):
                zs = [lax.select(bits[b], zs[(t - (1 << b)) % 8], zs[t]) for t in range(8)]
            for u in range(8):
                x_v[X_TMP + 4 * u + k, r:r + 16, :] = pltpu.bitcast(zs[u], f32)

    def perm_gather(s, half, u, k0, k1):
        n = 64 * (k1 - k0)
        lane = lax.broadcasted_iota(i32, (n, 128), 1)
        idx = 32 * ((lane >> 3) & 3) + 16 * (lane >> 6) + 2 * ((u + lane) & 7) + ((lane >> 5) & 1)
        t = pltpu.bitcast(x_v[X_TMP + 4 * u + k0:X_TMP + 4 * u + k1, 0:64, :].reshape(n, 128), u32)
        bw_v[8 * s + u, half * 256 + 64 * k0:half * 256 + 64 * k1, :] = jnp.take_along_axis(t, idx, axis=1)

    def perm_fill(fill, s, half):
        sel = (-1, -1, 0, 1, 2, 3, 4, 5)
        for k in range(8):
            put(fill, sel[k], P(perm_select, s, half, k // 2, 32 * (k % 2), 32 * (k % 2) + 32))
        t = 0.0
        for k0, k1 in ((0, 1), (1, 2), (2, 4)):
            for u in range(8):
                assert int(t) > sel[2 * k1 - 1]
                put(fill, int(t), P(perm_gather, s, half, u, k0, k1))
                t += 2.3 * (8 * (k1 - k0) + 3) / 64

    def pack_pairs(a, b):
        return (a & jnp.uint32(0xFFFF)) | (b << 16), (a >> 16) | (b & jnp.uint32(0xFFFF0000))

    def prep_bwo(n, v):
        r = STG_BWO + n * DM + 128 * v
        a = _u32(stg_v.at[pl.ds(r, 128), :]).reshape(8, 8, 128)
        b = _u32(stg_v.at[pl.ds(r + 128, 128), :]).reshape(8, 8, 128)
        a = pltpu.roll(a, 8 - v, 1) if v else a
        lo, hi = pack_pairs(a, pltpu.roll(b, 7 - v, 1))
        for k in range(8):
            d = 32 * (k % 2) + 4 * (k // 2) + v // 2
            bwo_v[n, pl.ds(d, 8, stride=OPITCH), :] = lo[k]
            bwo_v[n, pl.ds(d + 16, 8, stride=OPITCH), :] = hi[k]

    scale_b = DHB ** -0.5

    def b_qkv_dots(i, st, n0, n1, half=None):
        r0 = i * TB
        if not isinstance(r0, int):
            r0 = pl.multiple_of(r0, TB)
        j0, j1 = (0, NC) if half is None else (4 * half, 4 * half + 4)

        def dot(n):
            lhs = _lhs([_u32(bx_v.at[j, pl.ds(r0, TB), :]) for j in range(j0, j1)])
            y = jnp.dot(lhs, _b16(bw_v[n, 64 * j0:64 * j1, :]), preferred_element_type=f32)

            def store():
                t = y + x_v[st * 24 + n, HALO:HALO + TB, :] if half == 1 else y
                x_v[st * 24 + n, HALO:HALO + TB, :] = t * scale_b if n < 8 and half != 0 else t
                if n >= 8 and half != 0:
                    x_v[((st + 1) % UB) * 24 + n, 0:HALO, :] = t[TB - HALO:TB]
            return y, store
        return [P(dot, n) for n in range(n0, n1)]

    def b_proj_dots(i, st):
        r0 = i * TB
        if not isinstance(r0, int):
            r0 = pl.multiple_of(r0, TB)

        def dot(n):
            lhs = _lhs([_u32(ob_v.at[st, j]) for j in range(NC)])
            w = _b16(jnp.concatenate([bwo_v[n, OPITCH * u:OPITCH * u + 64, :] for u in range(8)], axis=0))
            y = jnp.dot(lhs, w, preferred_element_type=f32)

            def store():
                outb_v[pl.ds(r0, TB), 128 * n:128 * n + 128] = y.astype(bf16)
            return y, store
        return [P(dot, n) for n in range(NC)]

    def rows8(s0, r):
        return x_v[s0:s0 + 8, r:r + 8, :]

    def pos_ok(g, w):
        return lax.broadcasted_iota(i32, (8, 8, 128), 1) + (8 * g) - DIL * w >= 0

    def at_qk(st, g, half):
        q = rows8(st * 24, HALO + 8 * g)
        p = [jnp.sum(q * rows8(st * 24 + 8, HALO + 8 * g - DIL * w), axis=0) for w in range(4 * half, 4 * half + 4)]
        x_v[X_PART + (st % 2) * NG + g, 32 * half:32 * half + 32, :] = jnp.concatenate(p, axis=0)

    def at_softmax(st, g, first, pend):
        p = x_v[X_PART + (st % 2) * NG + g, 0:64, :]
        p = p + pltpu.roll(p, 32, 1)
        p = (p + pltpu.roll(p, 64, 1)).reshape(WIN, 8, 128)
        if first and 8 * g < DIL * (WIN - 1):
            p = jnp.where(pos_ok(g, lax.broadcasted_iota(i32, (8, 8, 128), 0)), p, -1e9)
        e = jnp.exp(p - jnp.max(p, axis=0, keepdims=True))
        l = jnp.sum(e, axis=0, keepdims=True)
        rc = pl.reciprocal(l, approx=True)
        pend[st, g] = e * (rc * (2.0 - l * rc))

    def at_store(st, g, pend):
        x_v[X_PROB + (st % 2) * NG + g, 0:64, :] = pend.pop((st, g)).reshape(64, 128)

    def at_pv(st, g, first, half):
        acc = None
        s0 = st * 24 + 16 + 4 * half
        for w in range(WIN):
            e = x_v[X_PROB + (st % 2) * NG + g:X_PROB + (st % 2) * NG + g + 1, 8 * w:8 * w + 8, :]
            r = HALO + 8 * g - DIL * w
            vv = x_v[s0:s0 + 4, r:r + 8, :]
            if first and 8 * g - DIL * w < 0:
                vv = jnp.where(pos_ok(g, w)[0:4], vv, x_v[s0:s0 + 4, HALO:HALO + 1, :])
            acc = e * vv if acc is None else acc + e * vv
        x_v[X_OUT + (st % 2) * NG + g, 32 * half:32 * half + 32, :] = acc.reshape(32, 128)

    def at_pack(st, g):
        o = [x_v[X_OUT + (st % 2) * NG + k, 0:64, :].reshape(8, 8, 128) for k in (g - 1, g)]
        ob_v[st, :, 8 * g - 8:8 * g + 8, :] = jnp.concatenate(o, axis=1).astype(bf16)

    pend = {}

    def attn_fill(fill, st, first, e_qk, e_sm, e_pv, step, lat=3):
        for g, e in e_qk.items():
            put(fill, e, P(at_qk, st, g, 0))
            put(fill, e + step, P(at_qk, st, g, 1))
        for g, e in e_sm.items():
            put(fill, e, P(at_softmax, st, g, first, pend))
            put(fill, e + lat, P(at_store, st, g, pend))
        for g, e in e_pv.items():
            put(fill, e, P(at_pv, st, g, first, 0))
            put(fill, e + step, P(at_pv, st, g, first, 1))
            if g % 2 == 1:
                put(fill, e + 2 * step, P(at_pack, st, g))

    def ramp(e0, per, g0=0, g1=NG):
        return {g: e0 + per * g for g in range(g0, g1)}

    def a_relayout(src0, dst0, g):
        src = stg_v.at[pl.ds(pl.multiple_of(src0, 512), HW), :].bitcast(u32)
        dst = wa_v.at[pl.ds(dst0, DM // 32)]
        t = src[64 * g:64 * g + 64, :].reshape(2, 4, 8, 128)
        ev, od = pack_pairs(t[:, 0:2], t[:, 2:4])
        for dp in range(2):
            r = 2 * (g % 4) + dp
            for o in range(2):
                dst[g // 4, pl.ds(8 * o * PITCH + r, 8, stride=PITCH), :] = ev[dp, o]
                dst[g // 4, pl.ds((16 + 8 * o) * PITCH + r, 8, stride=PITCH), :] = od[dp, o]

    def a_weight(wh, k0, k1):
        s0, r = (wh // H) * (DM // 16), ((wh % H) // 2 + (H // 2) * (wh % 2)) * PITCH
        return _b16(wa_v[s0 + k0 // 16:s0 + k1 // 16, r:r + 8, :].reshape((k1 - k0) // 2, 128))

    def sec(h, k0, nk=2):
        return [d for k in range(k0, k0 + nk) for d in b_qkv_dots(k, k, 8 * (h // 2), 8 * (h // 2) + 8, h % 2)]

    with _scope("perm_q"):
        x_v[8:24, 0:HALO, :] = jnp.zeros((16, HALO, 128), f32)
        wait(bx_cps(0) + bw_cps(0, 0))
        start(bw_cps(2, 0) + bw_cps(2, 1) + bwo_cps() + bx_cps(1))
        z = pl.multiple_of(zero_s[0], 64)
        for k in range(4):
            perm_select(0, 0, k)
            if k % 2 == 1:
                x_v[z + X_FEN, 0:8, :] = x_v[X_FEN + 1, 0:8, :]
                for u in range(8):
                    perm_gather(0, 0, u, k - 1, k + 1)
        run(sec(0, 0), {})
    for h in range(1, 6):
        with _scope("half%d" % h):
            wait(bw_cps(h // 2, h % 2))
            if h == 3:
                start(bx_cps(2) + [aw_cp(0), mem_cp])
            fill = {}
            perm_fill(fill, h // 2, h % 2)
            if h == 4:
                attn_fill(fill, 0, True, {0: 2, 1: 4, **ramp(10, 2, 2)}, {}, {}, 1)
                attn_fill(fill, 1, False, ramp(26, 2, 0, 2), {}, {}, 1)
            if h == 5:
                attn_fill(fill, 1, False, ramp(-2, 2, 2), {}, {}, 1)
                attn_fill(fill, 2, False, {0: 14}, {}, {}, 1)
                pv = [23 + k * 15 // (NG + GC) for k in range(NG + GC)]
                attn_fill(fill, 0, True, {}, ramp(11, 1), dict(enumerate(pv[:NG])), 1, lat=6)
                attn_fill(fill, 1, False, {}, ramp(19, 1), dict(enumerate(pv[NG:])), 1, lat=6)
            run(sec(h - 1, 2) + sec(h, 0, 3 if h == 5 else 2), fill)
    with _scope("last"):
        wait(bwo_cps())
        fill = {}
        for n in range(4 * NC):
            put(fill, max(n // 3 - 3, -1), P(prep_bwo, n // 4, 2 * (n % 4)))
        run(sec(5, 3, 1), fill)

    def b_body(it, carry):
        with _scope("it"):
            for c in (1, 2):
                @pl.when(it == c)
                def _():
                    wait(bx_cps(c))

            @pl.when(it >= 2)
            def _():
                cw = jnp.maximum(it - 2, 0)
                dst = stg_v.at[pl.ds(pl.multiple_of(STG_AW + cw * HW, HW), HW), :]
                pltpu.make_async_copy(dst, dst, sem.at[SEM_AW + cw]).wait()

            for c in range(1, NIT):
                @pl.when(it == c)
                def _():
                    cols = {6: (5, 6, 7), 7: ()}.get(c, (c - 1,))
                    start(([ob_cp(UB * TB * (c - 2), UB * TB)] if c >= 2 else []) + ([aw_cp(c)] if c < 6 else [])
                          + [cp(n) for n in cols for cp in (awo_cp, ax_cp)])
            c = jnp.maximum(it - 2, 0)
            src0 = jnp.where(it == 1, STG_BW, STG_AW + c * HW)
            dst0 = c * (DM // 32)
            dots, fill = [], {}
            for k in range(UB):
                i, e0 = UB * it + k, 32 * k
                dots += b_qkv_dots(i, k, 0, 24) + b_proj_dots(i - 4, k)
                e0 -= 1
                attn_fill(fill, (k - 3) % UB, False, {}, {}, ramp(e0 - 4 * GC, 4, GC), 1)
                attn_fill(fill, (k - 2) % UB, False, ramp(e0 - 2, 4, 1), ramp(e0, 4), ramp(e0 + 32 - 4 * GC, 4, 0, GC), 1)
                attn_fill(fill, (k - 1) % UB, False, {0: e0 + 30}, {}, {}, 1)
                for g in range(32):
                    put(fill, e0 + g + 0.5, P(a_relayout, src0, dst0, 32 * k + g))
            run(dots, fill)
        return carry
    lax.fori_loop(1, NIT, b_body, 0)
    nb = S // TB
    wait([awo_cp(n) for n in range(NC)] + [ax_cp(j) for j in range(NC)] + [mem_cp])
    with _scope("tailB"):
        ob_cp(S - 2 * UB * TB, UB * TB).start()
        fill = {}
        attn_fill(fill, 1, False, {}, {}, ramp(-2, 1, GC), 0.5)
        attn_fill(fill, 2, False, ramp(-2, 1, 1), ramp(-1, 1), ramp(6.5, 1), 0.5)
        attn_fill(fill, 3, False, ramp(5, 1.5), {}, {}, 0.5)
        attn_fill(fill, 3, False, {}, ramp(10, 1), ramp(14.5, 1), 0.5)

        def with_q0(d, hh):
            y, store = d()
            x0 = _lhs([_u32(ax_v.at[j, pl.ds(0, 16), :]) for j in range(NC)])
            stash[hh] = jnp.dot(x0, a_weight(hh, 0, DM), preferred_element_type=f32)[0:8]
            return y, store
        dots = [d for k in range(UB) for d in b_proj_dots(nb - 4 + k, k)]
        run([P(with_q0, d, hh) for hh, d in enumerate(dots)], fill)
        ob_cp(S - UB * TB, UB * TB).start()


    scale_a = DH ** -0.5
    for nv in (1, 2):
        rm = L - 8 * nv
        rr = lax.broadcasted_iota(i32, (2 * rm, 2 * L), 0)
        cc = lax.broadcasted_iota(i32, (2 * rm, 2 * L), 1)
        rb_, cb_ = rr >= rm, cc >= L
        ri, ci = jnp.where(rb_, rr - rm, rr), jnp.where(cb_, cc - L, cc)
        same = rb_ == cb_
        cap_v[nv - 1, 0:2 * rm, :] = jnp.where(same & ((ri < M) | (ri + 8 * nv >= ci)), 1.0,
                                               jnp.where(same, -1e9, -jnp.inf)).astype(f32)
    slot_ok = (lax.broadcasted_iota(i32, (7, 8, 128), 0) + lax.broadcasted_iota(i32, (7, 8, 128), 1)) >= 7

    mem_s[...] = mem_v[...].astype(f32)
    xa_v[0:H, AK - 8:AK, :] = jnp.zeros((H, 8, 128), f32)
    xa_v[0:H, AV - 8:AV, :] = jnp.zeros((H, 8, 128), f32)
    NP = H // 2

    def a_step(lhs, even, z):
        qkv, pp, pend, lo, ya = {}, {}, {}, {}, {}
        nrow = 32 if even else 48

        def nv(hh):
            return 2 if hh // 2 in PAIRS2[0 if even else 1] else 1

        def dot(wi, hh, k0, k1):
            rows = 48 if even != (wi == 0) else 32
            return jnp.dot(lhs[0:rows, k0:k1], a_weight(wi * H + hh, k0, k1), preferred_element_type=f32)

        def proj(wi, hh):
            y = dot(wi, hh, DM // 2, DM) + lo[wi, hh] if (wi, hh) in lo else dot(wi, hh, 0, DM)
            if y.shape[0] == 48:
                t0 = y[32:40]
                stash[wi * H + hh] = y[40:48]
            else:
                t0 = stash[wi * H + hh]
            t, n = jnp.concatenate([y[0:8], t0, y[8:32]], axis=0), 8 * nv(hh)
            if wi == 0:
                xa_v[hh, AQ:AQ + n, :] = t[8:8 + n] * (scale_a * LOG2E)
                qkv[wi, hh] = jnp.concatenate([y[0:8], y[n:32]], axis=0)
            else:
                xa_v[hh, (AK, AV)[wi - 1]:(AK, AV)[wi - 1] + 8 + n, :] = t[0:8 + n]
                qkv[wi, hh] = t
            return y[y.shape[0] - 8:]

        def pair(wi, j):
            return jnp.concatenate([qkv.pop((wi, 2 * j)), qkv.pop((wi, 2 * j + 1))], axis=0).astype(bf16)

        def do_qk(j):
            q2, k2 = pair(0, j), pair(1, j)
            qkv[j] = pair(2, j)
            s = lax.dot_general(q2, k2, (((1,), (1,)), ((), ())), preferred_element_type=f32) * scale_a
            cap = cap_v[nv(2 * j) - 1, 0:s.shape[0], :]
            s = jnp.where(cap > 0, s, cap)
            m = jnp.max(s, axis=1, keepdims=True)
            e = jnp.exp(s - m)
            l = jnp.sum(e, axis=1, keepdims=True)
            rc = pl.reciprocal(l, approx=True)
            rc = rc * (2.0 - l * rc)
            pp[j] = (e * rc).astype(bf16)

        def do_pv(j):
            o2 = jnp.dot(pp.pop(j), qkv.pop(j), preferred_element_type=f32)
            for i, hh in enumerate((2 * j, 2 * j + 1)):
                rm = L - 8 * nv(hh)
                o = jnp.concatenate([o2[rm * i:rm * i + 8], xa_v[hh, AO:AO + 8 * nv(hh), :],
                                     o2[rm * i + 8:rm * (i + 1)]], axis=0)
                if even:
                    o_s[hh, 0:32, :] = o[0:32].astype(bf16)
                    ostash[hh] = o[32:40]
                else:
                    o_s[hh] = jnp.concatenate([o[0:8], ostash[hh], o[8:40]], axis=0).astype(bf16)

        def windows(hh, r, j0, j1):
            return jnp.concatenate([xa_v[hh:hh + 1, r + j - 7:r + j + 1, :] for j in range(j0, j1)], axis=0)

        def scores(hh, g):
            return sa_v.at[hh % 4] if g == 0 else sb_v.at[hh % 2]

        def v_qk(hh, g, j0, j1):
            q = xa_v[hh:hh + 1, AQ + 8 * g:AQ + 8 * g + 8, :]
            s = jnp.sum(q * windows(hh, AK, j0, j1), axis=2, keepdims=True)
            s = jnp.broadcast_to(s, (j1 - j0, 8, 128))
            if j0 == 0:
                s = jnp.concatenate([jnp.where(slot_ok, s[0:7], -jnp.inf), s[7:]], axis=0)
            scores(hh, g)[j0:j1] = s
            m = jnp.max(s, axis=0)
            pend[hh, g] = m if j0 == 0 else jnp.maximum(m, pend[hh, g])

        def v_max(hh, g):
            xa_v[hh, AM + 8 * g:AM + 8 * g + 8, :] = pend.pop((hh, g))

        def v_pv(hh, g, j0, j1):
            e = jnp.exp2(scores(hh, g)[j0:j1] - xa_v[hh:hh + 1, AM + 8 * g:AM + 8 * g + 8, :])
            l, o = jnp.sum(e, axis=0), jnp.sum(e * windows(hh, AV, j0, j1), axis=0)
            if j0 > 0:
                l, o = l + xa_v[hh, AL:AL + 8, :], o + xa_v[hh, AO + 8 * g:AO + 8 * g + 8, :]
            if j1 == 16 + 8 * g:
                rc = pl.reciprocal(l, approx=True)
                o = o * (rc * (2.0 - l * rc))
            else:
                xa_v[hh, AL:AL + 8, :] = l
            xa_v[hh, AO + 8 * g:AO + 8 * g + 8, :] = o

        work = {}
        for hh in range(H):
            d = 3 * hh
            put(work, d + 5, P(v_max, hh, 0))
            put(work, d + 6, P(v_pv, hh, 0, 0, 16))
            put(work, d + 2, P(v_qk, hh, 0, 0, 16))
            if nv(hh) == 2:
                d += 3 * (hh % 2)
                put(work, d + 2, P(v_qk, hh, 1, 0, 12))
                put(work, d + 5, P(v_qk, hh, 1, 12, 24))
                put(work, d + 8, P(v_max, hh, 1))
                put(work, d + 10, P(v_pv, hh, 1, 0, 12))
                put(work, d + 13, P(v_pv, hh, 1, 12, 24))

        def epoch(d, y):
            if not work and d > 3 * H + 4:
                return
            xa_v[z + H, 0:8, :] = y
            if d % 6 == 5 and d < 3 * H:
                qkv[1, d // 3] = jnp.concatenate([xa_v[d // 3, AK:AK + 8, :], qkv[1, d // 3][8:]], axis=0)
            for f in work.pop(d, []):
                f()

        def wo_part(n, h0, h1):
            lo = _lhs([_u32(o_s.at[hh, pl.ds(0, nrow), :]) for hh in range(h0, h1)])
            w = _u32(wo_v.at[n, pl.ds(h0 * DH, (h1 - h0) * DH), :])
            r = jnp.dot(lo, _b16(w), preferred_element_type=f32)
            ya[n] = r + ya[n] if n in ya else r
            return ya[n][0:8]

        ni = NI[0 if even else 1]
        pieces = [(n, 4 * g, 4 * g + 4) for g in range(ni) for n in range(NC)]
        d0, done = 6 * (LPV + 2), 0
        if not even:
            lo.update({(wi, hh): dot(wi, hh, 0, DM // 2) for hh in (0, 1) for wi in range(3)})
        for d in range(3 * H):
            y = proj(d % 3, d // 3)
            ready = NC * max(((d + 1) // 6 - LPV - 1 + (1 if (d + 1) % 6 else 0)) // 2, 0)
            while done < min((d - d0 + 1) * len(pieces) // (3 * H - d0), ready):
                wo_part(*pieces[done])
                done += 1
            if d % 6 == 5:
                if d // 6 >= LQK:
                    do_qk(d // 6 - LQK)
                if d // 6 >= LPV:
                    do_pv(d // 6 - LPV)
            epoch(d, y)
        assert done == len(pieces)
        nper, n = NC // (LPV + 1), 0
        for j in range(NP, NP + LPV):
            for _ in range(nper):
                y = wo_part(n, 4 * ni, 2 * KA)
                for d in range(3 * (H + n), 3 * (H + n + 1)):
                    epoch(d, y)
                n += 1
            if j - LQK < NP:
                do_qk(j - LQK)
            do_pv(j - LPV)
        for n in range(n, NC):
            wo_part(n, 4 * ni, 2 * KA)
        for n in range(NC):
            wo_part(n, 2 * KA, H)
        assert not work
        return jnp.concatenate([ya[n] for n in range(NC)], axis=1)

    def a_body(t, c):
        with _scope("a_it"):
            return a_pair(t, c)

    def a_pair(t, c):
        @pl.when(t > 0)
        def _():
            oa_cp(pl.multiple_of(jnp.maximum(t - 1, 0) * 64, 64), 64).start()
        z = zero_s[0]
        o0 = pl.multiple_of(t * 64, 64)
        o1 = pl.multiple_of(jnp.minimum(t * 64 + 64, S - 64), 64)
        X = _lhs([_u32(ax_v.at[j, pl.ds(o0, 64), :]) for j in range(NC)])
        X0, X2 = X[0:16].astype(f32), X[32:48].astype(f32)
        X4 = _lhs([_u32(ax_v.at[j, pl.ds(o1, 16), :]) for j in range(NC)]).astype(f32)

        def pk(a, b):
            return jnp.concatenate([a, b], axis=0).astype(bf16)
        ye = a_step(jnp.concatenate([pk(mem_s[...], X0[8:16]), X[16:32], pk(X0[0:8], X2[0:8])], axis=0), True, z)
        yo = a_step(jnp.concatenate([pk(ye[0:8], X2[8:16]), X[48:64], pk(X2[0:8], X4[0:8])], axis=0), False, z)
        mem_s[...] = yo[0:8]
        outa_v[pl.ds(o0, 64), :] = jnp.concatenate([ye[8:32], yo[8:48]], axis=0).astype(bf16)
        return c
    lax.fori_loop(0, S // 64, a_body, 0)
    oa_cp(S - 64, 64).start()

    ob_cp(0, S).wait()
    oa_cp(0, S).wait()


@jax.jit
def _run(A_x, A_mem0, A_Wq, A_Wk, A_Wv, A_Wo, B_x, B_wqkv, B_wo):
    hbm = pl.BlockSpec(memory_space=pl.ANY)
    known = {f.name for f in dataclasses.fields(pltpu.CompilerParams)}
    optional = {k: True for k in ("disable_bounds_checks", "disable_semaphore_checks") if k in known}
    out = pl.pallas_call(
        _kernel,
        out_shape=jax.ShapeDtypeStruct((S, 2 * DM), bf16),
        in_specs=[hbm] * 9,
        out_specs=hbm,
        scratch_shapes=[
            pltpu.VMEM((NC, S, 128), bf16),
            pltpu.VMEM((M, DM), bf16),
            pltpu.VMEM((STG_ROWS, 128), bf16),
            pltpu.VMEM((3 * DM // 16, H * PITCH + 8, 128), u32),
            pltpu.VMEM((NC, H * DH, 128), bf16),
            pltpu.VMEM((NC, S, 128), bf16),
            pltpu.VMEM((24, DM // 2, 128), u32),
            pltpu.VMEM((NC, 9 * OPITCH - 1, 128), u32),
            pltpu.VMEM((S, DM), bf16),
            pltpu.VMEM((S, DM), bf16),
            pltpu.VMEM((X_SLABS, TB + HALO, 128), f32),
            pltpu.VMEM((UB, 8, TB, 128), bf16),
            pltpu.VMEM((M, DM), f32),
            pltpu.VMEM((3 * H, 8, DH), f32),
            pltpu.VMEM((H, 8, DH), f32),
            pltpu.VMEM((H, 48, DH), bf16),
            pltpu.VMEM((H + 1, AROWS, 128), f32),
            pltpu.VMEM((4, 16, 8, 128), f32),
            pltpu.VMEM((2, 24, 8, 128), f32),
            pltpu.VMEM((2, 64, 2 * L), f32),
            pltpu.SMEM((1,), i32),
            pltpu.SemaphoreType.DMA((NSEM,)),
        ],
        compiler_params=pltpu.CompilerParams(vmem_limit_bytes=110 * 1024 * 1024, **optional),
    )(
        A_x.reshape(S, DM), A_mem0.reshape(M, DM),
        A_Wq.reshape(DM * H, DH), A_Wk.reshape(DM * H, DH), A_Wv.reshape(DM * H, DH),
        A_Wo.reshape(H * DH, DM),
        B_x.reshape(S, DM), B_wqkv, B_wo,
    )
    return out.reshape(1, S, 2 * DM)


def pallas_concat_heads__memory_aug_recurrent_mem_tr__sliding_local_dilated__prompt_kernel(
    A_x, A_mem0, A_Wq, A_Wk, A_Wv, A_Wo, A_seg_len, B_x, B_wqkv, B_wo,
):
    if isinstance(A_seg_len, int):
        assert A_seg_len == SEG
    return _run(A_x, A_mem0, A_Wq, A_Wk, A_Wv, A_Wo, B_x, B_wqkv, B_wo)
```
